```python
import jax
import jax.numpy as jnp

def _softmax(x, axis=-1):
    return jax.nn.softmax(x, axis=axis)
def _gelu(x):
    return jax.nn.gelu(x, approximate=True)
def _silu(x):
    return jax.nn.silu(x)
def _sigmoid(x):
    return jax.nn.sigmoid(x)
def _layernorm(x, axis=-1, eps=1e-5):
    m = jnp.mean(x, axis=axis, keepdims=True)
    v = jnp.var(x, axis=axis, keepdims=True)
    return (x - m) / jnp.sqrt(v + eps)
def _scatter_add(tgt, idx, src, axis=0):
    return tgt.at[idx].add(src)
def _segment_sum(src, seg, n):
    return jax.ops.segment_sum(src, seg, n)
class _Rng:
    def __init__(self, key):
        self._k = key
    def _next(self):
        self._k, sub = jax.random.split(self._k)
        return sub
    def normal(self, shape):
        return jax.random.normal(self._next(), shape, dtype=jnp.bfloat16)
    def randint(self, lo, hi, shape):
        return jax.random.randint(self._next(), shape, lo, hi, dtype=jnp.int32)
    def uniform(self, shape, lo=0.0, hi=1.0):
        return jax.random.uniform(self._next(), shape, jnp.bfloat16, lo, hi)
    def permutation(self, n):
        return jax.random.permutation(self._next(), n)


kernel_name = 'gated_mix__compressed_kv_cla__moe_arch_mod__prompt'

def setup_inputs():
    _rng = _Rng(jax.random.key(int.from_bytes(__import__("os").urandom(4), "little")))
    _w = (lambda a: (lambda t: t.astype(jnp.bfloat16) if jnp.issubdtype(t.dtype, jnp.floating) else t)(jnp.asarray(a)))
    def _A_setup():
        B, H, Sq, Sk, D, M = 1, 16, 2048, 2048, 256, 448
        Dc = 4 * D
        return {
            "x": _w((lambda *s: _rng.normal(s) * 0.05)(B, Sq, M)),
            "c_kv": _w((lambda *s: _rng.normal(s) * 0.05)(B, Sk, Dc)),
            "w_q": _w((lambda *s: _rng.normal(s) * 0.05)(M, H, D) * (M ** -0.5)),
            "w_uk": _w((lambda *s: _rng.normal(s) * 0.05)(Dc, H, D) * (Dc ** -0.5)),
            "w_uv": _w((lambda *s: _rng.normal(s) * 0.05)(Dc, H, D) * (Dc ** -0.5)),
            "w_o": _w((lambda *s: _rng.normal(s) * 0.05)(H, D, M) * ((H * D) ** -0.5)),
        }
    _A_in = _A_setup()

    def _B_setup():
        B, S, D, F, C = 1, 2048, 448, 1792, 2
        return {
            "x": _w((lambda *s: _rng.normal(s) * 0.05)(B, S, D)),
            "w_r": _w((lambda *s: _rng.normal(s) * 0.05)(D)),
            "w_gate": _w((lambda *s: _rng.normal(s) * 0.05)(D, F)),
            "w_up": _w((lambda *s: _rng.normal(s) * 0.05)(D, F)),
            "w_down": _w((lambda *s: _rng.normal(s) * 0.05)(F, D)),
        }
    _B_in = _B_setup()

    return {
        "A_x": _A_in["x"],
        "A_c_kv": _A_in["c_kv"],
        "A_w_q": _A_in["w_q"],
        "A_w_uk": _A_in["w_uk"],
        "A_w_uv": _A_in["w_uv"],
        "A_w_o": _A_in["w_o"],
        "B_x": _B_in["x"],
        "B_w_r": _B_in["w_r"],
        "B_w_gate": _B_in["w_gate"],
        "B_w_up": _B_in["w_up"],
        "B_w_down": _B_in["w_down"],
        "gate_w": _w((lambda *s: _rng.normal(s) * 0.05)(448)),
    }

def reference(A_x, A_c_kv, A_w_q, A_w_uk, A_w_uv, A_w_o, B_x, B_w_r, B_w_gate, B_w_up, B_w_down, gate_w):
    def _A_ref(x, c_kv, w_q, w_uk, w_uv, w_o):
        B, Sq, M = x.shape[0], x.shape[1], x.shape[2]
        Sk = c_kv.shape[1]
        H, D = w_q.shape[1], w_q.shape[2]
        q = jnp.einsum("bqm,mhd->bhqd", x, w_q)
        k = jnp.einsum("bkc,chd->bhkd", c_kv, w_uk)
        v = jnp.einsum("bkc,chd->bhkd", c_kv, w_uv)
        scores = jnp.einsum("bhqd,bhkd->bhqk", q, k) * (D ** -0.5)
        off = Sk - Sq
        qi = jnp.arange(Sq)[:, None]
        kj = jnp.arange(Sk)[None, :]
        cmask = kj <= (qi + off)
        scores = jnp.where(cmask[None, None], scores, -1e9)
        p = _softmax(scores, axis=-1)
        ctx = jnp.einsum("bhqk,bhkd->bhqd", p, v)
        return jnp.einsum("bhqd,hdm->bqm", ctx, w_o)

    def _B_ref(x, w_r, w_gate, w_up, w_down):
        B, S, D = x.shape
        C = 2
        r = x @ w_r
        idx = jnp.argsort(-r, axis=-1)[:, :C]
        idx_e = jnp.repeat(idx.reshape(B, C, 1), D, axis=2)
        x_sel = jnp.take_along_axis(x, idx_e, axis=1)
        g = _silu(x_sel @ w_gate)
        u = x_sel @ w_up
        y = (g * u) @ w_down
        r_sel = _sigmoid(jnp.take_along_axis(r, idx, axis=1))
        y = y * r_sel.reshape(B, C, 1)
        b_off = (jnp.arange(B) * S).reshape(B, 1)
        flat_idx = (idx + b_off).reshape(B * C)
        zero = (x * 0.0).reshape(B * S, D)
        upd = _scatter_add(zero, flat_idx, y.reshape(B * C, D), axis=0)
        return x + upd.reshape(B, S, D)

    x = A_x
    g = _sigmoid((x * gate_w).sum(-1, keepdims=True))
    a = _A_ref(x, A_c_kv, A_w_q, A_w_uk, A_w_uv, A_w_o)
    b = _B_ref(x, B_w_r, B_w_gate, B_w_up, B_w_down)
    return g * a + (1 - g) * b
```

```python
import functools
import math

import jax
import jax.numpy as jnp
from jax import lax
import jax.experimental.pallas as pl
import jax.experimental.pallas.tpu as pltpu

_NN = (((1,), (0,)), ((), ()))
_NT = (((1,), (1,)), ((), ()))
_LOG2E = math.log2(math.e)
_F32 = jnp.float32
_BF16 = jnp.bfloat16


def _dot(a, b, dims=_NN):
    return lax.dot_general(a, b, dims, preferred_element_type=_F32)


def _take_head(words, shift):
    bits = (words << shift) & jnp.uint32(0xFFFF0000)
    return pltpu.bitcast(bits, _F32)


def make(bq=256, flags=None):
    def kernel(xT_ref, c_ref, wq_hbm, wuk_hbm, wuv_hbm, woT_ref, wr_ref, wg_ref, wu_ref, wdT_ref, gw_ref,
               outT_ref, wq32, wuk32, wuv32, sems, qT_s, k_s, vT_s, acc_s):
        h = pl.program_id(0)
        n_heads = pl.num_programs(0)
        M, S = xT_ref.shape
        D = k_s.shape[1]
        pair = h // 2
        slot = pair % 2

        def copies(p, s):
            return [
                pltpu.make_async_copy(src.bitcast(jnp.uint32).at[:, p, :], dst.at[s], sems.at[i, s])
                for i, (src, dst) in enumerate(((wq_hbm, wq32), (wuk_hbm, wuk32), (wuv_hbm, wuv32)))
            ]

        @pl.when(h == 0)
        def _():
            for cp in copies(0, 0):
                cp.start()
            acc_s[...] = jnp.zeros_like(acc_s)

        @pl.when(h % 2 == 0)
        def _():
            @pl.when(pair + 1 < n_heads // 2)
            def _():
                for cp in copies(pair + 1, 1 - slot):
                    cp.start()
            for cp in copies(pair, slot):
                cp.wait()

        shift = (16 * (1 - h % 2)).astype(jnp.uint32)
        wuk = _take_head(wuk32[slot], shift).astype(_BF16)
        k_s[...] = _dot(c_ref[...], wuk).astype(_BF16)
        wqT = _take_head(wq32[slot], shift).T.astype(_BF16)
        qT_s[...] = (_dot(wqT, xT_ref[...]) * (D ** -0.5 * _LOG2E)).astype(_BF16)
        wuvT = _take_head(wuv32[slot], shift).T.astype(_BF16)
        vT_s[...] = _dot(wuvT, c_ref[...], _NT).astype(_BF16)

        row = lax.broadcasted_iota(jnp.int32, (bq, bq), 0)
        col = lax.broadcasted_iota(jnp.int32, (bq, bq), 1)
        causal = row <= col
        for i in range(S // bq):
            lo, hi = i * bq, (i + 1) * bq
            qT = qT_s[:, lo:hi]
            s_d = jnp.where(causal, _dot(k_s[lo:hi, :], qT), -1e9 * _LOG2E)
            m = jnp.max(s_d, axis=0, keepdims=True)
            if i > 0:
                s = _dot(k_s[:lo, :], qT)
                m = jnp.maximum(m, jnp.max(s, axis=0, keepdims=True))
            p_d = jnp.exp2(s_d - m)
            l = jnp.sum(p_d, axis=0, keepdims=True)
            ctx = _dot(vT_s[:, lo:hi], p_d.astype(_BF16))
            if i > 0:
                p = jnp.exp2(s - m)
                l = l + jnp.sum(p, axis=0, keepdims=True)
                ctx = ctx + _dot(vT_s[:, :lo], p.astype(_BF16))
            ctx = (ctx * (1.0 / l)).astype(_BF16)
            acc_s[:, lo:hi] += _dot(woT_ref[...], ctx)

        @pl.when(h == n_heads - 1)
        def _():
            xT = xT_ref[...]
            wr = wr_ref[...].astype(_F32).reshape(1, M)
            gw = gw_ref[...].astype(_F32).reshape(1, M)
            r16 = lax.broadcasted_iota(jnp.int32, (16, M), 0)
            lhs = jnp.where(r16 == 0, wr, jnp.where(r16 == 1, gw, 0.0)).astype(_BF16)
            rg = _dot(lhs, xT)
            r = rg[0:1].astype(_BF16).astype(_F32)
            gate = jax.nn.sigmoid(rg[1:2])
            tok = lax.broadcasted_iota(jnp.int32, (1, S), 1)
            m0 = jnp.max(r, axis=1, keepdims=True)
            i0 = jnp.min(jnp.where(r == m0, tok, S), axis=1, keepdims=True)
            r1 = jnp.where(tok == i0, -jnp.inf, r)
            m1 = jnp.max(r1, axis=1, keepdims=True)
            i1 = jnp.min(jnp.where((r1 == m1) & (tok != i0), tok, S), axis=1, keepdims=True)
            t16 = lax.broadcasted_iota(jnp.int32, (16, S), 0)
            tok16 = lax.broadcasted_iota(jnp.int32, (16, S), 1)
            onehot = jnp.where(((t16 == 0) & (tok16 == i0)) | ((t16 == 1) & (tok16 == i1)), 1.0, 0.0).astype(_BF16)
            x_sel = _dot(onehot, xT, _NT).astype(_BF16)
            g = jax.nn.silu(_dot(x_sel, wg_ref[...]))
            u = _dot(x_sel, wu_ref[...])
            y = _dot((g * u).astype(_BF16), wdT_ref[...], _NT)
            rs = jnp.where(r16[:, 0:1] == 0, m0, m1)
            y = y * jax.nn.sigmoid(rs)
            yT = jnp.concatenate([y, jnp.zeros((112, M), _F32)], axis=0).T
            upd = jnp.where(tok == i0, yT[:, 0:1], 0.0) + jnp.where(tok == i1, yT[:, 1:2], 0.0)
            b = xT.astype(_F32) + upd
            outT_ref[...] = (gate * acc_s[...] + (1.0 - gate) * b).astype(outT_ref.dtype)

    def fn(A_x, A_c_kv, A_w_q, A_w_uk, A_w_uv, A_w_o, B_x, B_w_r, B_w_gate, B_w_up, B_w_down, gate_w):
        del B_x
        _, S, M = A_x.shape
        Dc, H, D = A_w_uk.shape
        F = B_w_gate.shape[1]
        whole = lambda shape: pl.BlockSpec(shape, lambda h: (0,) * len(shape))
        hbm = pl.BlockSpec(memory_space=pl.ANY)
        outT = pl.pallas_call(
            kernel,
            grid=(H,),
            in_specs=[whole((M, S)), whole((S, Dc)), hbm, hbm, hbm,
                      pl.BlockSpec((None, M, D), lambda h: (h, 0, 0)),
                      whole((M,)), whole((M, F)), whole((M, F)), whole((M, F)), whole((M,))],
            out_specs=whole((M, S)),
            out_shape=jax.ShapeDtypeStruct((M, S), A_x.dtype),
            scratch_shapes=[
                pltpu.VMEM((2, M, D), jnp.uint32), pltpu.VMEM((2, Dc, D), jnp.uint32), pltpu.VMEM((2, Dc, D), jnp.uint32),
                pltpu.SemaphoreType.DMA((3, 2)),
                pltpu.VMEM((D, S), _BF16), pltpu.VMEM((S, D), _BF16), pltpu.VMEM((D, S), _BF16),
                pltpu.VMEM((M, S), _F32),
            ],
            compiler_params=pltpu.CompilerParams(dimension_semantics=("arbitrary",), vmem_limit_bytes=110 * 2**20, flags=flags),
            name="gm_kernel",
        )(A_x[0].T, A_c_kv[0], A_w_q, A_w_uk, A_w_uv, A_w_o.transpose(0, 2, 1), B_w_r, B_w_gate, B_w_up, B_w_down.T, gate_w)
        return outT.T[None]
    return fn


@jax.jit
def pallas_gated_mix__compressed_kv_cla__moe_arch_mod__prompt_kernel(
    A_x, A_c_kv, A_w_q, A_w_uk, A_w_uv, A_w_o, B_x, B_w_r, B_w_gate, B_w_up, B_w_down, gate_w
):
    return make()(A_x, A_c_kv, A_w_q, A_w_uk, A_w_uv, A_w_o, B_x, B_w_r, B_w_gate, B_w_up, B_w_down, gate_w)
```

```python
import contextlib
import functools
import math

import jax
import jax.numpy as jnp
from jax import lax
import jax.experimental.pallas as pl
import jax.experimental.pallas.tpu as pltpu

_NN = (((1,), (0,)), ((), ()))
_NT = (((1,), (1,)), ((), ()))
_LOG2E = math.log2(math.e)
_F32 = jnp.float32
_BF16 = jnp.bfloat16
_U32 = jnp.uint32
_T = 128


def _dot(a, b, dims=_NN):
    return lax.dot_general(a, b, dims, preferred_element_type=_F32)


def _lhs_operands(a11, a12, a21, a22):
    return (a11 + a22, a21 + a22, a11, a22, a11 + a12, a21 - a11, a12 - a22)


def _rhs_operands(b11, b12, b21, b22):
    return (b11 + b22, b11, b12 - b22, b21 - b11, b22, b11 + b12, b21 + b22)


def _combine(m1, m2, m3, m4, m5, m6, m7):
    c21 = m4 if m2 is None else m2 + m4
    c12 = m3 + m5
    c22 = (m1 + m3 if m2 is None else m1 - m2 + m3) + m6
    c11 = None if m7 is None else (m1 + m4 - m5)[:m7.shape[0]] + m7
    return c11, c12, c21, c22


def _rows(ref, lead, lo, hi):
    return pltpu.bitcast(ref.bitcast(_U32)[(*lead, slice(lo // 2, hi // 2))], _BF16)


def _cat(xs, axis):
    xs = list(xs)
    return xs[0] if len(xs) == 1 else jnp.concatenate(xs, axis=axis)


def _fold(x):
    return functools.reduce(jnp.add, [x[r:r + 8] for r in range(0, x.shape[0], 8)])


def _merge(streams):
    keyed = []
    for s, steps in enumerate(streams):
        total = sum(c for c, _ in steps)
        done = 0
        for c, fn in steps:
            keyed.append(((done + c / 2) / total, s, len(keyed), fn))
            done += c
    return [fn for *_, fn in sorted(keyed, key=lambda t: t[:3])]


def make(flags=None, pchunk=16, kchunk=8, opaque="kqvc", nh=16, scopes=False,
         dma="wk c0 wv c1 c2 c3 c4 c5 vec wq x0 x1 c6 c7",
         first="wk c0 K0 wv V0 c1 K1 V1 c2 K2 V2 c3 K3 V3 c4 K4 V4 c5 K5 V5 wq x0 Q0-2 Q2-4 x1 Q4-6 Q6-8 route c6 K6 V6 c7 K7 V7",
         a="wk wq wv ffn; K0-8 V0-2 V2-4 V4-6 V6-8 | O0 O1 Q0-2 O2 O3 Q2-4 O4 O5 Q4-6 O6 O7 Q6-8",
         b="S1 S0 S2 C0 C1 S3 C2 S4 C3 S5 C4 S6 C5 S7 C6 C7"):
    scope = jax.named_scope if scopes else (lambda name: contextlib.nullcontext())

    def kernel(xT_hbm, c_hbm, wq_hbm, wuk_hbm, wuv_hbm, woT_hbm, wr_hbm, wg_hbm, wu_hbm, wdT_hbm, gw_hbm,
               outT_hbm,
               wq32, wuk32, wuv32, woT_s, wsems, xT_s, c_s, wg_s, wu_s, wdT_s, wr_s, gw_s, out_s, sems,
               xops, cops, wq_s, wk_s, wv_s, wo_s, q_s, k_s, v_s, p_s, ctx_s, acc_s, base_s,
               gate_s, r_s, xsel_s, y_s, scale_s, idx_s):
        M, S = xT_s.shape
        Dc = c_s.shape[1]
        D = wq32.shape[2]
        F = wg_s.shape[1]
        U = S // (2 * _T)
        mh = M // 2
        kt = Dc // 2 // _T
        weights = {"wq": (wq_hbm, wq32, wq_s, 0), "wk": (wuk_hbm, wuk32, wk_s, 1), "wv": (wuv_hbm, wuv32, wv_s, 2)}

        def w_copy(name, pair):
            src, dst, _, i = weights[name]
            return pltpu.make_async_copy(src.bitcast(_U32).at[:, pair, :], dst.at[pair % 2], wsems.at[i, pair % 2])

        def wo_copy(head):
            return pltpu.make_async_copy(woT_hbm.at[head], woT_s.at[head % 2], wsems.at[3, head % 2])

        copies = {n: [w_copy(n, 0)] for n in weights}
        for u in range(U):
            rows = slice(2 * u * _T, 2 * (u + 1) * _T)
            copies[f"c{u}"] = [pltpu.make_async_copy(c_hbm.at[rows], c_s.at[rows], sems.at[u])]
            copies[f"o{u}"] = [pltpu.make_async_copy(out_s.at[:, rows], outT_hbm.at[:, rows], sems.at[u])]
        for g in range(2):
            cols = slice(g * S // 2, (g + 1) * S // 2)
            copies[f"x{g}"] = [pltpu.make_async_copy(xT_hbm.at[:, cols], xT_s.at[:, cols], sems.at[U + g])]
        copies["vec"] = [pltpu.make_async_copy(wr_hbm, wr_s, sems.at[U + 2]),
                         pltpu.make_async_copy(gw_hbm, gw_s, sems.at[U + 3])]
        copies["ffn"] = [pltpu.make_async_copy(src, dst, sems.at[U + 4 + i])
                         for i, (src, dst) in enumerate(((wg_hbm, wg_s), (wu_hbm, wu_s), (wdT_hbm, wdT_s)))]

        def wait(name):
            for cp in copies[name]:
                cp.wait()

        def tile(name, ref, j):
            return ref[j] if name in opaque else _rows(ref, (j,), 0, _T)

        def weight_operands(name, head):
            _, w32, dst, _ = weights[name]
            transpose = name != "wk"
            slot = (head // 2) % 2
            shift = jnp.asarray(16 * (1 - head % 2)).astype(_U32)
            fb = w32.shape[1] // 2
            step = _T if transpose else 16
            for r in range(0, fb, step):
                rows = min(step, fb - r)
                quads = []
                for f in range(2):
                    for n in range(2):
                        w = w32[slot, f * fb + r:f * fb + r + rows, n * _T:(n + 1) * _T]
                        w = w.T if transpose else w
                        quads.append(pltpu.bitcast((w << shift) & _U32(0xFFFF0000), _F32))
                for i, op in enumerate(_rhs_operands(*quads)):
                    if transpose:
                        if rows < _T:
                            op = jnp.concatenate([op, jnp.zeros((_T, _T - rows), _F32)], axis=1)
                        dst[i, r // _T] = op.astype(_BF16)
                    else:
                        dst[i, r:r + rows] = op.astype(_BF16)

        def wo_operands(head):
            for r in range(0, mh, 16):
                top = woT_s[head % 2, r:r + 16, :].astype(_F32)
                bot = woT_s[head % 2, mh + r:mh + r + 16, :].astype(_F32)
                for i, op in enumerate(_lhs_operands(top[:, :_T], top[:, _T:], bot[:, :_T], bot[:, _T:])):
                    wo_s[i, r:r + 16] = op.astype(_BF16)

        def c_operands(u):
            fb = Dc // 2
            for r in range(0, _T, 16):
                ca = c_s[2 * u * _T + r:2 * u * _T + r + 16, :].astype(_F32)
                cb = c_s[(2 * u + 1) * _T + r:(2 * u + 1) * _T + r + 16, :].astype(_F32)
                for i, op in enumerate(_lhs_operands(ca[:, :fb], ca[:, fb:], cb[:, :fb], cb[:, fb:])):
                    for t in range(kt):
                        cops[i, t, u * _T + r:u * _T + r + 16] = op[:, t * _T:(t + 1) * _T].astype(_BF16)

        def column(vec_ref):
            return jnp.broadcast_to(vec_ref[...].astype(_F32).reshape(1, M), (_T, M)).T

        def x_operands(u, wr, gw):
            cols = slice(2 * u * _T, 2 * (u + 1) * _T)
            dots = [None] * 4
            for r in range(0, mh, 16):
                xf = [xT_s[f * mh + r:f * mh + r + 16, cols].astype(_F32) for f in range(2)]
                for i, op in enumerate(_lhs_operands(xf[0][:, :_T], xf[1][:, :_T], xf[0][:, _T:], xf[1][:, _T:])):
                    xops[i, u, r:r + 16] = op.astype(_BF16)
                for i, (w, half) in enumerate(((wr, 0), (wr, 1), (gw, 0), (gw, 1))):
                    t = _fold(functools.reduce(jnp.add, [
                        xf[f][:, half * _T:(half + 1) * _T] * w[f * mh + r:f * mh + r + 16] for f in range(2)]))
                    dots[i] = t if dots[i] is None else dots[i] + t
            dots = [jnp.sum(d, axis=0, keepdims=True) for d in dots]
            gates = [jax.nn.sigmoid(d) for d in dots[2:]]
            for half in range(2):
                r_s[2 * u + half:2 * u + half + 1] = dots[half].astype(_BF16).astype(_F32)
                gate_s[2 * u + half:2 * u + half + 1] = gates[half]
            keep = 1.0 - jnp.concatenate(gates, axis=1)
            for r in range(0, M, 16):
                base_s[r:r + 16, cols] = keep * xT_s[r:r + 16, cols].astype(_F32)

        lane = lax.broadcasted_iota(jnp.int32, (1, _T), 1)

        def token_tile(i):
            return pl.ds(pl.multiple_of(i // _T * _T, _T), _T)

        def route():
            r = r_s[...]
            r = jnp.where(r == r, r, -jnp.inf)
            tok = (lax.broadcasted_iota(jnp.int32, r.shape, 0) * _T
                   + lax.broadcasted_iota(jnp.int32, r.shape, 1))
            tokf = tok.astype(_F32)
            live = tok >= 0
            for n in range(2):
                best = jnp.max(jnp.where(live, r, -jnp.inf), keepdims=True)
                pick = jnp.min(jnp.where(live & (r == best), tokf, S - 1.0))
                hit = tokf == pick
                i = pick.astype(jnp.int32)
                idx_s[n] = i
                live = live & ~hit
                keep = jnp.sum(jnp.where(hit, 1.0 - gate_s[...], 0.0), keepdims=True)
                scale_s[n:n + 1] = jnp.broadcast_to(jax.nn.sigmoid(best) * keep, (1, _T))
                x = xT_s[:, token_tile(i)].astype(_F32)
                x = jnp.sum(jnp.where(lane == i % _T, x, 0.0), axis=1, keepdims=True)
                xsel_s[n] = jnp.broadcast_to(x, (M, _T))

        def ffn_chunk(chunk):
            cols = pl.ds(pl.multiple_of(jnp.minimum(chunk, F // _T - 1) * _T, _T), _T)
            wg = wg_s[:, cols].astype(_F32)
            wu = wu_s[:, cols].astype(_F32)
            wd = wdT_s[:, cols].astype(_F32)
            for n in range(2):
                x = xsel_s[n]
                g = jnp.sum(_fold(x * wg), axis=0, keepdims=True)
                up = jnp.sum(_fold(x * wu), axis=0, keepdims=True)
                hidden = jnp.where(chunk < F // _T, g * jax.nn.sigmoid(g) * up, 0.0)
                y_s[n] += wd * hidden

        def scatter():
            for n in range(2):
                i = idx_s[n]
                y = jnp.sum(y_s[n], axis=1, keepdims=True) * scale_s[n:n + 1]
                base_s[:, token_tile(i)] += jnp.where(lane == i % _T, y, 0.0)

        def seven(costs, product, finish):
            m = [None] * 7

            def step(j):
                m[j] = product(j) if costs[j] else None
                if j == 6:
                    finish(*m)
            return [(costs[j], functools.partial(step, j)) for j in range(7)]

        def c_operand(i, u0, u1):
            return _cat([_rows(cops, (i, t), u0 * _T, u1 * _T) for t in range(kt)], 1)

        def k_proj(u0, u1):
            def finish(*m):
                ka0, ka1, kb0, kb1 = _combine(*m)
                for i, op in enumerate(_lhs_operands(kb0, kb1, ka0, ka1)):
                    for u in range(u0, u1):
                        k_s[u][i] = op[(u - u0) * _T:(u - u0 + 1) * _T].astype(_BF16)
            return seven([kt * (u1 - u0) * _T] * 7,
                         lambda i: _dot(c_operand(i, u0, u1), _rows(wk_s, (i,), 0, Dc // 2)), finish)

        def q_proj(u0, u1):
            def prod(i):
                w = _cat([_rows(wq_s, (i, t), 0, _T) for t in range(2)], 1)[:, :mh]
                return _dot(w, _cat([_rows(xops, (i, u), 0, mh) for u in range(u0, u1)], 1))

            def finish(*m):
                qa0, qa1, qb0, qb1 = (q * (D ** -0.5 * _LOG2E) for q in _combine(*m))
                for i, op in enumerate(_rhs_operands(qa0, qb0, qa1, qb1)):
                    for u in range(u0, u1):
                        q_s[u][i] = op[:, (u - u0) * _T:(u - u0 + 1) * _T].astype(_BF16)
            return seven([2 * (u1 - u0) * _T] * 7, prod, finish)

        def v_proj(u0, u1):
            def prod(i):
                return _dot(_cat([_rows(wv_s, (i, t), 0, _T) for t in range(kt)], 1), c_operand(i, u0, u1), _NT)

            def finish(*m):
                va0, va1, vb0, vb1 = _combine(*m)
                for i, op in enumerate(_lhs_operands(vb0, va0, vb1, va1)):
                    for u in range(u0, u1):
                        v_s[u][i] = op[:, (u - u0) * _T:(u - u0 + 1) * _T].astype(_BF16)
            return seven([kt * (u1 - u0) * _T] * 7, prod, finish)

        svals = {}

        def mask_last(s):
            causal = (lax.broadcasted_iota(jnp.int32, (_T, _T), 0) <= lax.broadcasted_iota(jnp.int32, (_T, _T), 1))
            n = s.shape[0] - _T
            d = jnp.where(causal, s[n:], -1e9 * _LOG2E)
            return d if n == 0 else jnp.concatenate([s[:n], d], axis=0)

        def scores(u, _):
            n = u * _T
            rows = [n + _T] * 6 + [n]

            def prod(j):
                return _dot(_cat([tile("k", k_s[t], j) for t in range(rows[j] // _T)], 0), tile("q", q_s[u], j))

            def finish(*m):
                s_ba, s_bb, s_aa, s_ab = _combine(*m)
                s_aa = mask_last(s_aa)
                s_bb = mask_last(s_bb)
                m_a = jnp.max(s_aa, axis=0, keepdims=True)
                if n:
                    m_a = jnp.maximum(m_a, jnp.max(s_ba, axis=0, keepdims=True))
                m_b = jnp.maximum(jnp.max(s_bb, axis=0, keepdims=True), jnp.max(s_ab, axis=0, keepdims=True))
                svals[u] = (s_ba, s_bb, s_aa, s_ab, m_a, m_b)
            return seven(rows, prod, finish)

        def context(u, _):
            n = u * _T
            acc = [None] * 7
            sums = [None, None]

            def probs(lo, hi):
                s_ba, s_bb, s_aa, s_ab, m_a, m_b = svals[u]
                for r in range(lo, hi, pchunk):
                    p_bb = jnp.exp2(s_bb[r:r + pchunk] - m_b)
                    p_aa = jnp.exp2(s_aa[r:r + pchunk] - m_a)
                    p_ab = jnp.exp2(s_ab[r:r + pchunk] - m_b)
                    if r < n:
                        p_ba = jnp.exp2(s_ba[r:r + pchunk] - m_a)
                        ops = _rhs_operands(p_ba, p_bb, p_aa, p_ab)
                        t_a = p_aa + p_ba
                    else:
                        ops = (p_ab, None, p_bb - p_ab, p_aa, p_ab, p_bb, p_aa + p_ab)
                        t_a = p_aa
                    for i, t in enumerate((_fold(t_a), _fold(p_ab + p_bb))):
                        sums[i] = t if sums[i] is None else sums[i] + t
                    for i, op in enumerate(ops):
                        if op is not None:
                            p_s[u][r // _T][i, r % _T:r % _T + pchunk] = op.astype(_BF16)

            def finish():
                c0a, c0b, c1a, c1b = _combine(*acc)
                f_a, f_b = (gate_s[2 * u + i:2 * u + i + 1] / jnp.sum(sums[i], axis=0, keepdims=True)
                            for i in range(2))
                for i, op in enumerate(_rhs_operands(c0a * f_a, c0b * f_b, c1a * f_a, c1b * f_b)):
                    ctx_s[u][i] = op.astype(_BF16)

            def step(j, t0, t1):
                if j == 0:
                    probs(t0 * _T, t1 * _T)
                e = min(t1, u) if j == 1 else t1
                if e > t0:
                    m = _dot(_cat([tile("v", v_s[t], j) for t in range(t0, e)], 1),
                             _cat([tile("p", p_s[u][t], j) for t in range(t0, e)], 0))
                    acc[j] = m if acc[j] is None else acc[j] + m
                if j == 6 and t1 == u + 1:
                    finish()
            nchunks = -(-(u + 1) // kchunk)
            edges = [(u + 1) * i // nchunks for i in range(nchunks + 1)]
            return [((t1 - t0) * _T, functools.partial(step, j, t0, t1))
                    for t0, t1 in zip(edges, edges[1:]) for j in range(7)]

        def out_product(j, u0, u1):
            return _dot(_rows(wo_s, (j,), 0, mh), _cat([tile("c", ctx_s[u], j) for u in range(u0, u1)], 1))

        def project(u0, u1):
            def step(j):
                m = out_product(j, u0, u1)
                for u in range(u0, u1):
                    acc_s[u][j] += m[:, (u - u0) * _T:(u - u0 + 1) * _T]
            return [((u1 - u0) * mh, functools.partial(step, j)) for j in range(7)]

        def run(program, extra):
            def task(t):
                if t in extra:
                    return [(1e-3, extra[t])]
                rng = [int(x) for x in t[1:].split("-")]
                f = {"K": k_proj, "Q": q_proj, "V": v_proj, "O": project, "S": scores, "C": context}[t[0]]
                return f(rng[0], rng[1] if len(rng) > 1 else rng[0] + 1)
            for phase in program.split(";"):
                for fn in _merge([[st for t in s.split() for st in task(t)] for s in phase.split("|")]):
                    fn()

        with scope("first"):
            for name in dma.split() + ["ffn"]:
                for cp in copies[name]:
                    cp.start()
            for u in range(U):
                acc_s[u][...] = jnp.zeros_like(acc_s[u])
            y_s[...] = jnp.zeros_like(y_s)
            cols = []

            def first_w(name):
                wait(name)
                weight_operands(name, 0)

            def first_c(u):
                wait(f"c{u}")
                c_operands(u)

            def first_x(g):
                if not cols:
                    wait("vec")
                    cols.extend([column(wr_s), column(gw_s)])
                wait(f"x{g}")
                for u in range(g * U // 2, (g + 1) * U // 2):
                    x_operands(u, *cols)
            extra = {n: functools.partial(first_w, n) for n in weights}
            extra.update({f"c{u}": functools.partial(first_c, u) for u in range(U)})
            extra.update({f"x{g}": functools.partial(first_x, g) for g in range(2)})
            extra["route"] = route
            run(first, extra)

        def head_step(h, carry):
            wo_copy(h).start()

            @pl.when((h % 2 == 0) & (h + 2 < nh))
            def _():
                for name in weights:
                    w_copy(name, h // 2 + 1).start()

            with scope("attn"):
                run(b, {})
            wo_copy(h).wait()

            @pl.when(h == 0)
            def _():
                wait("ffn")

            @pl.when(h + 1 < nh)
            def _():
                @pl.when(h % 2 == 1)
                def _():
                    for name in weights:
                        w_copy(name, h // 2 + 1).wait()
                with scope("proj"):
                    wo_operands(h)
                    extra = {n: functools.partial(weight_operands, n, h + 1) for n in weights}
                    extra["ffn"] = functools.partial(ffn_chunk, h)
                    run(a, extra)
            return carry

        lax.fori_loop(0, nh, head_step, None)

        with scope("last"):
            wo_operands(nh - 1)
            scatter()
            for u in range(U):
                o = _combine(*(acc_s[u][j] + out_product(j, u, u + 1) for j in range(7)))
                cols_u = slice(2 * u * _T, 2 * (u + 1) * _T)
                for half in range(2):
                    rows = slice(half * mh, (half + 1) * mh)
                    new = base_s[rows, cols_u] + jnp.concatenate(o[2 * half:2 * half + 2], axis=1)
                    out_s[rows, cols_u] = new.astype(out_s.dtype)
                copies[f"o{u}"][0].start()
            for u in range(U):
                wait(f"o{u}")

    def fn(A_x, A_c_kv, A_w_q, A_w_uk, A_w_uv, A_w_o, B_x, B_w_r, B_w_gate, B_w_up, B_w_down, gate_w):
        del B_x
        _, S, M = A_x.shape
        Dc, H, D = A_w_uk.shape
        F = B_w_gate.shape[1]
        U = S // (2 * _T)
        tile = pltpu.VMEM((7, _T, _T), _BF16)
        hbm = pl.BlockSpec(memory_space=pl.ANY)
        outT = pl.pallas_call(
            kernel,
            in_specs=[hbm] * 11,
            out_specs=hbm,
            out_shape=jax.ShapeDtypeStruct((M, S), A_x.dtype),
            scratch_shapes=[
                pltpu.VMEM((2, M, D), _U32), pltpu.VMEM((2, Dc, D), _U32), pltpu.VMEM((2, Dc, D), _U32),
                pltpu.VMEM((2, M, D), _BF16),
                pltpu.SemaphoreType.DMA((4, 2)),
                pltpu.VMEM((M, S), _BF16), pltpu.VMEM((S, Dc), _BF16),
                pltpu.VMEM((M, F), _BF16), pltpu.VMEM((M, F), _BF16), pltpu.VMEM((M, F), _BF16),
                pltpu.VMEM((M,), _BF16), pltpu.VMEM((M,), _BF16), pltpu.VMEM((M, S), _BF16),
                pltpu.SemaphoreType.DMA((U + 7,)),
                pltpu.VMEM((7, U, M // 2, _T), _BF16), pltpu.VMEM((7, Dc // 2 // _T, S // 2, _T), _BF16),
                pltpu.VMEM((7, 2, _T, _T), _BF16), pltpu.VMEM((7, Dc // 2, _T), _BF16),
                pltpu.VMEM((7, Dc // 2 // _T, _T, _T), _BF16), pltpu.VMEM((7, M // 2, _T), _BF16),
                [tile] * U, [tile] * U, [tile] * U,
                [[tile] * (u + 1) for u in range(U)],
                [tile] * U,
                [pltpu.VMEM((7, M // 2, _T), _F32)] * U, pltpu.VMEM((M, S), _F32),
                pltpu.VMEM((2 * U, _T), _F32), pltpu.VMEM((2 * U, _T), _F32),
                pltpu.VMEM((2, M, _T), _F32), pltpu.VMEM((2, M, _T), _F32), pltpu.VMEM((8, _T), _F32),
                pltpu.SMEM((2,), jnp.int32),
            ],
            compiler_params=pltpu.CompilerParams(vmem_limit_bytes=110 * 2**20, flags=flags),
            name="gm_kernel",
        )(A_x[0].T, A_c_kv[0], A_w_q, A_w_uk, A_w_uv, A_w_o.transpose(0, 2, 1), B_w_r, B_w_gate, B_w_up, B_w_down.T, gate_w)
        return outT.T[None]
    return fn


@jax.jit
def pallas_gated_mix__compressed_kv_cla__moe_arch_mod__prompt_kernel(
    A_x, A_c_kv, A_w_q, A_w_uk, A_w_uv, A_w_o, B_x, B_w_r, B_w_gate, B_w_up, B_w_down, gate_w
):
    return make()(A_x, A_c_kv, A_w_q, A_w_uk, A_w_uv, A_w_o, B_x, B_w_r, B_w_gate, B_w_up, B_w_down, gate_w)
```

```python
import contextlib
import functools
import math

import jax
import jax.numpy as jnp
from jax import lax
import jax.experimental.pallas as pl
import jax.experimental.pallas.tpu as pltpu

_NN = (((1,), (0,)), ((), ()))
_NT = (((1,), (1,)), ((), ()))
_LOG2E = math.log2(math.e)
_F32 = jnp.float32
_BF16 = jnp.bfloat16
_U32 = jnp.uint32
_T = 128


def _dot(a, b, dims=_NN):
    return lax.dot_general(a, b, dims, preferred_element_type=_F32)


def _lhs_operands(a11, a12, a21, a22):
    return (a11 + a22, a21 + a22, a11, a22, a11 + a12, a21 - a11, a12 - a22)


def _rhs_operands(b11, b12, b21, b22):
    return (b11 + b22, b11, b12 - b22, b21 - b11, b22, b11 + b12, b21 + b22)


def _combine(m1, m2, m3, m4, m5, m6, m7):
    c21 = m4 if m2 is None else m2 + m4
    c12 = m3 + m5
    c22 = (m1 + m3 if m2 is None else m1 - m2 + m3) + m6
    c11 = None if m7 is None else (m1 + m4 - m5)[:m7.shape[0]] + m7
    return c11, c12, c21, c22


def _rows(ref, lead, lo, hi):
    return pltpu.bitcast(ref.bitcast(_U32)[(*lead, slice(lo // 2, hi // 2))], _BF16)


def _cat(xs, axis):
    xs = list(xs)
    return xs[0] if len(xs) == 1 else jnp.concatenate(xs, axis=axis)


def _fold(x):
    return functools.reduce(jnp.add, [x[r:r + 8] for r in range(0, x.shape[0], 8)])


def _merge(streams):
    keyed = []
    for s, steps in enumerate(streams):
        total = sum(c for c, _ in steps)
        done = 0
        for c, fn in steps:
            keyed.append(((done + c / 2) / total, s, len(keyed), fn))
            done += c
    return [fn for *_, fn in sorted(keyed, key=lambda t: t[:3])]


def make(flags=None, pchunk=16, kchunk=8, opaque="", nh=16, scopes=False,
         dma="wk c0 wv c1 c2 c3 c4 c5 vec wq x0 x1 c6 c7",
         first="!wk wk !c0 c0 K0 !wv wv V0 !c1 c1 K1 V1 !c2 !c3 c2 c3 K2-4 V2-4 !c4 !c5 !vec !wq c4 c5 wq K4-6 V4-6 !x0 !x1 !c6 c6 x0; K6 V6 | R0-8; Q0-2 Q2-4; !c7 c7 x1 route K7 Q4-6; V7 | Q6-8",
         a="wk wq wv ffn O0 O1 O2; K0-2 K2-8 V0-2 V2-4 V4-6 V6-8 | O3 Q0-2 Q2-4 O4 Q4-6 Q6-8 O5; O6 O7",
         b=([[2, 0, 1], [3], [4], [5], [6], [7]], 3), defer=None, corder=(4, 1, 0, 6, 3, 5, 2)):
    scope = jax.named_scope if scopes else (lambda name: contextlib.nullcontext())

    def kernel(xT_hbm, c_hbm, wq_hbm, wuk_hbm, wuv_hbm, woT_hbm, wr_hbm, wg_hbm, wu_hbm, wdT_hbm, gw_hbm,
               outT_hbm,
               wq32, wuk32, wuv32, woT_s, wsems, xT_s, c_s, wg_s, wu_s, wdT_s, wr_s, gw_s, out_s, sems,
               xops, cops, wq_s, wk_s, wv_s, wo_s, q_s, k_s, v_s, s_s, p_s, ctx_s, acc_s,
               gate_s, r_s, xsel_s, y_s, scale_s, raw_s, idx_s):
        M, S = xT_s.shape
        Dc = c_s.shape[1]
        D = wq32.shape[2]
        F = wg_s.shape[1]
        U = S // (2 * _T)
        mh = M // 2
        kt = Dc // 2 // _T
        weights = {"wq": (wq_hbm, wq32, wq_s, 0), "wk": (wuk_hbm, wuk32, wk_s, 1), "wv": (wuv_hbm, wuv32, wv_s, 2)}

        def w_copy(name, pair):
            src, dst, _, i = weights[name]
            return pltpu.make_async_copy(src.bitcast(_U32).at[:, pair, :], dst.at[pair % 2], wsems.at[i, pair % 2])

        def wo_copy(head):
            return pltpu.make_async_copy(woT_hbm.at[head], woT_s.at[head % 2], wsems.at[3, head % 2])

        copies = {n: [w_copy(n, 0)] for n in weights}
        for u in range(U):
            rows = slice(2 * u * _T, 2 * (u + 1) * _T)
            copies[f"c{u}"] = [pltpu.make_async_copy(c_hbm.at[rows], c_s.at[rows], sems.at[u])]
            copies[f"o{u}"] = [pltpu.make_async_copy(out_s.at[:, rows], outT_hbm.at[:, rows], sems.at[u])]
        for g in range(2):
            cols = slice(g * S // 2, (g + 1) * S // 2)
            copies[f"x{g}"] = [pltpu.make_async_copy(xT_hbm.at[:, cols], xT_s.at[:, cols], sems.at[U + g])]
        copies["vec"] = [pltpu.make_async_copy(wr_hbm, wr_s, sems.at[U + 2]),
                         pltpu.make_async_copy(gw_hbm, gw_s, sems.at[U + 3])]
        copies["ffn"] = [pltpu.make_async_copy(src, dst, sems.at[U + 4 + i])
                         for i, (src, dst) in enumerate(((wg_hbm, wg_s), (wu_hbm, wu_s), (wdT_hbm, wdT_s)))]

        def wait(name):
            for cp in copies[name]:
                cp.wait()

        def tile(name, ref, j):
            return ref[j] if name in opaque else _rows(ref, (j,), 0, _T)

        def weight_operands(name, head):
            _, w32, dst, _ = weights[name]
            transpose = name != "wk"
            slot = (head // 2) % 2
            shift = jnp.asarray(16 * (1 - head % 2)).astype(_U32)
            fb = w32.shape[1] // 2
            step = _T if transpose else 16
            for r in range(0, fb, step):
                rows = min(step, fb - r)
                quads = []
                for f in range(2):
                    for n in range(2):
                        w = w32[slot, f * fb + r:f * fb + r + rows, n * _T:(n + 1) * _T]
                        w = w.T if transpose else w
                        quads.append(pltpu.bitcast((w << shift) & _U32(0xFFFF0000), _F32))
                for i, op in enumerate(_rhs_operands(*quads)):
                    if transpose:
                        if rows < _T:
                            op = jnp.concatenate([op, jnp.zeros((_T, _T - rows), _F32)], axis=1)
                        dst[i, r // _T] = op.astype(_BF16)
                    else:
                        dst[i, r:r + rows] = op.astype(_BF16)

        def wo_operands(head):
            for r in range(0, mh, 16):
                top = woT_s[head % 2, r:r + 16, :].astype(_F32)
                bot = woT_s[head % 2, mh + r:mh + r + 16, :].astype(_F32)
                for i, op in enumerate(_lhs_operands(top[:, :_T], top[:, _T:], bot[:, :_T], bot[:, _T:])):
                    wo_s[i, r:r + 16] = op.astype(_BF16)

        def c_operands(u):
            fb = Dc // 2
            for r in range(0, _T, 16):
                ca = c_s[2 * u * _T + r:2 * u * _T + r + 16, :].astype(_F32)
                cb = c_s[(2 * u + 1) * _T + r:(2 * u + 1) * _T + r + 16, :].astype(_F32)
                for i, op in enumerate(_lhs_operands(ca[:, :fb], ca[:, fb:], cb[:, :fb], cb[:, fb:])):
                    for t in range(kt):
                        cops[i, t, u * _T + r:u * _T + r + 16] = op[:, t * _T:(t + 1) * _T].astype(_BF16)

        def x_operands(u):
            cols = slice(2 * u * _T, 2 * (u + 1) * _T)
            for r in range(0, mh, 16):
                xf = [xT_s[f * mh + r:f * mh + r + 16, cols].astype(_F32) for f in range(2)]
                for i, op in enumerate(_lhs_operands(xf[0][:, :_T], xf[1][:, :_T], xf[0][:, _T:], xf[1][:, _T:])):
                    xops[i, u, r:r + 16] = op.astype(_BF16)

        def score_tokens(u0, u1):
            def step(t):
                wr, gw = (ref[...].astype(_F32).reshape(1, M) for ref in (wr_s, gw_s))
                row = lax.broadcasted_iota(jnp.int32, (16, M), 0)
                rg = _dot(jnp.where(row == 0, wr, gw).astype(_BF16), xT_s[:, t * _T:(t + 1) * _T])
                r_s[t:t + 1] = rg[0:1].astype(_BF16).astype(_F32)
                gate_s[t:t + 1] = jax.nn.sigmoid(rg[1:2])
            return [(64, functools.partial(step, t)) for t in range(2 * u0, 2 * u1)]

        lane = lax.broadcasted_iota(jnp.int32, (1, _T), 1)

        def token_tile(i):
            return pl.ds(pl.multiple_of(i // _T * _T, _T), _T)

        def route():
            r = r_s[...]
            r = jnp.where(r == r, r, -jnp.inf)
            tok = (lax.broadcasted_iota(jnp.int32, r.shape, 0) * _T
                   + lax.broadcasted_iota(jnp.int32, r.shape, 1))
            tokf = tok.astype(_F32)
            live = tok >= 0
            for n in range(2):
                best = jnp.max(jnp.where(live, r, -jnp.inf), keepdims=True)
                pick = jnp.min(jnp.where(live & (r == best), tokf, S - 1.0))
                hit = tokf == pick
                i = pick.astype(jnp.int32)
                idx_s[n] = i
                live = live & ~hit
                scale_s[n:n + 1] = jnp.broadcast_to(jax.nn.sigmoid(best), (1, _T))
                x = xT_s[:, token_tile(i)].astype(_F32)
                x = jnp.sum(jnp.where(lane == i % _T, x, 0.0), axis=1, keepdims=True)
                xsel_s[n] = jnp.broadcast_to(x, (M, _T))

        def ffn_chunk(chunk):
            cols = pl.ds(pl.multiple_of(jnp.minimum(chunk, F // _T - 1) * _T, _T), _T)
            wg = wg_s[:, cols].astype(_F32)
            wu = wu_s[:, cols].astype(_F32)
            wd = wdT_s[:, cols].astype(_F32)
            for n in range(2):
                x = xsel_s[n]
                g = jnp.sum(_fold(x * wg), axis=0, keepdims=True)
                up = jnp.sum(_fold(x * wu), axis=0, keepdims=True)
                hidden = jnp.where(chunk < F // _T, g * jax.nn.sigmoid(g) * up, 0.0)
                y_s[n] += wd * hidden

        def scatter():
            for n in range(2):
                i = idx_s[n]
                y = jnp.sum(y_s[n], axis=1, keepdims=True) * scale_s[n:n + 1]
                x = xT_s[:, token_tile(i)].astype(_F32)
                xT_s[:, token_tile(i)] = jnp.where(lane == i % _T, x + y, x).astype(xT_s.dtype)

        def seven(costs, product, finish):
            m = [None] * 7

            def step(j):
                m[j] = product(j) if costs[j] else None
                if j == 6:
                    finish(*m)
            return [(costs[j], functools.partial(step, j)) for j in range(7)]

        def c_operand(i, u0, u1):
            return _cat([_rows(cops, (i, t), u0 * _T, u1 * _T) for t in range(kt)], 1)

        def k_proj(u0, u1):
            def finish(*m):
                ka0, ka1, kb0, kb1 = _combine(*m)
                for i, op in enumerate(_lhs_operands(kb0, kb1, ka0, ka1)):
                    for u in range(u0, u1):
                        k_s[u][i] = op[(u - u0) * _T:(u - u0 + 1) * _T].astype(_BF16)
            return seven([kt * (u1 - u0) * _T] * 7,
                         lambda i: _dot(c_operand(i, u0, u1), _rows(wk_s, (i,), 0, Dc // 2)), finish)

        def q_proj(u0, u1):
            def prod(i):
                w = _cat([_rows(wq_s, (i, t), 0, _T) for t in range(2)], 1)[:, :mh]
                return _dot(w, _cat([_rows(xops, (i, u), 0, mh) for u in range(u0, u1)], 1))

            def finish(*m):
                qa0, qa1, qb0, qb1 = (q * (D ** -0.5 * _LOG2E) for q in _combine(*m))
                for i, op in enumerate(_rhs_operands(qa0, qb0, qa1, qb1)):
                    for u in range(u0, u1):
                        q_s[u][i] = op[:, (u - u0) * _T:(u - u0 + 1) * _T].astype(_BF16)
            return seven([2 * (u1 - u0) * _T] * 7, prod, finish)

        def v_proj(u0, u1):
            def prod(i):
                return _dot(_cat([_rows(wv_s, (i, t), 0, _T) for t in range(kt)], 1), c_operand(i, u0, u1), _NT)

            def finish(*m):
                va0, va1, vb0, vb1 = _combine(*m)
                for i, op in enumerate(_lhs_operands(vb0, va0, vb1, va1)):
                    for u in range(u0, u1):
                        v_s[u][i] = op[:, (u - u0) * _T:(u - u0 + 1) * _T].astype(_BF16)
            return seven([kt * (u1 - u0) * _T] * 7, prod, finish)

        svals = {}

        def mask_last(s):
            causal = (lax.broadcasted_iota(jnp.int32, (_T, _T), 0) <= lax.broadcasted_iota(jnp.int32, (_T, _T), 1))
            n = s.shape[0] - _T
            d = jnp.where(causal, s[n:], -1e9 * _LOG2E)
            return d if n == 0 else jnp.concatenate([s[:n], d], axis=0)

        def scores(u, _):
            n = u * _T
            rows = [n + _T] * 6 + [n]

            def prod(j):
                return _dot(_cat([tile("k", k_s[t], j) for t in range(rows[j] // _T)], 0), tile("q", q_s[u], j))

            def finish(*m):
                s_ba, s_bb, s_aa, s_ab = _combine(*m)
                s_aa = mask_last(s_aa)
                s_bb = mask_last(s_bb)
                m_a = jnp.max(s_aa, axis=0, keepdims=True)
                if n:
                    m_a = jnp.maximum(m_a, jnp.max(s_ba, axis=0, keepdims=True))
                m_b = jnp.maximum(jnp.max(s_bb, axis=0, keepdims=True), jnp.max(s_ab, axis=0, keepdims=True))
                if "s" in opaque:
                    for i, s in enumerate((s_ba, s_bb, s_aa, s_ab)):
                        if s is not None:
                            pltpu.store(s_s[u].at[i, :s.shape[0]], s, mask=jnp.broadcast_to(idx_s[0] >= 0, s.shape))
                    s_ba, s_bb, s_aa, s_ab = (s_s[u].at[i] for i in range(4))
                svals[u] = (s_ba, s_bb, s_aa, s_ab, m_a, m_b)
            return seven(rows, prod, finish)

        early = {}

        def ctx_operands(u, m, f_a, f_b):
            c0a, c0b, c1a, c1b = _combine(*m)
            for i, op in enumerate(_rhs_operands(c0a * f_a, c0b * f_b, c1a * f_a, c1b * f_b)):
                ctx_s[u][i] = op.astype(_BF16)

        def deferred():
            if defer is not None:
                ctx_operands(defer, [raw_s[j] for j in range(7)], scale_s[2:3], scale_s[3:4])

        def prob_task(u, _):
            steps = context(u, None, True)
            return [(1e-3, early[u])]

        def context(u, _, split=False, units=False):
            if u in early and not split:
                return early.pop((u, "steps"))
            n = u * _T
            acc = [None] * 7
            sums = [None] * 4

            def probs(lo, hi):
                s_ba, s_bb, s_aa, s_ab, m_a, m_b = svals[u]
                for r in range(lo, hi, pchunk):
                    p_bb = jnp.exp2(s_bb[r:r + pchunk] - m_b)
                    p_aa = jnp.exp2(s_aa[r:r + pchunk] - m_a)
                    p_ab = jnp.exp2(s_ab[r:r + pchunk] - m_b)
                    if r < n:
                        p_ba = jnp.exp2(s_ba[r:r + pchunk] - m_a)
                        ops = _rhs_operands(p_ba, p_bb, p_aa, p_ab)
                        terms = (p_ba, p_bb, p_aa, p_ab)
                    else:
                        ops = (p_ab, None, p_bb - p_ab, p_aa, p_ab, p_bb, p_aa + p_ab)
                        terms = (None, p_bb, p_aa, p_ab)
                    for i, t in enumerate(terms):
                        if t is not None:
                            sums[i] = _fold(t) if sums[i] is None else sums[i] + _fold(t)
                    for i, op in enumerate(ops):
                        if op is not None:
                            p_s[u][r // _T][i, r % _T:r % _T + pchunk] = op.astype(_BF16)

            def finish():
                l = [sums[2] if sums[0] is None else sums[0] + sums[2], sums[1] + sums[3]]
                f = [gate_s[2 * u + i:2 * u + i + 1] / jnp.sum(l[i], axis=0, keepdims=True) for i in range(2)]
                if u == defer:
                    for j in range(7):
                        raw_s[j] = acc[j]
                    for i in range(2):
                        scale_s[2 + i:3 + i] = f[i]
                else:
                    ctx_operands(u, acc, *f)

            def step(j, t0, t1):
                if j == 0 and not split:
                    probs(t0 * _T, t1 * _T)
                e = min(t1, u) if j == 1 else t1
                if e > t0:
                    m = _dot(_cat([tile("v", v_s[t], j) for t in range(t0, e)], 1),
                             _cat([tile("p", p_s[u][t], j) for t in range(t0, e)], 0))
                    acc[j] = m if acc[j] is None else acc[j] + m
                if j == 6 and t1 == u + 1:
                    finish()
            nchunks = -(-(u + 1) // kchunk)
            edges = [(u + 1) * i // nchunks for i in range(nchunks + 1)]
            if units:
                seq = [(j, t) for t0, t1 in zip(edges, edges[1:]) for j in corder
                       for t in range(t0, t1) if j != 1 or t < u]

                def unit(j, t):
                    if (j, t) == seq[0]:
                        probs(0, n + _T)
                    m = _dot(tile("v", v_s[t], j), tile("p", p_s[u][t], j))
                    acc[j] = m if acc[j] is None else acc[j] + m
                    if (j, t) == seq[-1]:
                        finish()
                return [functools.partial(unit, j, t) for j, t in seq]
            steps = [((t1 - t0) * _T, functools.partial(step, j, t0, t1))
                     for t0, t1 in zip(edges, edges[1:]) for j in range(7)]
            if split:
                early[u] = functools.partial(probs, 0, n + _T)
                early[u, "steps"] = steps
            return steps

        def out_product(j, u0, u1):
            return _dot(_rows(wo_s, (j,), 0, mh), _cat([tile("c", ctx_s[u], j) for u in range(u0, u1)], 1))

        def project(u0, u1):
            def step(j):
                m = out_product(j, u0, u1)
                for u in range(u0, u1):
                    acc_s[u][j] += m[:, (u - u0) * _T:(u - u0 + 1) * _T]
            return [((u1 - u0) * mh, functools.partial(step, j)) for j in range(7)]

        def run(program, extra):
            def task(t):
                if t in extra:
                    return [(1e-3, extra[t])]
                rng = [int(x) for x in t[1:].split("-")]
                f = {"K": k_proj, "Q": q_proj, "V": v_proj, "O": project, "S": scores, "C": context, "P": prob_task, "R": score_tokens}[t[0]]
                return f(rng[0], rng[1] if len(rng) > 1 else rng[0] + 1)
            for phase in program.split(";"):
                for fn in _merge([[st for t in s.split() for st in task(t)] for s in phase.split("|")]):
                    fn()

        def attention(order, carry):
            load = [0] * 4
            queue = []

            def emit(units, fn):
                for n in units:
                    load[load.index(min(load))] += n
                fn()

            def level():
                while queue and min(load) < max(load):
                    emit([1], queue.pop(0))

            def score_rounds(u):
                n = u * _T
                m = {}

                def prod(j):
                    tiles = u if j == 6 else u + 1
                    m[j] = _dot(_cat([tile("k", k_s[t], j) for t in range(tiles)], 0), tile("q", q_s[u], j))
                for j in (1, 3, 5, 6):
                    if j < 6 or u:
                        emit([u if j == 6 else u + 1], functools.partial(prod, j))
                s_aa = mask_last(m[1] + m[3])
                s_ab = m[5] - m[1]
                s_ba = m[3][:n] + m[6] if u else None
                level()
                for j in (0, 2, 4):
                    emit([u + 1], functools.partial(prod, j))
                s_bb = mask_last(m[2] + m[4])
                s_ab = s_ab + (m[0] + m[2])
                m_a = jnp.max(s_aa, axis=0, keepdims=True)
                if u:
                    s_ba = s_ba + (m[0] - m[4])[:n]
                    m_a = jnp.maximum(m_a, jnp.max(s_ba, axis=0, keepdims=True))
                m_b = jnp.maximum(jnp.max(s_bb, axis=0, keepdims=True), jnp.max(s_ab, axis=0, keepdims=True))
                svals[u] = (s_ba, s_bb, s_aa, s_ab, m_a, m_b)

            ready = []
            for group in order:
                for u in group:
                    score_rounds(u)
                    level()
                while len(queue) >= 4 + carry:
                    for _ in range(4):
                        emit([1], queue.pop(0))
                for u in group:
                    queue.extend(context(u, None, units=True))
            for fn in queue:
                fn()

        with scope("first"):
            for name in dma.split() + ["ffn"]:
                for cp in copies[name]:
                    cp.start()
            for u in range(U):
                acc_s[u][...] = jnp.zeros_like(acc_s[u])
            y_s[...] = jnp.zeros_like(y_s)
            cols = []

            def first_w(name):
                weight_operands(name, 0)

            def first_c(u):
                c_operands(u)

            def first_x(g):
                for u in range(g * U // 2, (g + 1) * U // 2):
                    x_operands(u)
            extra = {n: functools.partial(first_w, n) for n in weights}
            extra.update({f"c{u}": functools.partial(first_c, u) for u in range(U)})
            extra.update({f"x{g}": functools.partial(first_x, g) for g in range(2)})
            extra["route"] = route
            extra.update({"!" + n: functools.partial(wait, n) for n in copies})
            run(first, extra)

        def head_step(h, carry):
            wo_copy(h).start()

            @pl.when((h % 2 == 0) & (h + 2 < nh))
            def _():
                for name in weights:
                    w_copy(name, h // 2 + 1).start()

            with scope("attn"):
                run(b, {}) if isinstance(b, str) else attention(*b)
            wo_copy(h).wait()

            @pl.when(h == 0)
            def _():
                wait("ffn")

            @pl.when(h + 1 < nh)
            def _():
                @pl.when(h % 2 == 1)
                def _():
                    for name in weights:
                        w_copy(name, h // 2 + 1).wait()
                with scope("proj"):
                    wo_operands(h)
                    deferred()
                    extra = {n: functools.partial(weight_operands, n, h + 1) for n in weights}
                    extra["ffn"] = functools.partial(ffn_chunk, h)
                    run(a, extra)
            return carry

        lax.fori_loop(0, nh, head_step, None)

        with scope("last"):
            wo_operands(nh - 1)
            deferred()
            scatter()
            for u in range(U):
                o = _combine(*(acc_s[u][j] + out_product(j, u, u + 1) for j in range(7)))
                cols_u = slice(2 * u * _T, 2 * (u + 1) * _T)
                for half in range(2):
                    rows = slice(half * mh, (half + 1) * mh)
                    keep = 1.0 - jnp.concatenate([gate_s[2 * u:2 * u + 1], gate_s[2 * u + 1:2 * u + 2]], axis=1)
                    new = keep * xT_s[rows, cols_u].astype(_F32) + jnp.concatenate(o[2 * half:2 * half + 2], axis=1)
                    out_s[rows, cols_u] = new.astype(out_s.dtype)
                copies[f"o{u}"][0].start()
            for u in range(U):
                wait(f"o{u}")

    def fn(A_x, A_c_kv, A_w_q, A_w_uk, A_w_uv, A_w_o, B_x, B_w_r, B_w_gate, B_w_up, B_w_down, gate_w):
        del B_x
        _, S, M = A_x.shape
        Dc, H, D = A_w_uk.shape
        F = B_w_gate.shape[1]
        U = S // (2 * _T)
        tile = pltpu.VMEM((7, _T, _T), _BF16)
        hbm = pl.BlockSpec(memory_space=pl.ANY)
        outT = pl.pallas_call(
            kernel,
            in_specs=[hbm] * 11,
            out_specs=hbm,
            out_shape=jax.ShapeDtypeStruct((M, S), A_x.dtype),
            scratch_shapes=[
                pltpu.VMEM((2, M, D), _U32), pltpu.VMEM((2, Dc, D), _U32), pltpu.VMEM((2, Dc, D), _U32),
                pltpu.VMEM((2, M, D), _BF16),
                pltpu.SemaphoreType.DMA((4, 2)),
                pltpu.VMEM((M, S), _BF16), pltpu.VMEM((S, Dc), _BF16),
                pltpu.VMEM((M, F), _BF16), pltpu.VMEM((M, F), _BF16), pltpu.VMEM((M, F), _BF16),
                pltpu.VMEM((M,), _BF16), pltpu.VMEM((M,), _BF16), pltpu.VMEM((M, S), _BF16),
                pltpu.SemaphoreType.DMA((U + 7,)),
                pltpu.VMEM((7, U, M // 2, _T), _BF16), pltpu.VMEM((7, Dc // 2 // _T, S // 2, _T), _BF16),
                pltpu.VMEM((7, 2, _T, _T), _BF16), pltpu.VMEM((7, Dc // 2, _T), _BF16),
                pltpu.VMEM((7, Dc // 2 // _T, _T, _T), _BF16), pltpu.VMEM((7, M // 2, _T), _BF16),
                [tile] * U, [tile] * U, [tile] * U,
                [pltpu.VMEM((4, (u + 1) * _T, _T), _F32) for u in range(U)],
                [[tile] * (u + 1) for u in range(U)],
                [tile] * U,
                [pltpu.VMEM((7, M // 2, _T), _F32)] * U,
                pltpu.VMEM((2 * U, _T), _F32), pltpu.VMEM((2 * U, _T), _F32),
                pltpu.VMEM((2, M, _T), _F32), pltpu.VMEM((2, M, _T), _F32), pltpu.VMEM((8, _T), _F32),
                pltpu.VMEM((7, _T, _T), _F32),
                pltpu.SMEM((2,), jnp.int32),
            ],
            compiler_params=pltpu.CompilerParams(vmem_limit_bytes=110 * 2**20, flags=flags),
            name="gm_kernel",
        )(A_x[0].T, A_c_kv[0], A_w_q, A_w_uk, A_w_uv, A_w_o.transpose(0, 2, 1), B_w_r, B_w_gate, B_w_up, B_w_down.T, gate_w)
        return outT.T[None]
    return fn


@jax.jit
def pallas_gated_mix__compressed_kv_cla__moe_arch_mod__prompt_kernel(
    A_x, A_c_kv, A_w_q, A_w_uk, A_w_uv, A_w_o, B_x, B_w_r, B_w_gate, B_w_up, B_w_down, gate_w
):
    return make()(A_x, A_c_kv, A_w_q, A_w_uk, A_w_uv, A_w_o, B_x, B_w_r, B_w_gate, B_w_up, B_w_down, gate_w)
```

```python
import contextlib
import functools
import math

import jax
import jax.numpy as jnp
from jax import lax
import jax.experimental.pallas as pl
import jax.experimental.pallas.tpu as pltpu

_NN = (((1,), (0,)), ((), ()))
_NT = (((1,), (1,)), ((), ()))
_LOG2E = math.log2(math.e)
_F32 = jnp.float32
_BF16 = jnp.bfloat16
_U32 = jnp.uint32
_T = 128


def _dot(a, b, dims=_NN):
    return lax.dot_general(a, b, dims, preferred_element_type=_F32)


def _lhs_operands(a11, a12, a21, a22):
    return (a11 + a22, a21 + a22, a11, a22, a11 + a12, a21 - a11, a12 - a22)


def _rhs_operands(b11, b12, b21, b22):
    return (b11 + b22, b11, b12 - b22, b21 - b11, b22, b11 + b12, b21 + b22)


def _combine(m1, m2, m3, m4, m5, m6, m7):
    c21 = m4 if m2 is None else m2 + m4
    c12 = m3 + m5
    c22 = (m1 + m3 if m2 is None else m1 - m2 + m3) + m6
    c11 = None if m7 is None else (m1 + m4 - m5)[:m7.shape[0]] + m7
    return c11, c12, c21, c22


def _rows(ref, lead, lo, hi):
    return pltpu.bitcast(ref.bitcast(_U32)[(*lead, slice(lo // 2, hi // 2))], _BF16)


def _cat(xs, axis):
    xs = list(xs)
    return xs[0] if len(xs) == 1 else jnp.concatenate(xs, axis=axis)


def _fold(x):
    return functools.reduce(jnp.add, [x[r:r + 8] for r in range(0, x.shape[0], 8)])


def _merge(streams):
    keyed = []
    for s, steps in enumerate(streams):
        total = sum(c for c, _ in steps)
        done = 0
        for c, fn in steps:
            keyed.append(((done + c / 2) / total, s, len(keyed), fn))
            done += c
    return [fn for *_, fn in sorted(keyed, key=lambda t: t[:3])]


def make(flags=None, pchunk=16, kchunk=8, opaque="", nh=16, scopes=False,
         dma="wv c0 wk c1 c2 c3 c4 c5 c6 c7 vec wq x0 x1",
         first="!wv wv !c0 c0 V0 !wk wk K0 !c1 c1 K1 V1 !c2 !c3 c2 c3 K2-4 V2-4 !c4 !c5 !c6 c4 c5 c6 V4-6 V6 K4-6 !c7 !vec !wq !x0 !x1 c7 wq x0 x1; K6 | R0-8; K7 | Q0 Q1 Q2 Q3; route; V7 | Q4 Q5 Q6 Q7",
         a="wk wq wv O0 O1 O2; K0-2 K2-8 V0-2 V2-4 V4-6 V6-8 | O3 up Q0-2 down Q2-4 O4 Q4-6 Q6-8 O5; O6 O7",
         b=([[1, 0, 2], [3], [4], [5], [6], [7]], [1, 3, 5, 3, 3, 1, 3, 3], [0, 8, 12, 0, 0, 0, 2, 6]), defer=None, nocheck=True, only=None, corder=[[4, 1, 0, 6, 3, 5, 2], [4, 1, 0, 6, 2, 5, 3], [4, 1, 0, 6, 3, 5, 2], [1, 4, 0, 3, 6, 5, 2], [1, 4, 0, 5, 3, 6, 2], [4, 1, 0, 3, 5, 6, 2], [4, 1, 0, 6, 3, 5, 2], [4, 1, 0, 2, 3, 6, 5]]):
    scope = jax.named_scope if scopes else (lambda name: contextlib.nullcontext())

    def kernel(xT_hbm, c_hbm, wq_hbm, wuk_hbm, wuv_hbm, woT_hbm, wr_hbm, wg_hbm, wu_hbm, wdT_hbm, gw_hbm,
               outT_hbm,
               w0_s, wq32, wuk32, wuv32, woT_s, wsems, xT_s, c_s, wg_s, wu_s, wdT_s, wr_s, gw_s, out_s, sems,
               xops, cops, wq_s, wk_s, wv_s, wo_s, q_s, k_s, v_s, s_s, p_s, ctx_s, acc_s,
               gate_s, r_s, xsel_s, y_s, scale_s, raw_s, idx_s):
        M, S = xT_s.shape
        Dc = c_s.shape[1]
        D = woT_s.shape[1]
        F = wg_hbm.shape[1]
        U = S // (2 * _T)
        mh = M // 2
        kt = Dc // 2 // _T
        weights = {"wq": (wq_hbm, wq32, wq_s, 0), "wk": (wuk_hbm, wuk32, wk_s, 1), "wv": (wuv_hbm, wuv32, wv_s, 2)}

        def w_copy(name, pair):
            src, dst, _, i = weights[name]
            return [pltpu.make_async_copy(src.bitcast(_U32).at[:, pair, n * _T:(n + 1) * _T], dst.at[n], wsems.at[7 + 2 * i + n])
                    for n in range(2)]

        def wo_copy(head):
            return pltpu.make_async_copy(woT_hbm.at[head], woT_s, wsems.at[3])

        def ffn_copies(chunk):
            cols = pl.ds(pl.multiple_of(chunk * _T, _T), _T)
            return [pltpu.make_async_copy(src.at[:, cols], dst, wsems.at[4 + i])
                    for i, (src, dst) in enumerate(((wg_hbm, wg_s), (wu_hbm, wu_s), (wdT_hbm, wdT_s)))]

        copies = {n: [pltpu.make_async_copy(src.bitcast(_U32).at[:, 0, :], w0_s[i], wsems.at[i])]
                  for n, (src, _, _, i) in weights.items()}
        for u in range(U):
            rows = slice(2 * u * _T, 2 * (u + 1) * _T)
            copies[f"c{u}"] = [pltpu.make_async_copy(c_hbm.at[rows], c_s.at[rows], sems.at[u])]
            copies[f"o{u}"] = [pltpu.make_async_copy(out_s.at[:, rows], outT_hbm.at[:, rows], sems.at[u])]
        for g in range(2):
            cols = slice(g * S // 2, (g + 1) * S // 2)
            copies[f"x{g}"] = [pltpu.make_async_copy(xT_hbm.at[:, cols], xT_s.at[:, cols], sems.at[U + g])]
        copies["vec"] = [pltpu.make_async_copy(wr_hbm, wr_s, sems.at[U + 2]),
                         pltpu.make_async_copy(gw_hbm, gw_s, sems.at[U + 3])]

        def wait(name):
            with scope("w_" + name):
                for cp in copies[name]:
                    cp.wait()

        def tile(name, ref, j):
            return ref[j] if name in opaque else _rows(ref, (j,), 0, _T)

        def weight_operands(name, head, first=False):
            _, w32, dst, i0 = weights[name]
            transpose = name != "wk"
            shift = jnp.asarray(16 * (1 - head % 2)).astype(_U32)
            fb = w32.shape[1] // 2
            step = _T if transpose else 16
            for r in range(0, fb, step):
                rows = min(step, fb - r)
                quads = []
                for f in range(2):
                    for n in range(2):
                        src = slice(f * fb + r, f * fb + r + rows)
                        w = w0_s[i0][src, n * _T:(n + 1) * _T] if first else w32[n, src]
                        w = w.T if transpose else w
                        quads.append(pltpu.bitcast((w << shift) & _U32(0xFFFF0000), _F32))
                for i, op in enumerate(_rhs_operands(*quads)):
                    if transpose:
                        if rows < _T:
                            op = jnp.concatenate([op, jnp.zeros((_T, _T - rows), _F32)], axis=1)
                        dst[i, r // _T] = op.astype(_BF16)
                    else:
                        dst[i, r:r + rows] = op.astype(_BF16)

        def wo_operands(head):
            for r in range(0, mh, 16):
                top = woT_s[r:r + 16, :].astype(_F32)
                bot = woT_s[mh + r:mh + r + 16, :].astype(_F32)
                for i, op in enumerate(_lhs_operands(top[:, :_T], top[:, _T:], bot[:, :_T], bot[:, _T:])):
                    wo_s[i, r:r + 16] = op.astype(_BF16)

        def c_operands(u):
            fb = Dc // 2
            for r in range(0, _T, 16):
                ca = c_s[2 * u * _T + r:2 * u * _T + r + 16, :].astype(_F32)
                cb = c_s[(2 * u + 1) * _T + r:(2 * u + 1) * _T + r + 16, :].astype(_F32)
                for i, op in enumerate(_lhs_operands(ca[:, :fb], ca[:, fb:], cb[:, :fb], cb[:, fb:])):
                    for t in range(kt):
                        cops[i, t, u * _T + r:u * _T + r + 16] = op[:, t * _T:(t + 1) * _T].astype(_BF16)

        def x_operands(u):
            cols = slice(2 * u * _T, 2 * (u + 1) * _T)
            for r in range(0, mh, 16):
                xf = [xT_s[f * mh + r:f * mh + r + 16, cols].astype(_F32) for f in range(2)]
                for i, op in enumerate(_lhs_operands(xf[0][:, :_T], xf[1][:, :_T], xf[0][:, _T:], xf[1][:, _T:])):
                    xops[i, u, r:r + 16] = op.astype(_BF16)

        def score_tokens(u0, u1):
            def step(t):
                wr, gw = (ref[...].astype(_F32).reshape(1, M) for ref in (wr_s, gw_s))
                row = lax.broadcasted_iota(jnp.int32, (16, M), 0)
                rg = _dot(jnp.where(row == 0, wr, gw).astype(_BF16), xT_s[:, t * _T:(t + 1) * _T])
                r_s[t:t + 1] = rg[0:1].astype(_BF16).astype(_F32)
                gate_s[t:t + 1] = jax.nn.sigmoid(rg[1:2])
            return [(64, functools.partial(step, t)) for t in range(2 * u0, 2 * u1)]

        lane = lax.broadcasted_iota(jnp.int32, (1, _T), 1)

        def token_tile(i):
            return pl.ds(pl.multiple_of(i // _T * _T, _T), _T)

        def route():
            r = r_s[...]
            r = jnp.where(r == r, r, -jnp.inf)
            tok = (lax.broadcasted_iota(jnp.int32, r.shape, 0) * _T
                   + lax.broadcasted_iota(jnp.int32, r.shape, 1))
            tokf = tok.astype(_F32)
            live = tok >= 0
            slot = lax.broadcasted_iota(jnp.int32, (16, _T), 0)
            picked = None
            for n in range(2):
                best = jnp.max(jnp.where(live, r, -jnp.inf), keepdims=True)
                pick = jnp.min(jnp.where(live & (r == best), tokf, S - 1.0))
                hit = tokf == pick
                i = pick.astype(jnp.int32)
                idx_s[n] = i
                live = live & ~hit
                scale_s[n:n + 1] = jnp.broadcast_to(jax.nn.sigmoid(best), (1, _T))
                onehot = jnp.where((slot == n) & (lane == i % _T), 1.0, 0.0).astype(_BF16)
                x = _dot(onehot, xT_s[:, token_tile(i)], _NT)
                picked = x if picked is None else picked + x
            xsel_s[...] = picked.astype(_BF16)

        ffn = {}

        def ffn_up(chunk):
            x = xsel_s[...]
            g = _dot(x, _rows(wg_s, (), 0, M))
            up = _dot(x, _rows(wu_s, (), 0, M))
            ffn["hidden"] = jnp.where(chunk < F // _T, g * jax.nn.sigmoid(g) * up, 0.0)

        def ffn_down():
            y_s[...] += _dot(ffn["hidden"].astype(_BF16), _rows(wdT_s, (), 0, M), _NT)

        def scatter():
            yT = jnp.concatenate([y_s[...], jnp.zeros((_T - 16, M), _F32)], axis=0).T
            for n in range(2):
                i = idx_s[n]
                y = yT[:, n:n + 1] * scale_s[n:n + 1]
                x = xT_s[:, token_tile(i)].astype(_F32)
                xT_s[:, token_tile(i)] = jnp.where(lane == i % _T, x + y, x).astype(xT_s.dtype)

        def seven(costs, product, finish):
            m = [None] * 7

            def step(j):
                m[j] = product(j) if costs[j] else None
                if j == 6:
                    finish(*m)
            return [(costs[j], functools.partial(step, j)) for j in range(7)]

        def c_operand(i, u0, u1):
            return _cat([_rows(cops, (i, t), u0 * _T, u1 * _T) for t in range(kt)], 1)

        def k_proj(u0, u1):
            def finish(*m):
                ka0, ka1, kb0, kb1 = _combine(*m)
                for i, op in enumerate(_lhs_operands(kb0, kb1, ka0, ka1)):
                    for u in range(u0, u1):
                        k_s[u][i] = op[(u - u0) * _T:(u - u0 + 1) * _T].astype(_BF16)
            return seven([kt * (u1 - u0) * _T] * 7,
                         lambda i: _dot(c_operand(i, u0, u1), _rows(wk_s, (i,), 0, Dc // 2)), finish)

        def q_proj(u0, u1):
            def prod(i):
                w = _cat([_rows(wq_s, (i, t), 0, _T) for t in range(2)], 1)[:, :mh]
                return _dot(w, _cat([_rows(xops, (i, u), 0, mh) for u in range(u0, u1)], 1))

            def finish(*m):
                qa0, qa1, qb0, qb1 = (q * (D ** -0.5 * _LOG2E) for q in _combine(*m))
                for i, op in enumerate(_rhs_operands(qa0, qb0, qa1, qb1)):
                    for u in range(u0, u1):
                        q_s[u][i] = op[:, (u - u0) * _T:(u - u0 + 1) * _T].astype(_BF16)
            return seven([2 * (u1 - u0) * _T] * 7, prod, finish)

        def v_proj(u0, u1):
            def prod(i):
                return _dot(_cat([_rows(wv_s, (i, t), 0, _T) for t in range(kt)], 1), c_operand(i, u0, u1), _NT)

            def finish(*m):
                va0, va1, vb0, vb1 = _combine(*m)
                for i, op in enumerate(_lhs_operands(vb0, va0, vb1, va1)):
                    for u in range(u0, u1):
                        v_s[u][i] = op[:, (u - u0) * _T:(u - u0 + 1) * _T].astype(_BF16)
            return seven([kt * (u1 - u0) * _T] * 7, prod, finish)

        svals = {}

        def mask_last(s):
            causal = (lax.broadcasted_iota(jnp.int32, (_T, _T), 0) <= lax.broadcasted_iota(jnp.int32, (_T, _T), 1))
            n = s.shape[0] - _T
            d = jnp.where(causal, s[n:], -1e9 * _LOG2E)
            return d if n == 0 else jnp.concatenate([s[:n], d], axis=0)

        def scores(u, _):
            n = u * _T
            rows = [n + _T] * 6 + [n]

            def prod(j):
                return _dot(_cat([tile("k", k_s[t], j) for t in range(rows[j] // _T)], 0), tile("q", q_s[u], j))

            def finish(*m):
                s_ba, s_bb, s_aa, s_ab = _combine(*m)
                s_aa = mask_last(s_aa)
                s_bb = mask_last(s_bb)
                m_a = jnp.max(s_aa, axis=0, keepdims=True)
                if n:
                    m_a = jnp.maximum(m_a, jnp.max(s_ba, axis=0, keepdims=True))
                m_b = jnp.maximum(jnp.max(s_bb, axis=0, keepdims=True), jnp.max(s_ab, axis=0, keepdims=True))
                if "s" in opaque:
                    for i, s in enumerate((s_ba, s_bb, s_aa, s_ab)):
                        if s is not None:
                            pltpu.store(s_s[u].at[i, :s.shape[0]], s, mask=jnp.broadcast_to(idx_s[0] >= 0, s.shape))
                    s_ba, s_bb, s_aa, s_ab = (s_s[u].at[i] for i in range(4))
                svals[u] = (s_ba, s_bb, s_aa, s_ab, m_a, m_b)
            return seven(rows, prod, finish)

        early = {}

        def ctx_operands(u, m, f_a, f_b):
            c0a, c0b, c1a, c1b = _combine(*m)
            for i, op in enumerate(_rhs_operands(c0a * f_a, c0b * f_b, c1a * f_a, c1b * f_b)):
                ctx_s[u][i] = op.astype(_BF16)

        def deferred():
            if defer is not None:
                ctx_operands(defer, [raw_s[j] for j in range(7)], scale_s[2:3], scale_s[3:4])

        def prob_task(u, _):
            steps = context(u, None, True)
            return [(1e-3, early[u])]

        def context(u, _, split=False, units=False):
            if u in early and not split:
                return early.pop((u, "steps"))
            n = u * _T
            acc = [None] * 7
            sums = [None] * 4

            def probs(lo, hi):
                s_ba, s_bb, s_aa, s_ab, m_a, m_b = svals[u]
                for r in range(lo, hi, pchunk):
                    p_bb = jnp.exp2(s_bb[r:r + pchunk] - m_b)
                    p_aa = jnp.exp2(s_aa[r:r + pchunk] - m_a)
                    p_ab = jnp.exp2(s_ab[r:r + pchunk] - m_b)
                    if r < n:
                        p_ba = jnp.exp2(s_ba[r:r + pchunk] - m_a)
                        ops = _rhs_operands(p_ba, p_bb, p_aa, p_ab)
                        terms = (p_ba, p_bb, p_aa, p_ab)
                    else:
                        ops = (p_ab, None, p_bb - p_ab, p_aa, p_ab, p_bb, p_aa + p_ab)
                        terms = (None, p_bb, p_aa, p_ab)
                    for i, t in enumerate(terms):
                        if t is not None:
                            sums[i] = _fold(t) if sums[i] is None else sums[i] + _fold(t)
                    for i, op in enumerate(ops):
                        if op is not None:
                            p_s[u][r // _T][i, r % _T:r % _T + pchunk] = op.astype(_BF16)

            def finish():
                l = [sums[2] if sums[0] is None else sums[0] + sums[2], sums[1] + sums[3]]
                f = [gate_s[2 * u + i:2 * u + i + 1] / jnp.sum(l[i], axis=0, keepdims=True) for i in range(2)]
                if u == defer:
                    for j in range(7):
                        raw_s[j] = acc[j]
                    for i in range(2):
                        scale_s[2 + i:3 + i] = f[i]
                else:
                    ctx_operands(u, acc, *f)

            def step(j, t0, t1):
                if j == 0 and not split:
                    probs(t0 * _T, t1 * _T)
                e = min(t1, u) if j == 1 else t1
                if e > t0:
                    m = _dot(_cat([tile("v", v_s[t], j) for t in range(t0, e)], 1),
                             _cat([tile("p", p_s[u][t], j) for t in range(t0, e)], 0))
                    acc[j] = m if acc[j] is None else acc[j] + m
                if j == 6 and t1 == u + 1:
                    finish()
            nchunks = -(-(u + 1) // kchunk)
            edges = [(u + 1) * i // nchunks for i in range(nchunks + 1)]
            if units:
                seq = [(j, t) for t0, t1 in zip(edges, edges[1:]) for j in corder[u]
                       for t in range(t0, t1) if j != 1 or t < u]

                def unit(j, t):
                    if (j, t) == seq[0]:
                        probs(0, n + _T)
                    m = _dot(tile("v", v_s[t], j), tile("p", p_s[u][t], j))
                    acc[j] = m if acc[j] is None else acc[j] + m
                    if (j, t) == seq[-1]:
                        finish()
                return [functools.partial(unit, j, t) for j, t in seq]
            steps = [((t1 - t0) * _T, functools.partial(step, j, t0, t1))
                     for t0, t1 in zip(edges, edges[1:]) for j in range(7)]
            if split:
                early[u] = functools.partial(probs, 0, n + _T)
                early[u, "steps"] = steps
            return steps

        def out_product(j, u0, u1):
            return _dot(_rows(wo_s, (j,), 0, mh), _cat([tile("c", ctx_s[u], j) for u in range(u0, u1)], 1))

        def project(u0, u1):
            def step(j):
                m = out_product(j, u0, u1)
                for u in range(u0, u1):
                    acc_s[u][j] += m[:, (u - u0) * _T:(u - u0 + 1) * _T]
            return [((u1 - u0) * mh, functools.partial(step, j)) for j in range(7)]

        def run(program, extra):
            def task(t):
                if t in extra:
                    return [(1e-3, extra[t])]
                rng = [int(x) for x in t[1:].split("-")]
                f = {"K": k_proj, "Q": q_proj, "V": v_proj, "O": project, "S": scores, "C": context, "P": prob_task, "R": score_tokens}[t[0]]
                return f(rng[0], rng[1] if len(rng) > 1 else rng[0] + 1)
            for phase in program.split(";"):
                for fn in _merge([[st for t in s.split() for st in task(t)] for s in phase.split("|")]):
                    fn()

        def attention(order, carry, overlap):
            load = [0] * 4
            queue = []

            def emit(units, fn):
                for n in units:
                    load[load.index(min(load))] += n
                fn()

            def level():
                while queue and min(load) < max(load):
                    emit([1], queue.pop(0))

            def score_rounds(u):
                n = u * _T
                m = {}

                def prod(j):
                    tiles = u if j == 6 else u + 1
                    m[j] = _dot(_cat([tile("k", k_s[t], j) for t in range(tiles)], 0), tile("q", q_s[u], j))
                for j in (1, 3, 5, 6):
                    if j < 6 or u:
                        emit([u if j == 6 else u + 1], functools.partial(prod, j))
                s_aa = mask_last(m[1] + m[3])
                s_ab = m[5] - m[1]
                s_ba = m[3][:n] + m[6] if u else None
                level()
                for j in (0, 2, 4):
                    emit([u + 1], functools.partial(prod, j))
                s_bb = mask_last(m[2] + m[4])
                s_ab = s_ab + (m[0] + m[2])
                m_a = jnp.max(s_aa, axis=0, keepdims=True)
                if u:
                    s_ba = s_ba + (m[0] - m[4])[:n]
                    m_a = jnp.maximum(m_a, jnp.max(s_ba, axis=0, keepdims=True))
                m_b = jnp.maximum(jnp.max(s_bb, axis=0, keepdims=True), jnp.max(s_ab, axis=0, keepdims=True))
                svals[u] = (s_ba, s_bb, s_aa, s_ab, m_a, m_b)

            ready = []
            for g, group in enumerate(order):
                for u in group:
                    score_rounds(u)
                    level()
                while len(queue) >= 4 + carry[g]:
                    for _ in range(4):
                        emit([1], queue.pop(0))
                for u in group:
                    new = context(u, None, units=True)
                    n = min(overlap[u], len(queue), len(new))
                    tail = [queue.pop() for _ in range(n)][::-1]
                    queue.extend([fn for pair in zip(tail, new) for fn in pair] + new[n:])
            for fn in queue:
                fn()

        with scope("first"):
            for name in dma.split():
                for cp in copies[name]:
                    cp.start()
            for u in range(U):
                acc_s[u][...] = jnp.zeros_like(acc_s[u])
            y_s[...] = jnp.zeros_like(y_s)
            cols = []

            def first_w(name):
                weight_operands(name, 0, True)

            def first_c(u):
                c_operands(u)

            def first_x(g):
                for u in range(g * U // 2, (g + 1) * U // 2):
                    x_operands(u)
            extra = {n: functools.partial(first_w, n) for n in weights}
            extra.update({f"c{u}": functools.partial(first_c, u) for u in range(U)})
            extra.update({f"x{g}": functools.partial(first_x, g) for g in range(2)})
            extra["route"] = route
            extra.update({"!" + n: functools.partial(wait, n) for n in copies})
            if only is None:
                run(first, extra)
            else:
                for name in dma.split():
                    wait(name)

        def fetch(h):
            return ([wo_copy(h)] + [cp for name in weights for cp in w_copy(name, jnp.minimum(h + 1, nh - 1) // 2)]
                    + ffn_copies(jnp.minimum(h, F // _T - 1)))

        for cp in fetch(0):
            cp.start()

        def head_step(h, carry):
            with scope("attn"):
                if only != 'a':
                    attention(*b)
            for cp in fetch(h):
                cp.wait()

            @pl.when(h + 1 < nh)
            def _():
                with scope("proj"):
                    wo_operands(h)
                    deferred()
                    extra = {n: functools.partial(weight_operands, n, h + 1) for n in weights}
                    extra["up"] = functools.partial(ffn_up, h)
                    extra["down"] = ffn_down
                    if only != 'b':
                        run(a, extra)
                    for cp in fetch(h + 1):
                        cp.start()
            return carry

        lax.fori_loop(0, nh, head_step, None)

        with scope("last"):
            wo_operands(nh - 1)
            deferred()
            scatter()
            for u in range(U):
                o = _combine(*(acc_s[u][j] + out_product(j, u, u + 1) for j in range(7)))
                cols_u = slice(2 * u * _T, 2 * (u + 1) * _T)
                for half in range(2):
                    rows = slice(half * mh, (half + 1) * mh)
                    keep = 1.0 - jnp.concatenate([gate_s[2 * u:2 * u + 1], gate_s[2 * u + 1:2 * u + 2]], axis=1)
                    new = keep * xT_s[rows, cols_u].astype(_F32) + jnp.concatenate(o[2 * half:2 * half + 2], axis=1)
                    out_s[rows, cols_u] = new.astype(out_s.dtype)
                copies[f"o{u}"][0].start()
            for u in range(U):
                wait(f"o{u}")

    def fn(A_x, A_c_kv, A_w_q, A_w_uk, A_w_uv, A_w_o, B_x, B_w_r, B_w_gate, B_w_up, B_w_down, gate_w):
        del B_x
        _, S, M = A_x.shape
        Dc, H, D = A_w_uk.shape
        F = B_w_gate.shape[1]
        U = S // (2 * _T)
        tile = pltpu.VMEM((7, _T, _T), _BF16)
        hbm = pl.BlockSpec(memory_space=pl.ANY)
        outT = pl.pallas_call(
            kernel,
            in_specs=[hbm] * 11,
            out_specs=hbm,
            out_shape=jax.ShapeDtypeStruct((M, S), A_x.dtype),
            scratch_shapes=[
                [pltpu.VMEM((n, D), _U32) for n in (M, Dc, Dc)],
                pltpu.VMEM((2, M, _T), _U32), pltpu.VMEM((2, Dc, _T), _U32), pltpu.VMEM((2, Dc, _T), _U32),
                pltpu.VMEM((M, D), _BF16),
                pltpu.SemaphoreType.DMA((13,)),
                pltpu.VMEM((M, S), _BF16), pltpu.VMEM((S, Dc), _BF16),
                pltpu.VMEM((M, _T), _BF16), pltpu.VMEM((M, _T), _BF16), pltpu.VMEM((M, _T), _BF16),
                pltpu.VMEM((M,), _BF16), pltpu.VMEM((M,), _BF16), pltpu.VMEM((M, S), _BF16),
                pltpu.SemaphoreType.DMA((U + 4,)),
                pltpu.VMEM((7, U, M // 2, _T), _BF16), pltpu.VMEM((7, Dc // 2 // _T, S // 2, _T), _BF16),
                pltpu.VMEM((7, 2, _T, _T), _BF16), pltpu.VMEM((7, Dc // 2, _T), _BF16),
                pltpu.VMEM((7, Dc // 2 // _T, _T, _T), _BF16), pltpu.VMEM((7, M // 2, _T), _BF16),
                [tile] * U, [tile] * U, [tile] * U,
                [pltpu.VMEM((4, (u + 1) * _T, _T), _F32) for u in range(U)],
                [[tile] * (u + 1) for u in range(U)],
                [tile] * U,
                [pltpu.VMEM((7, M // 2, _T), _F32)] * U,
                pltpu.VMEM((2 * U, _T), _F32), pltpu.VMEM((2 * U, _T), _F32),
                pltpu.VMEM((16, M), _BF16), pltpu.VMEM((16, M), _F32), pltpu.VMEM((8, _T), _F32),
                pltpu.VMEM((7, _T, _T), _F32),
                pltpu.SMEM((2,), jnp.int32),
            ],
            compiler_params=pltpu.CompilerParams(vmem_limit_bytes=110 * 2**20, flags=flags, disable_bounds_checks=nocheck),
            name="gm_kernel",
        )(A_x[0].T, A_c_kv[0], A_w_q, A_w_uk, A_w_uv, A_w_o.transpose(0, 2, 1), B_w_r, B_w_gate, B_w_up, B_w_down.T, gate_w)
        return outT.T[None]
    return fn


@jax.jit
def pallas_gated_mix__compressed_kv_cla__moe_arch_mod__prompt_kernel(
    A_x, A_c_kv, A_w_q, A_w_uk, A_w_uv, A_w_o, B_x, B_w_r, B_w_gate, B_w_up, B_w_down, gate_w
):
    return make()(A_x, A_c_kv, A_w_q, A_w_uk, A_w_uv, A_w_o, B_x, B_w_r, B_w_gate, B_w_up, B_w_down, gate_w)
```

```python
import functools
import math

import jax
import jax.numpy as jnp
from jax import lax
import jax.experimental.pallas as pl
import jax.experimental.pallas.tpu as pltpu

_NN = (((1,), (0,)), ((), ()))
_NT = (((1,), (1,)), ((), ()))
_F32 = jnp.float32
_BF16 = jnp.bfloat16
_U32 = jnp.uint32
_LOG2E = math.log2(math.e)
_T = 128
_ROWS = 16
_CAPACITY = 2

_TUNING = dict(
    first_copies="wv c0 wk c1 c2 c3 c4 c5 c6 c7 vec wq x",
    first="!wv wv !c0 c0 V0 !wk wk K0 !c1 c1 K1 V1 !c2 !c3 c2 c3 K2-4 V2-4"
          " !c4 !c5 !c6 c4 c5 c6 V4-6 V6 K4-6 !c7 !vec !wq !x c7 wq x;"
          " K6 | R0-8; K7 | Q0 Q1 Q2 Q3; route; V7 | Q4 Q5 Q6 Q7",
    projections="wo wk wq wv O0 O1 O2;"
                " K0-2 K2-8 V0-2 V2-4 V4-6 V6-8 | O3 up Q0-2 down Q2-4 O4 Q4-6 Q6-8 O5; O6 O7",
    score_order=[[0, 1, 2], [3], [4], [5], [6], [7]],
    held_back=[7, 5, 3, 5, 5, 7, 3, 3],
    overlap=[8, 0, 0, 0, 0, 0, 0, 0],
    pv_order=[[4, 1, 0, 6, 3, 5, 2, 7], [1, 4, 0, 5, 7, 6, 2, 3], [1, 4, 0, 3, 6, 2, 5, 7], [1, 4, 0, 2, 7, 6, 5, 3], [4, 1, 0, 6, 3, 5, 2, 7], [1, 4, 0, 7, 2, 3, 6, 5], [1, 4, 0, 5, 3, 6, 2, 7], [1, 4, 0, 3, 6, 2, 5, 7]],
    diag_order=[[0, 1, 2, 3, 4, 5], [2, 1, 5, 3, 4, 0], [3, 0, 4, 1, 5, 2], [4, 2, 1, 0, 3, 5], [4, 2, 1, 5, 0, 3], [4, 0, 2, 3, 1, 5], [0, 2, 4, 1, 5, 3], [1, 4, 3, 5, 0, 2]],
    sum_rows=[4096, 4096, 4096, 128, 4096, 32, 16, 32],
)


def _dot(a, b, dims=_NN):
    return lax.dot_general(a, b, dims, preferred_element_type=_F32)


def _lhs_operands(a11, a12, a21, a22):
    return (a11 + a22, a21 + a22, a11, a22, a11 + a12, a21 - a11, a12 - a22)


def _rhs_operands(b11, b12, b21, b22):
    return (b11 + b22, b11, b12 - b22, b21 - b11, b22, b11 + b12, b21 + b22)


def _combine(m1, m2, m3, m4, m5, m6, m7):
    return m1 + m4 - m5 + m7, m3 + m5, m2 + m4, m1 - m2 + m3 + m6


def _slab(ref, *lead, rows=None):
    lo, hi = rows or (0, ref.shape[-2])
    return pltpu.bitcast(ref.bitcast(_U32)[(*lead, slice(lo // 2, hi // 2))], _BF16)


def _cat(xs, axis):
    return xs[0] if len(xs) == 1 else jnp.concatenate(xs, axis=axis)


def _fold(op, x, rows):
    return [functools.reduce(op, [x[r:r + 8] for r in range(lo, min(lo + rows, x.shape[0]), 8)])
            for lo in range(0, x.shape[0], rows)]


def _interleave(streams):
    keyed = []
    for steps in streams:
        total, done = sum(cost for cost, _ in steps), 0
        for cost, step in steps:
            keyed.append(((done + cost / 2) / total, len(keyed), step))
            done += cost
    return [step for _, _, step in sorted(keyed, key=lambda item: item[:2])]


def _kernel(
    xT_hbm, c_hbm, wq_hbm, wuk_hbm, wuv_hbm, woT_hbm, wr_hbm, wg_hbm, wu_hbm, wdT_hbm, gw_hbm,
    outT_hbm,
    xT, c, wr, gw, first_words, next_words, woT, ffn_w, outT, io_sems, head_sems,
    x_ops, c_ops, wq_ops, wk_ops, wv_ops, wo_ops, q_ops, k_ops, v_ops, ctx_ops, acc,
    gate, score, x_sel, y_sel, y_scale, routed,
    *, tuning, only=None,
):
    M, S = xT.shape
    Dc, H, D = wuk_hbm.shape
    U = S // (2 * _T)
    n_chunks = wg_hbm.shape[1] // _T
    mh, kt = M // 2, Dc // 2 // _T
    block = lambda u: slice(2 * u * _T, 2 * (u + 1) * _T)
    tile = lambda t: slice(t * _T, (t + 1) * _T)
    weights = {"wq": (0, wq_hbm, wq_ops), "wk": (1, wuk_hbm, wk_ops), "wv": (2, wuv_hbm, wv_ops)}

    io = {name: [(src.bitcast(_U32).at[:, 0, :], first_words[i])]
          for name, (i, src, _) in weights.items()}
    io["x"] = [(xT_hbm, xT)]
    io["vec"] = [(wr_hbm, wr), (gw_hbm, gw)]
    for u in range(U):
        io[f"c{u}"] = [(c_hbm.at[block(u)], c.at[block(u)])]
        io[f"out{u}"] = [(outT.at[:, block(u)], outT_hbm.at[:, block(u)])]
    slots = iter(range(io_sems.shape[0]))
    io = {name: [pltpu.make_async_copy(src, dst, io_sems.at[next(slots)]) for src, dst in pairs]
          for name, pairs in io.items()}

    def wait(name):
        for copy in io[name]:
            copy.wait()

    def head_copies(h):
        pair = jnp.minimum(h + 1, H - 1) // 2
        chunk = pl.ds(pl.multiple_of(jnp.minimum(h, n_chunks - 1) * _T, _T), _T)
        pairs = [(woT_hbm.at[h], woT)]
        pairs += [(src.bitcast(_U32).at[:, pair, tile(n)], next_words[i].at[n])
                  for i, src, _ in weights.values() for n in range(2)]
        pairs += [(src.at[:, chunk], dst) for src, dst in zip((wg_hbm, wu_hbm, wdT_hbm), ffn_w)]
        return [pltpu.make_async_copy(src, dst, head_sems.at[i]) for i, (src, dst) in enumerate(pairs)]

    def prepare_weight(name, head, first):
        i, src, dst = weights[name]
        transposed = name != "wk"
        shift = jnp.asarray(16 * (1 - head % 2)).astype(_U32)
        half = src.shape[0] // 2
        step = _T if transposed else _ROWS
        for r in range(0, half, step):
            n_rows = min(step, half - r)
            quads = []
            for f in range(2):
                rows = slice(f * half + r, f * half + r + n_rows)
                for n in range(2):
                    words = first_words[i][rows, tile(n)] if first else next_words[i][n, rows]
                    words = words.T if transposed else words
                    quads.append(pltpu.bitcast((words << shift) & _U32(0xFFFF0000), _F32))
            for j, op in enumerate(_rhs_operands(*quads)):
                if not transposed:
                    dst[j, r:r + n_rows] = op.astype(_BF16)
                    continue
                if n_rows < _T:
                    op = jnp.concatenate([op, jnp.zeros((_T, _T - n_rows), _F32)], axis=1)
                dst[j, r // _T] = op.astype(_BF16)

    def prepare_wo():
        for r in range(0, mh, _ROWS):
            top, bottom = (woT[f * mh + r:f * mh + r + _ROWS].astype(_F32) for f in range(2))
            for j, op in enumerate(_lhs_operands(top[:, :_T], top[:, _T:], bottom[:, :_T], bottom[:, _T:])):
                wo_ops[j, r:r + _ROWS] = op.astype(_BF16)

    def prepare_c(u):
        for r in range(0, _T, _ROWS):
            ca, cb = (c[(2 * u + f) * _T + r:(2 * u + f) * _T + r + _ROWS].astype(_F32) for f in range(2))
            ops = _lhs_operands(ca[:, :Dc // 2], ca[:, Dc // 2:], cb[:, :Dc // 2], cb[:, Dc // 2:])
            for j, op in enumerate(ops):
                for t in range(kt):
                    c_ops[j, t, u * _T + r:u * _T + r + _ROWS] = op[:, tile(t)].astype(_BF16)

    def prepare_x():
        for u in range(U):
            for r in range(0, mh, _ROWS):
                x0, x1 = (xT[f * mh + r:f * mh + r + _ROWS, block(u)].astype(_F32) for f in range(2))
                for j, op in enumerate(_lhs_operands(x0[:, :_T], x1[:, :_T], x0[:, _T:], x1[:, _T:])):
                    x_ops[j, u, r:r + _ROWS] = op.astype(_BF16)

    lane = lax.broadcasted_iota(jnp.int32, (1, _T), 1)
    tile_of = lambda token: pl.ds(pl.multiple_of(token // _T * _T, _T), _T)

    def score_tokens(u0, u1):
        def step(t):
            row = lax.broadcasted_iota(jnp.int32, (_ROWS, M), 0)
            vectors = jnp.where(row == 0, *(v[...].astype(_F32).reshape(1, M) for v in (wr, gw)))
            dots = _dot(vectors.astype(_BF16), xT[:, tile(t)])
            score[t:t + 1] = dots[0:1].astype(xT.dtype).astype(_F32)
            gate[t:t + 1] = jax.nn.sigmoid(dots[1:2])
        return [(1, functools.partial(step, t)) for t in range(2 * u0, 2 * u1)]

    def route():
        r = score[...]
        r = jnp.where(r == r, r, -jnp.inf)
        token = (lax.broadcasted_iota(jnp.int32, r.shape, 0) * _T
                 + lax.broadcasted_iota(jnp.int32, r.shape, 1)).astype(_F32)
        free = token >= 0
        slot = lax.broadcasted_iota(jnp.int32, (_ROWS, _T), 0)
        picked = []
        for n in range(_CAPACITY):
            best = jnp.max(jnp.where(free, r, -jnp.inf), keepdims=True)
            choice = jnp.min(jnp.where(free & (r == best), token, S - 1.0))
            free = free & (token != choice)
            index = choice.astype(jnp.int32)
            routed[n] = index
            y_scale[n:n + 1] = jnp.broadcast_to(jax.nn.sigmoid(best), (1, _T))
            onehot = jnp.where((slot == n) & (lane == index % _T), 1.0, 0.0)
            picked.append(_dot(onehot.astype(_BF16), xT[:, tile_of(index)], _NT))
        x_sel[...] = functools.reduce(jnp.add, picked).astype(_BF16)

    def ffn_steps(chunk):
        hidden = []

        def up():
            g, u = (_dot(x_sel[...], _slab(w)) for w in ffn_w[:2])
            hidden.append(jnp.where(chunk < n_chunks, g * jax.nn.sigmoid(g) * u, 0.0))

        def down():
            y_sel[...] += _dot(hidden.pop().astype(_BF16), _slab(ffn_w[2]), _NT)
        return {"up": up, "down": down}

    def add_routed_update():
        yT = jnp.concatenate([y_sel[...], jnp.zeros((_T - _ROWS, M), _F32)], axis=0).T
        for n in range(_CAPACITY):
            index = routed[n]
            x = xT[:, tile_of(index)].astype(_F32)
            y = yT[:, n:n + 1] * y_scale[n:n + 1]
            xT[:, tile_of(index)] = jnp.where(lane == index % _T, x + y, x).astype(xT.dtype)

    def seven_products(cost, product, finish):
        m = []

        def step(j):
            m.append(product(j))
            if j == 6:
                finish(*_combine(*m))
        return [(cost, functools.partial(step, j)) for j in range(7)]

    def c_operand(j, u0, u1):
        return _cat([_slab(c_ops, j, t, rows=(u0 * _T, u1 * _T)) for t in range(kt)], 1)

    def project_k(u0, u1):
        def finish(ka0, ka1, kb0, kb1):
            for j, op in enumerate(_lhs_operands(kb0, kb1, ka0, ka1)):
                for u in range(u0, u1):
                    k_ops[u][j] = op[tile(u - u0)].astype(_BF16)
        product = lambda j: _dot(c_operand(j, u0, u1), _slab(wk_ops, j))
        return seven_products(kt * (u1 - u0) * _T, product, finish)

    def project_q(u0, u1):
        def product(j):
            w = _cat([_slab(wq_ops, j, t) for t in range(wq_ops.shape[1])], 1)[:, :mh]
            return _dot(w, _cat([_slab(x_ops, j, u) for u in range(u0, u1)], 1))

        def finish(*q):
            qa0, qa1, qb0, qb1 = (part * (D ** -0.5 * _LOG2E) for part in q)
            for j, op in enumerate(_rhs_operands(qa0, qb0, qa1, qb1)):
                for u in range(u0, u1):
                    q_ops[u][j] = op[:, tile(u - u0)].astype(_BF16)
        return seven_products(2 * (u1 - u0) * _T, product, finish)

    def project_v(u0, u1):
        def product(j):
            return _dot(_cat([_slab(wv_ops, j, t) for t in range(kt)], 1), c_operand(j, u0, u1), _NT)

        def finish(va0, va1, vb0, vb1):
            for j, op in enumerate(_lhs_operands(vb0, va0, vb1, va1) + (va0, vb1)):
                for u in range(u0, u1):
                    v_ops[u][j] = op[:, tile(u - u0)].astype(_BF16)
        return seven_products(kt * (u1 - u0) * _T, product, finish)

    out_product = lambda u, j: _dot(_slab(wo_ops, j), _slab(ctx_ops[u], j))

    def project_out(u, _):
        def step(j):
            acc[u][j] += out_product(u, j)
        return [(mh, functools.partial(step, j)) for j in range(7)]

    def run(program, actions):
        ranged = {"K": project_k, "Q": project_q, "V": project_v, "O": project_out, "R": score_tokens}

        def steps(word):
            if word in actions:
                return [(1e-3, actions[word])]
            lo, _, hi = word[1:].partition("-")
            return ranged[word[0]](int(lo), int(hi) if hi else int(lo) + 1)
        for phase in program.split(";"):
            for step in _interleave([[s for word in part.split() for s in steps(word)]
                                     for part in phase.split("|")]):
                step()

    def mask_last_tile(s):
        key = lax.broadcasted_iota(jnp.int32, (_T, _T), 0)
        query = lax.broadcasted_iota(jnp.int32, (_T, _T), 1)
        n = s.shape[0] - _T
        return _cat([s[:n]] * (n > 0) + [jnp.where(key <= query, s[n:], -1e9 * _LOG2E)], 0)

    def softmax_shift(parts, prescale):
        peaks = [peak for s in parts for peak in _fold(jnp.maximum, s, _T)]
        top = jnp.max(functools.reduce(jnp.maximum, peaks), axis=0, keepdims=True)
        if not prescale:
            return top
        bound = functools.reduce(jnp.add, [jnp.exp2(peak - top) for peak in peaks])
        bound = jnp.sum(bound, axis=0, keepdims=True)
        return top + ((pltpu.bitcast(bound, jnp.int32) >> 23) - 127).astype(_F32)

    def weighted_values(u, s):
        p, total, m = {}, {}, {}

        def softmax():
            for half in "ab":
                names = [name for name in s if name[1] == half]
                shift = softmax_shift([s[name] for name in names], u > 0)
                p.update({name: jnp.exp2(s[name] - shift) for name in names})
                sums = [x for name in names for x in _fold(jnp.add, p[name], tuning["sum_rows"][u])]
                total[half] = jnp.sum(functools.reduce(jnp.add, sums), axis=0, keepdims=True)

        def step(into, v, t, probs):
            if not p:
                softmax()
            product = _dot(_slab(v_ops[t], v), probs(lambda name: p[name][tile(t)]).astype(_BF16))
            m[into] = m[into] + product if into in m else product

        def finish():
            c0a, c0b, c1a, c1b = m["0a"], m["0b"], m["1a"], m["1b"]
            if u:
                c0a, c0b = c0a + (m[3] - m[4]) + m[0], c0b + m[2] + m[4]
                c1a, c1b = c1a + m[1] + m[3], c1b + (m[2] - m[1]) + m[0]
            fa, fb = (gate[2 * u + i:2 * u + i + 1] / total[half] for i, half in enumerate("ab"))
            for j, op in enumerate(_rhs_operands(c0a * fa, c0b * fb, c1a * fa, c1b * fb)):
                ctx_ops[u][j] = op.astype(_BF16)

        rhs = lambda j: lambda get: _rhs_operands(get("ba"), get("bb"), get("aa"), get("ab"))[j]
        diagonal = [("0a", 7, "aa"), ("0b", 7, "ab"), ("0b", 2, "bb"),
                    ("1a", 3, "aa"), ("1b", 3, "ab"), ("1b", 8, "bb")]
        steps = []
        for j in tuning["pv_order"][u]:
            if j == 7:
                steps += [functools.partial(step, into, v, u, lambda get, name=name: get(name))
                          for into, v, name in (diagonal[i] for i in tuning["diag_order"][u])]
            else:
                into = {5: "1b", 6: "0a"}.get(j, j)
                steps += [functools.partial(step, into, j, t, rhs(j)) for t in range(u)]
        last = steps.pop()
        return steps + [lambda: (last(), finish())]

    def attention():
        load, pending = [0] * 4, []

        def issue(tiles, step):
            load[load.index(min(load))] += tiles
            return step()

        def level():
            while pending and min(load) < max(load):
                issue(1, pending.pop(0))

        def scores(u):
            def product(j):
                n = u if j == 6 else u + 1
                keys = lambda: _cat([_slab(k_ops[t], j) for t in range(n)], 0)
                return issue(n, lambda: _dot(keys(), _slab(q_ops[u], j)))
            m2, m4, m6 = product(1), product(3), product(5)
            s = {"aa": mask_last_tile(m2 + m4)}
            ab = m6 - m2
            if u:
                ba = m4[:u * _T] + product(6)
            level()
            m1, m3, m5 = product(0), product(2), product(4)
            if u:
                s["ba"] = ba + (m1 - m5)[:u * _T]
            s["bb"] = mask_last_tile(m3 + m5)
            s["ab"] = ab + (m1 + m3)
            level()
            return s

        for group, held in zip(tuning["score_order"], tuning["held_back"]):
            done = [(u, scores(u)) for u in group]
            while len(pending) >= 4 + held:
                for _ in range(4):
                    issue(1, pending.pop(0))
            for u, s in done:
                steps = weighted_values(u, s)
                n = min(tuning["overlap"][u], len(pending), len(steps))
                tail = [pending.pop() for _ in range(n)][::-1]
                pending.extend([step for pair in zip(tail, steps) for step in pair] + steps[n:])
        for step in pending:
            step()

    for name in tuning["first_copies"].split():
        for copy in io[name]:
            copy.start()
    for ref in (*acc, y_sel):
        ref[...] = jnp.zeros_like(ref)
    actions = {"!" + name: functools.partial(wait, name) for name in io}
    actions.update({name: functools.partial(prepare_weight, name, 0, True) for name in weights})
    actions.update({f"c{u}": functools.partial(prepare_c, u) for u in range(U)})
    actions.update(x=prepare_x, route=route)
    run(tuning["first"] if only != "b" else " ".join("!" + n for n in tuning["first_copies"].split()), actions)
    for copy in head_copies(0):
        copy.start()

    def head(h, carry):
        if only != "first":
            attention()
        for copy in head_copies(h):
            copy.wait()

        @pl.when(h + 1 < H)
        def _():
            actions = {name: functools.partial(prepare_weight, name, h + 1, False) for name in weights}
            if only is None:
                run(tuning["projections"], dict(actions, wo=prepare_wo, **ffn_steps(h)))
            for copy in head_copies(h + 1):
                copy.start()
        return carry

    lax.fori_loop(0, H, head, None)

    prepare_wo()
    add_routed_update()
    for u in range(U):
        attended = _combine(*(acc[u][j] + out_product(u, j) for j in range(7)))
        keep = 1.0 - jnp.concatenate([gate[2 * u:2 * u + 1], gate[2 * u + 1:2 * u + 2]], axis=1)
        for f in range(2):
            rows = slice(f * mh, (f + 1) * mh)
            mixed = (keep * xT[rows, block(u)].astype(_F32)
                     + jnp.concatenate(attended[2 * f:2 * f + 2], axis=1))
            outT[rows, block(u)] = mixed.astype(outT.dtype)
        io[f"out{u}"][0].start()
    for u in range(U):
        wait(f"out{u}")


def make(only=None, **tuning):
    def fn(A_x, A_c_kv, A_w_q, A_w_uk, A_w_uv, A_w_o, B_x, B_w_r, B_w_gate, B_w_up, B_w_down, gate_w):
        del B_x
        _, S, M = A_x.shape
        Dc, H, D = A_w_uk.shape
        U = S // (2 * _T)
        assert D == 2 * _T and A_c_kv.shape[1] == S and B_w_gate.shape[1] // _T < H
        vmem = pltpu.VMEM
        tiles = lambda n: [vmem((n, _T, _T), _BF16)] * U
        hbm = pl.BlockSpec(memory_space=pl.ANY)
        outT = pl.pallas_call(
            functools.partial(_kernel, tuning=dict(_TUNING, **tuning), only=only),
            in_specs=[hbm] * 11,
            out_specs=hbm,
            out_shape=jax.ShapeDtypeStruct((M, S), A_x.dtype),
            scratch_shapes=[
                vmem((M, S), _BF16), vmem((S, Dc), _BF16), vmem((M,), _BF16), vmem((M,), _BF16),
                [vmem((n, D), _U32) for n in (M, Dc, Dc)],
                [vmem((2, n, _T), _U32) for n in (M, Dc, Dc)],
                vmem((M, D), _BF16), [vmem((M, _T), _BF16)] * 3, vmem((M, S), _BF16),
                pltpu.SemaphoreType.DMA((6 + 2 * U,)), pltpu.SemaphoreType.DMA((10,)),
                vmem((7, U, M // 2, _T), _BF16), vmem((7, Dc // 2 // _T, S // 2, _T), _BF16),
                vmem((7, pl.cdiv(M // 2, _T), _T, _T), _BF16), vmem((7, Dc // 2, _T), _BF16),
                vmem((7, Dc // 2 // _T, _T, _T), _BF16), vmem((7, M // 2, _T), _BF16),
                tiles(7), tiles(7), tiles(9), tiles(7), [vmem((7, M // 2, _T), _F32)] * U,
                vmem((2 * U, _T), _F32), vmem((2 * U, _T), _F32),
                vmem((_ROWS, M), _BF16), vmem((_ROWS, M), _F32), vmem((_CAPACITY, _T), _F32),
                pltpu.SMEM((_CAPACITY,), jnp.int32),
            ],
            compiler_params=pltpu.CompilerParams(vmem_limit_bytes=100 * 2**20, disable_bounds_checks=True),
            name="gm_kernel",
        )(A_x[0].T, A_c_kv[0], A_w_q, A_w_uk, A_w_uv, A_w_o.transpose(0, 2, 1),
          B_w_r, B_w_gate, B_w_up, B_w_down.T, gate_w)
        return outT.T[None]
    return fn


@jax.jit
def pallas_gated_mix__compressed_kv_cla__moe_arch_mod__prompt_kernel(
    A_x, A_c_kv, A_w_q, A_w_uk, A_w_uv, A_w_o, B_x, B_w_r, B_w_gate, B_w_up, B_w_down, gate_w
):
    return make()(A_x, A_c_kv, A_w_q, A_w_uk, A_w_uv, A_w_o, B_x, B_w_r, B_w_gate, B_w_up, B_w_down, gate_w)
```

```python
import functools
import math

import jax
import jax.numpy as jnp
from jax import lax
import jax.experimental.pallas as pl
import jax.experimental.pallas.tpu as pltpu

_NN = (((1,), (0,)), ((), ()))
_NT = (((1,), (1,)), ((), ()))
_F32 = jnp.float32
_BF16 = jnp.bfloat16
_U32 = jnp.uint32
_LOG2E = math.log2(math.e)
_T = 128
_ROWS = 16
_CAPACITY = 2

_FIRST_COPIES = "wv c0 wk c1 c2 c3 c4 c5 c6 c7 vec wq x"
_FIRST_PROJECTIONS = (
    "!wv wv !c0 c0 V0 !wk wk K0 !c1 c1 K1 V1 !c2 !c3 c2 c3 K2-4 V2-4"
    " !c4 !c5 !c6 c4 c5 c6 V4-6 V6 K4-6 !c7 !vec !wq !x c7 wq x;"
    " K6 | R0-8; K7 | Q0 Q1 Q2 Q3; route; V7 | Q4 Q5 Q6 Q7")
_PROJECTIONS = (
    "wo wk wq wv O0 O1 O2;"
    " K0-2 K2-8 V0-2 V2-4 V4-6 V6-8 | O3 up Q0-2 down Q2-4 O4 Q4-6 Q6-8 O5; O6 O7")
_ATTENTION = (
    'D0@6 D1@12 D3@0 S1 S2 D2@2 -1 C1@12 D4@6 S3 -0 C2@0 C0@2 S4 D5@4'
    ' -3 C3@8 S5 D6@2 -3 C4@2 D7@2 S6 -3 C5@2 S7 -0 C7@12 C6@0')
_PV_ORDER = ("41063527", "14052637", "14036257", "14036752", "41073265", "14073562", "14023567", "14036257")
_DIAGONAL_ORDER = ("531024", "012345", "012345", "341205", "420153", "530421", "012345", "250413")
_SUM_ROWS = (64, 1024, 1024, 1024, 256, 32, 256, 32)
_THREE_FIRST = (4, 5)
_REVERSED_MAX = ('', '', 'b', 'a', 'a', '', '', 'b')


def _dot(a, b, dims=_NN):
    return lax.dot_general(a, b, dims, preferred_element_type=_F32)


def _lhs_operands(a11, a12, a21, a22):
    return (a11 + a22, a21 + a22, a11, a22, a11 + a12, a21 - a11, a12 - a22)


def _rhs_operands(b11, b12, b21, b22):
    return (b11 + b22, b11, b12 - b22, b21 - b11, b22, b11 + b12, b21 + b22)


def _combine(m1, m2, m3, m4, m5, m6, m7):
    return m1 + m4 - m5 + m7, m3 + m5, m2 + m4, m1 - m2 + m3 + m6


def _slab(ref, *lead):
    return pltpu.bitcast(ref.bitcast(_U32)[(*lead, slice(None), slice(None))], _BF16)


def _cat(xs, axis):
    return xs[0] if len(xs) == 1 else jnp.concatenate(xs, axis=axis)


def _fold(op, x, rows):
    return [functools.reduce(op, [x[r:r + 8] for r in range(lo, min(lo + rows, x.shape[0]), 8)])
            for lo in range(0, x.shape[0], rows)]


def _interleave(streams):
    keyed = []
    for steps in streams:
        total, done = sum(cost for cost, _ in steps), 0
        for cost, step in steps:
            keyed.append(((done + cost / 2) / total, len(keyed), step))
            done += cost
    return [step for _, _, step in sorted(keyed, key=lambda item: item[:2])]


def _kernel(
    xT_hbm, c_hbm, wq_hbm, wuk_hbm, wuv_hbm, woT_hbm, wr_hbm, wg_hbm, wu_hbm, wdT_hbm, gw_hbm,
    outT_hbm,
    xT, c, wr, gw, first_words, next_words, woT, ffn_w, outT, io_sems, head_sems,
    x_ops, c_ops, wq_ops, wk_ops, wv_ops, wo_ops, q_ops, k_ops, v_ops, ctx_ops, acc,
    gate, score, x_sel, y_sel, y_scale, routed,
):
    M, S = xT.shape
    Dc, H, D = wuk_hbm.shape
    U = S // (2 * _T)
    n_chunks = wg_hbm.shape[1] // _T
    mh, kt = M // 2, Dc // 2 // _T
    block = lambda u: slice(2 * u * _T, 2 * (u + 1) * _T)
    tile = lambda t: slice(t * _T, (t + 1) * _T)
    weights = {"wq": (0, wq_hbm, wq_ops), "wk": (1, wuk_hbm, wk_ops), "wv": (2, wuv_hbm, wv_ops)}

    io = {name: [(src.bitcast(_U32).at[:, 0, :], first_words[i])]
          for name, (i, src, _) in weights.items()}
    io["x"] = [(xT_hbm, xT)]
    io["vec"] = [(wr_hbm, wr), (gw_hbm, gw)]
    for u in range(U):
        io[f"c{u}"] = [(c_hbm.at[block(u)], c.at[block(u)])]
        io[f"out{u}"] = [(outT.at[:, block(u)], outT_hbm.at[:, block(u)])]
    slots = iter(range(io_sems.shape[0]))
    io = {name: [pltpu.make_async_copy(src, dst, io_sems.at[next(slots)]) for src, dst in pairs]
          for name, pairs in io.items()}

    def wait(name):
        for copy in io[name]:
            copy.wait()

    def head_copies(h):
        pair = jnp.minimum(h + 1, H - 1) // 2
        chunk = pl.ds(pl.multiple_of(jnp.minimum(h, n_chunks - 1) * _T, _T), _T)
        pairs = [(woT_hbm.at[h], woT)]
        pairs += [(src.bitcast(_U32).at[:, pair, tile(n)], next_words[i].at[n])
                  for i, src, _ in weights.values() for n in range(2)]
        pairs += [(src.at[:, chunk], dst) for src, dst in zip((wg_hbm, wu_hbm, wdT_hbm), ffn_w)]
        return [pltpu.make_async_copy(src, dst, head_sems.at[i]) for i, (src, dst) in enumerate(pairs)]

    def prepare_weight(name, head, first):
        i, src, dst = weights[name]
        transposed = name != "wk"
        shift = jnp.asarray(16 * (1 - head % 2)).astype(_U32)
        half = src.shape[0] // 2
        step = _T if transposed else _ROWS
        for r in range(0, half, step):
            n_rows = min(step, half - r)
            quads = []
            for f in range(2):
                rows = slice(f * half + r, f * half + r + n_rows)
                for n in range(2):
                    words = first_words[i][rows, tile(n)] if first else next_words[i][n, rows]
                    words = words.T if transposed else words
                    quads.append(pltpu.bitcast((words << shift) & _U32(0xFFFF0000), _F32))
            for j, op in enumerate(_rhs_operands(*quads)):
                if not transposed:
                    dst[j, r:r + n_rows] = op.astype(_BF16)
                    continue
                if n_rows < _T:
                    op = jnp.concatenate([op, jnp.zeros((_T, _T - n_rows), _F32)], axis=1)
                dst[j, r // _T] = op.astype(_BF16)

    def prepare_wo():
        for r in range(0, mh, _ROWS):
            top, bottom = (woT[f * mh + r:f * mh + r + _ROWS].astype(_F32) for f in range(2))
            for j, op in enumerate(_lhs_operands(top[:, :_T], top[:, _T:], bottom[:, :_T], bottom[:, _T:])):
                wo_ops[j, r:r + _ROWS] = op.astype(_BF16)

    def prepare_c(u):
        for r in range(0, _T, _ROWS):
            ca, cb = (c[(2 * u + f) * _T + r:(2 * u + f) * _T + r + _ROWS].astype(_F32) for f in range(2))
            ops = _lhs_operands(ca[:, :Dc // 2], ca[:, Dc // 2:], cb[:, :Dc // 2], cb[:, Dc // 2:])
            for j, op in enumerate(ops):
                for t in range(kt):
                    c_ops[u][j, t, r:r + _ROWS] = op[:, tile(t)].astype(_BF16)

    def prepare_x():
        for u in range(U):
            for r in range(0, mh, _ROWS):
                x0, x1 = (xT[f * mh + r:f * mh + r + _ROWS, block(u)].astype(_F32) for f in range(2))
                for j, op in enumerate(_lhs_operands(x0[:, :_T], x1[:, :_T], x0[:, _T:], x1[:, _T:])):
                    x_ops[j, u, r:r + _ROWS] = op.astype(_BF16)

    lane = lax.broadcasted_iota(jnp.int32, (1, _T), 1)
    tile_of = lambda token: pl.ds(pl.multiple_of(token // _T * _T, _T), _T)

    def score_tokens(u0, u1):
        def step(t):
            row = lax.broadcasted_iota(jnp.int32, (_ROWS, M), 0)
            vectors = jnp.where(row == 0, *(v[...].astype(_F32).reshape(1, M) for v in (wr, gw)))
            dots = _dot(vectors.astype(_BF16), xT[:, tile(t)])
            score[t:t + 1] = dots[0:1].astype(xT.dtype).astype(_F32)
            gate[t:t + 1] = jax.nn.sigmoid(dots[1:2])
        return [(1, functools.partial(step, t)) for t in range(2 * u0, 2 * u1)]

    def route():
        r = score[...]
        r = jnp.where(r == r, r, -jnp.inf)
        token = (lax.broadcasted_iota(jnp.int32, r.shape, 0) * _T
                 + lax.broadcasted_iota(jnp.int32, r.shape, 1)).astype(_F32)
        free = token >= 0
        slot = lax.broadcasted_iota(jnp.int32, (_ROWS, _T), 0)
        picked = []
        for n in range(_CAPACITY):
            best = jnp.max(jnp.where(free, r, -jnp.inf), keepdims=True)
            choice = jnp.min(jnp.where(free & (r == best), token, S - 1.0))
            free = free & (token != choice)
            index = choice.astype(jnp.int32)
            routed[n] = index
            y_scale[n:n + 1] = jnp.broadcast_to(jax.nn.sigmoid(best), (1, _T))
            onehot = jnp.where((slot == n) & (lane == index % _T), 1.0, 0.0)
            picked.append(_dot(onehot.astype(_BF16), xT[:, tile_of(index)], _NT))
        x_sel[...] = functools.reduce(jnp.add, picked).astype(_BF16)

    def ffn_steps(chunk):
        hidden = []

        def up():
            g, u = (_dot(x_sel[...], _slab(w)) for w in ffn_w[:2])
            hidden.append(jnp.where(chunk < n_chunks, g * jax.nn.sigmoid(g) * u, 0.0))

        def down():
            y_sel[...] += _dot(hidden.pop().astype(_BF16), _slab(ffn_w[2]), _NT)
        return {"up": up, "down": down}

    def add_routed_update():
        yT = jnp.concatenate([y_sel[...], jnp.zeros((_T - _ROWS, M), _F32)], axis=0).T
        for n in range(_CAPACITY):
            index = routed[n]
            x = xT[:, tile_of(index)].astype(_F32)
            y = yT[:, n:n + 1] * y_scale[n:n + 1]
            xT[:, tile_of(index)] = jnp.where(lane == index % _T, x + y, x).astype(xT.dtype)

    def seven_products(cost, product, finish):
        m = []

        def step(j):
            m.append(product(j))
            if j == 6:
                finish(*_combine(*m))
        return [(cost, functools.partial(step, j)) for j in range(7)]

    def c_operand(j, u0, u1):
        return _cat([_cat([_slab(c_ops[u], j, t) for t in range(kt)], 1) for u in range(u0, u1)], 0)

    def project_k(u0, u1):
        def finish(ka0, ka1, kb0, kb1):
            for j, op in enumerate(_lhs_operands(kb0, kb1, ka0, ka1) + (kb1, ka0)):
                for u in range(u0, u1):
                    k_ops[u][j] = op[tile(u - u0)].astype(_BF16)
        product = lambda j: _dot(c_operand(j, u0, u1), _slab(wk_ops, j))
        return seven_products(kt * (u1 - u0) * _T, product, finish)

    def project_q(u0, u1):
        def product(j):
            w = _cat([_slab(wq_ops, j, t) for t in range(wq_ops.shape[1])], 1)[:, :mh]
            return _dot(w, _cat([_slab(x_ops, j, u) for u in range(u0, u1)], 1))

        def finish(*q):
            qa0, qa1, qb0, qb1 = (part * (D ** -0.5 * _LOG2E) for part in q)
            for j, op in enumerate(_rhs_operands(qa0, qb0, qa1, qb1) + (qb0, qa1)):
                for u in range(u0, u1):
                    q_ops[u][j] = op[:, tile(u - u0)].astype(_BF16)
        return seven_products(2 * (u1 - u0) * _T, product, finish)

    def project_v(u0, u1):
        def product(j):
            return _dot(_cat([_slab(wv_ops, j, t) for t in range(kt)], 1), c_operand(j, u0, u1), _NT)

        def finish(va0, va1, vb0, vb1):
            for j, op in enumerate(_lhs_operands(vb0, va0, vb1, va1) + (va0, vb1)):
                for u in range(u0, u1):
                    v_ops[u][j] = op[:, tile(u - u0)].astype(_BF16)
        return seven_products(kt * (u1 - u0) * _T, product, finish)

    out_product = lambda u, j: _dot(_slab(wo_ops, j), _slab(ctx_ops[u], j))

    def project_out(u, _):
        def step(j):
            acc[u][j] += out_product(u, j)
        return [(mh, functools.partial(step, j)) for j in range(7)]

    def run(program, actions):
        ranged = {"K": project_k, "Q": project_q, "V": project_v, "O": project_out, "R": score_tokens}

        def steps(word):
            if word in actions:
                return [(1e-3, actions[word])]
            lo, _, hi = word[1:].partition("-")
            return ranged[word[0]](int(lo), int(hi) if hi else int(lo) + 1)
        for phase in program.split(";"):
            for step in _interleave([[s for word in part.split() for s in steps(word)]
                                     for part in phase.split("|")]):
                step()

    def causal(s):
        key = lax.broadcasted_iota(jnp.int32, (_T, _T), 0)
        query = lax.broadcasted_iota(jnp.int32, (_T, _T), 1)
        return jnp.where(key <= query, s, -1e9 * _LOG2E)

    def softmax_shift(parts, prescale):
        peaks = [peak for s in parts for peak in _fold(jnp.maximum, s, _T)]
        top = jnp.max(functools.reduce(jnp.maximum, peaks), axis=0, keepdims=True)
        if not prescale:
            return top
        bound = functools.reduce(jnp.add, [jnp.exp2(peak - top) for peak in peaks])
        bound = jnp.sum(bound, axis=0, keepdims=True)
        return top + ((pltpu.bitcast(bound, jnp.int32) >> 23) - 127).astype(_F32)

    def weighted_values(u, scores):
        p, total, m = {}, {}, {}

        def softmax():
            s = scores()
            for half in "ab":
                names = [name for name in s if name[1] == half]
                parts = [s[name] for name in names]
                shift = softmax_shift(parts[::-1] if half in _REVERSED_MAX[u] else parts, u > 0)
                p.update({name: jnp.exp2(s[name] - shift) for name in names})
                sums = [x for name in names for x in _fold(jnp.add, p[name], _SUM_ROWS[u])]
                total[half] = jnp.sum(functools.reduce(jnp.add, sums), axis=0, keepdims=True)

        def step(into, v, t, probs):
            if not p:
                softmax()
            product = _dot(_slab(v_ops[t], v), probs(lambda name: p[name][tile(t)]).astype(_BF16))
            m[into] = m[into] + product if into in m else product

        def finish():
            c0a, c0b, c1a, c1b = m["0a"], m["0b"], m["1a"], m["1b"]
            if u:
                c0a, c0b = c0a + (m[3] - m[4]) + m[0], c0b + m[2] + m[4]
                c1a, c1b = c1a + m[1] + m[3], c1b + (m[2] - m[1]) + m[0]
            fa, fb = (gate[2 * u + i:2 * u + i + 1] / total[half] for i, half in enumerate("ab"))
            for j, op in enumerate(_rhs_operands(c0a * fa, c0b * fb, c1a * fa, c1b * fb)):
                ctx_ops[u][j] = op.astype(_BF16)

        rhs = lambda j: lambda get: _rhs_operands(get("ba"), get("bb"), get("aa"), get("ab"))[j]
        diagonal = [("0a", 7, "aa"), ("0b", 7, "ab"), ("0b", 2, "bb"),
                    ("1a", 3, "aa"), ("1b", 3, "ab"), ("1b", 8, "bb")]
        steps = []
        for j in map(int, _PV_ORDER[u]):
            if j == 7:
                steps += [functools.partial(step, into, v, u, lambda get, name=name: get(name))
                          for into, v, name in (diagonal[int(i)] for i in _DIAGONAL_ORDER[u])]
            else:
                into = {5: "1b", 6: "0a"}.get(j, j)
                steps += [functools.partial(step, into, j, t, rhs(j)) for t in range(u)]
        last = steps.pop()
        return steps + [lambda: (last(), finish())]

    def attention():
        load, pending = [0] * 4, []

        def issue(tiles, step):
            load[load.index(min(load))] += tiles
            return step()

        def level():
            while pending and min(load) < max(load):
                issue(1, pending.pop(0))

        below, diagonal = {}, {}

        def diagonal_scores(u):
            def product(name, k, q):
                m = _dot(_slab(k_ops[u], k), _slab(q_ops[u], q))
                diagonal[u, name] = diagonal[u, name] + m if (u, name) in diagonal else m
            return [functools.partial(product, *spec) for spec in (
                ("aa", 8, 1), ("aa", 3, 8), ("ab", 8, 7), ("ab", 3, 4), ("bb", 2, 7), ("bb", 7, 4))]

        def scores(u):
            def product(j):
                keys = lambda: _cat([_slab(k_ops[t], j) for t in range(u)], 0)
                return issue(u, lambda: _dot(keys(), _slab(q_ops[u], j)))
            groups = ((1, 3, 5, 6), (0, 2, 4))
            m = {}
            for group in groups[::-1] if u in _THREE_FIRST else groups:
                m.update({j: product(j) for j in group})
                level()
            m1, m2, m3, m4, m5, m6, m7 = (m[j] for j in range(7))
            below[u] = dict(aa=m2 + m4, ba=(m4 + m7) + (m1 - m5), bb=m3 + m5, ab=(m6 - m2) + (m1 + m3))

        def all_scores(u):
            s = dict(aa=causal(diagonal[u, "aa"]), bb=causal(diagonal[u, "bb"]), ab=diagonal[u, "ab"])
            if u:
                s = {name: _cat([part] + ([s[name]] if name in s else []), 0)
                     for name, part in below[u].items()}
            return s

        for word in _ATTENTION.split():
            if word[0] == "S":
                scores(int(word[1:]))
            elif word[0] == "-":
                while len(pending) >= 4 + int(word[1:]):
                    for _ in range(4):
                        issue(1, pending.pop(0))
            else:
                u, _, n = word[1:].partition("@")
                steps = (diagonal_scores(int(u)) if word[0] == "D"
                         else weighted_values(int(u), functools.partial(all_scores, int(u))))
                n = min(int(n or 0), len(pending), len(steps))
                tail = [pending.pop() for _ in range(n)][::-1]
                pending.extend([step for pair in zip(tail, steps) for step in pair] + steps[n:])
        for step in pending:
            step()

    for name in _FIRST_COPIES.split():
        for copy in io[name]:
            copy.start()
    for ref in (*acc, y_sel):
        ref[...] = jnp.zeros_like(ref)
    actions = {"!" + name: functools.partial(wait, name) for name in io}
    actions.update({name: functools.partial(prepare_weight, name, 0, True) for name in weights})
    actions.update({f"c{u}": functools.partial(prepare_c, u) for u in range(U)})
    actions.update(x=prepare_x, route=route)
    run(_FIRST_PROJECTIONS, actions)
    for copy in head_copies(0):
        copy.start()

    def head(h, carry):
        attention()
        for copy in head_copies(h):
            copy.wait()

        @pl.when(h + 1 < H)
        def _():
            actions = {name: functools.partial(prepare_weight, name, h + 1, False) for name in weights}
            run(_PROJECTIONS, dict(actions, wo=prepare_wo, **ffn_steps(h)))
            for copy in head_copies(h + 1):
                copy.start()
        return carry

    lax.fori_loop(0, H, head, None)

    prepare_wo()
    add_routed_update()
    for u in range(U):
        attended = _combine(*(acc[u][j] + out_product(u, j) for j in range(7)))
        keep = 1.0 - jnp.concatenate([gate[2 * u:2 * u + 1], gate[2 * u + 1:2 * u + 2]], axis=1)
        for f in range(2):
            rows = slice(f * mh, (f + 1) * mh)
            mixed = (keep * xT[rows, block(u)].astype(_F32)
                     + jnp.concatenate(attended[2 * f:2 * f + 2], axis=1))
            outT[rows, block(u)] = mixed.astype(outT.dtype)
        io[f"out{u}"][0].start()
    for u in range(U):
        wait(f"out{u}")


@jax.jit
def pallas_gated_mix__compressed_kv_cla__moe_arch_mod__prompt_kernel(
    A_x: jax.Array,
    A_c_kv: jax.Array,
    A_w_q: jax.Array,
    A_w_uk: jax.Array,
    A_w_uv: jax.Array,
    A_w_o: jax.Array,
    B_x: jax.Array,
    B_w_r: jax.Array,
    B_w_gate: jax.Array,
    B_w_up: jax.Array,
    B_w_down: jax.Array,
    gate_w: jax.Array,
):
    del B_x
    _, S, M = A_x.shape
    Dc, H, D = A_w_uk.shape
    U = S // (2 * _T)
    assert D == 2 * _T and U == 8 and A_c_kv.shape[1] == S and B_w_gate.shape[1] // _T < H
    vmem = pltpu.VMEM
    tiles = lambda n: [vmem((n, _T, _T), _BF16)] * U
    hbm = pl.BlockSpec(memory_space=pl.ANY)
    outT = pl.pallas_call(
        _kernel,
        in_specs=[hbm] * 11,
        out_specs=hbm,
        out_shape=jax.ShapeDtypeStruct((M, S), A_x.dtype),
        scratch_shapes=[
            vmem((M, S), _BF16), vmem((S, Dc), _BF16), vmem((M,), _BF16), vmem((M,), _BF16),
            [vmem((n, D), _U32) for n in (M, Dc, Dc)],
            [vmem((2, n, _T), _U32) for n in (M, Dc, Dc)],
            vmem((M, D), _BF16), [vmem((M, _T), _BF16)] * 3, vmem((M, S), _BF16),
            pltpu.SemaphoreType.DMA((6 + 2 * U,)), pltpu.SemaphoreType.DMA((10,)),
            vmem((7, U, M // 2, _T), _BF16), [vmem((7, Dc // 2 // _T, _T, _T), _BF16)] * U,
            vmem((7, pl.cdiv(M // 2, _T), _T, _T), _BF16), vmem((7, Dc // 2, _T), _BF16),
            vmem((7, Dc // 2 // _T, _T, _T), _BF16), vmem((7, M // 2, _T), _BF16),
            tiles(9), tiles(9), tiles(9), tiles(7), [vmem((7, M // 2, _T), _F32)] * U,
            vmem((2 * U, _T), _F32), vmem((2 * U, _T), _F32),
            vmem((_ROWS, M), _BF16), vmem((_ROWS, M), _F32), vmem((_CAPACITY, _T), _F32),
            pltpu.SMEM((_CAPACITY,), jnp.int32),
        ],
        compiler_params=pltpu.CompilerParams(
            vmem_limit_bytes=100 * 2**20, disable_bounds_checks=True),
        name="gm_kernel",
    )(A_x[0].T, A_c_kv[0], A_w_q, A_w_uk, A_w_uv, A_w_o.transpose(0, 2, 1),
      B_w_r, B_w_gate, B_w_up, B_w_down.T, gate_w)
    return outT.T[None]
```

```python
import functools
import math

import jax
import jax.numpy as jnp
from jax import lax
import jax.experimental.pallas as pl
import jax.experimental.pallas.tpu as pltpu

_NN = (((1,), (0,)), ((), ()))
_NT = (((1,), (1,)), ((), ()))
_F32 = jnp.float32
_BF16 = jnp.bfloat16
_U32 = jnp.uint32
_LOG2E = math.log2(math.e)
_T = 128
_ROWS = 16
_CAPACITY = 2

_FIRST_COPIES = "wv c0 wk c1 c2 c3 c4 c5 c6 c7 vec wq x"
_FIRST_PROJECTIONS = (
    "!wv wv !c0 c0 V0 !wk wk K0 !c1 c1 K1 V1 !c2 !c3 c2 c3 K2-4 V2-4"
    " !c4 !c5 !c6 c4 c5 c6 V4-6 V6 K4-6 !c7 !vec !wq !x c7 wq x;"
    " K6 | R0-8; K7 | Q0 Q1 Q2 Q3; route; V7 | Q4 Q5 Q6 Q7")
_PROJECTIONS = (
    "wo wk wq wv O0 O1 O2;"
    " K0-2 K2-8 V0-2 V2-4 V4-6 V6-8 | O3 up Q0-2 down Q2-4 O4 Q4-6 Q6-8 O5; O6 O7")
_ATTENTION = (
    "D0@8 S1 D3@0 D1@6 S2 D2@2 -0 C1@2 D4@8 S3 -1 C2@8 S4 C0@0 D5@4"
    " -3 S5 C3@0 D6@4 -3 C4@2 D7@2 S6 -0 S7 C5@2 -1 C7@12 C6@0")
_SCORE_GROUPS = ("1356 024", "024 1356", "024 1356", "1356 024",
                 "1356 024", "1356 024", "2456 013", "1356 024")
_REVERSED_MAX = ("", "b", "a", "ab", "a", "b", "", "")
_SUM_ROWS = (64, 16, 1024, 1024, 256, 32, 256, 16)
_PV_ORDER = ("41063527", "41520367", "14325760", "14036752",
             "41073265", "41076523", "41023576", "14275063")
_DIAGONAL_ORDER = ("302145", "210435", "021534", "142530", "210354", "530421", "102354", "130245")


def _dot(a, b, dims=_NN):
    return lax.dot_general(a, b, dims, preferred_element_type=_F32)


def _lhs_operands(a11, a12, a21, a22):
    return (a11 + a22, a21 + a22, a11, a22, a11 + a12, a21 - a11, a12 - a22)


def _rhs_operands(b11, b12, b21, b22):
    return (b11 + b22, b11, b12 - b22, b21 - b11, b22, b11 + b12, b21 + b22)


def _combine(m1, m2, m3, m4, m5, m6, m7):
    return m1 + m4 - m5 + m7, m3 + m5, m2 + m4, m1 - m2 + m3 + m6


def _slab(ref, *lead):
    return pltpu.bitcast(ref.bitcast(_U32)[(*lead, slice(None), slice(None))], _BF16)


def _cat(xs, axis):
    return xs[0] if len(xs) == 1 else jnp.concatenate(xs, axis=axis)


def _fold(op, x, rows):
    return [functools.reduce(op, [x[r:r + 8] for r in range(lo, min(lo + rows, x.shape[0]), 8)])
            for lo in range(0, x.shape[0], rows)]


def _interleave(streams):
    keyed = []
    for steps in streams:
        total, done = sum(cost for cost, _ in steps), 0
        for cost, step in steps:
            keyed.append(((done + cost / 2) / total, len(keyed), step))
            done += cost
    return [step for _, _, step in sorted(keyed, key=lambda item: item[:2])]


def _kernel(
    xT_hbm, c_hbm, wq_hbm, wuk_hbm, wuv_hbm, woT_hbm, wr_hbm, wg_hbm, wu_hbm, wdT_hbm, gw_hbm,
    outT_hbm,
    xT, c, wr, gw, first_words, next_words, woT, ffn_w, outT, io_sems, head_sems,
    x_ops, c_ops, wq_ops, wk_ops, wv_ops, wo_ops, q_ops, k_ops, v_ops, ctx_ops, acc,
    gate, score, x_sel, y_sel, y_scale, routed,
):
    M, S = xT.shape
    Dc, H, D = wuk_hbm.shape
    U = S // (2 * _T)
    n_chunks = wg_hbm.shape[1] // _T
    mh, kt = M // 2, Dc // 2 // _T
    block = lambda u: slice(2 * u * _T, 2 * (u + 1) * _T)
    tile = lambda t: slice(t * _T, (t + 1) * _T)
    weights = {"wq": (0, wq_hbm, wq_ops), "wk": (1, wuk_hbm, wk_ops), "wv": (2, wuv_hbm, wv_ops)}

    io = {name: [(src.bitcast(_U32).at[:, 0, :], first_words[i])]
          for name, (i, src, _) in weights.items()}
    io["x"] = [(xT_hbm, xT)]
    io["vec"] = [(wr_hbm, wr), (gw_hbm, gw)]
    for u in range(U):
        io[f"c{u}"] = [(c_hbm.at[block(u)], c.at[block(u)])]
        io[f"out{u}"] = [(outT.at[:, block(u)], outT_hbm.at[:, block(u)])]
    slots = iter(range(io_sems.shape[0]))
    io = {name: [pltpu.make_async_copy(src, dst, io_sems.at[next(slots)]) for src, dst in pairs]
          for name, pairs in io.items()}

    def wait(name):
        for copy in io[name]:
            copy.wait()

    def head_copies(h):
        pair = jnp.minimum(h + 1, H - 1) // 2
        chunk = pl.ds(pl.multiple_of(jnp.minimum(h, n_chunks - 1) * _T, _T), _T)
        pairs = [(woT_hbm.at[h], woT)]
        pairs += [(src.bitcast(_U32).at[:, pair, tile(n)], next_words[i].at[n])
                  for i, src, _ in weights.values() for n in range(2)]
        pairs += [(src.at[:, chunk], dst) for src, dst in zip((wg_hbm, wu_hbm, wdT_hbm), ffn_w)]
        return [pltpu.make_async_copy(src, dst, head_sems.at[i]) for i, (src, dst) in enumerate(pairs)]

    def prepare_weight(name, head, first):
        i, src, dst = weights[name]
        transposed = name != "wk"
        shift = jnp.asarray(16 * (1 - head % 2)).astype(_U32)
        half = src.shape[0] // 2
        step = _T if transposed else _ROWS
        for r in range(0, half, step):
            n_rows = min(step, half - r)
            quads = []
            for f in range(2):
                rows = slice(f * half + r, f * half + r + n_rows)
                for n in range(2):
                    words = first_words[i][rows, tile(n)] if first else next_words[i][n, rows]
                    words = words.T if transposed else words
                    quads.append(pltpu.bitcast((words << shift) & _U32(0xFFFF0000), _F32))
            for j, op in enumerate(_rhs_operands(*quads)):
                if not transposed:
                    dst[j, r:r + n_rows] = op.astype(_BF16)
                    continue
                if n_rows < _T:
                    op = jnp.concatenate([op, jnp.zeros((_T, _T - n_rows), _F32)], axis=1)
                dst[j, r // _T] = op.astype(_BF16)

    def prepare_wo():
        for r in range(0, mh, _ROWS):
            top, bottom = (woT[f * mh + r:f * mh + r + _ROWS].astype(_F32) for f in range(2))
            for j, op in enumerate(_lhs_operands(top[:, :_T], top[:, _T:], bottom[:, :_T], bottom[:, _T:])):
                wo_ops[j, r:r + _ROWS] = op.astype(_BF16)

    def prepare_c(u):
        for r in range(0, _T, _ROWS):
            ca, cb = (c[(2 * u + f) * _T + r:(2 * u + f) * _T + r + _ROWS].astype(_F32) for f in range(2))
            ops = _lhs_operands(ca[:, :Dc // 2], ca[:, Dc // 2:], cb[:, :Dc // 2], cb[:, Dc // 2:])
            for j, op in enumerate(ops):
                for t in range(kt):
                    c_ops[u][j, t, r:r + _ROWS] = op[:, tile(t)].astype(_BF16)

    def prepare_x():
        for u in range(U):
            for r in range(0, mh, _ROWS):
                x0, x1 = (xT[f * mh + r:f * mh + r + _ROWS, block(u)].astype(_F32) for f in range(2))
                for j, op in enumerate(_lhs_operands(x0[:, :_T], x1[:, :_T], x0[:, _T:], x1[:, _T:])):
                    x_ops[j, u, r:r + _ROWS] = op.astype(_BF16)

    lane = lax.broadcasted_iota(jnp.int32, (1, _T), 1)
    tile_of = lambda token: pl.ds(pl.multiple_of(token // _T * _T, _T), _T)

    def score_tokens(u0, u1):
        def step(t):
            row = lax.broadcasted_iota(jnp.int32, (_ROWS, M), 0)
            vectors = jnp.where(row == 0, *(v[...].astype(_F32).reshape(1, M) for v in (wr, gw)))
            dots = _dot(vectors.astype(_BF16), xT[:, tile(t)])
            score[t:t + 1] = dots[0:1].astype(xT.dtype).astype(_F32)
            gate[t:t + 1] = jax.nn.sigmoid(dots[1:2])
        return [(1, functools.partial(step, t)) for t in range(2 * u0, 2 * u1)]

    def route():
        r = score[...]
        r = jnp.where(r == r, r, -jnp.inf)
        token = (lax.broadcasted_iota(jnp.int32, r.shape, 0) * _T
                 + lax.broadcasted_iota(jnp.int32, r.shape, 1)).astype(_F32)
        free = token >= 0
        slot = lax.broadcasted_iota(jnp.int32, (_ROWS, _T), 0)
        picked = []
        for n in range(_CAPACITY):
            best = jnp.max(jnp.where(free, r, -jnp.inf), keepdims=True)
            choice = jnp.min(jnp.where(free & (r == best), token, S - 1.0))
            free = free & (token != choice)
            index = choice.astype(jnp.int32)
            routed[n] = index
            y_scale[n:n + 1] = jnp.broadcast_to(jax.nn.sigmoid(best), (1, _T))
            onehot = jnp.where((slot == n) & (lane == index % _T), 1.0, 0.0)
            picked.append(_dot(onehot.astype(_BF16), xT[:, tile_of(index)], _NT))
        x_sel[...] = functools.reduce(jnp.add, picked).astype(_BF16)

    def ffn_steps(chunk):
        hidden = []

        def up():
            g, u = (_dot(x_sel[...], _slab(w)) for w in ffn_w[:2])
            hidden.append(jnp.where(chunk < n_chunks, g * jax.nn.sigmoid(g) * u, 0.0))

        def down():
            y_sel[...] += _dot(hidden.pop().astype(_BF16), _slab(ffn_w[2]), _NT)
        return {"up": up, "down": down}

    def add_routed_update():
        yT = jnp.concatenate([y_sel[...], jnp.zeros((_T - _ROWS, M), _F32)], axis=0).T
        for n in range(_CAPACITY):
            index = routed[n]
            x = xT[:, tile_of(index)].astype(_F32)
            y = yT[:, n:n + 1] * y_scale[n:n + 1]
            xT[:, tile_of(index)] = jnp.where(lane == index % _T, x + y, x).astype(xT.dtype)

    def seven_products(cost, product, finish):
        m = []

        def step(j):
            m.append(product(j))
            if j == 6:
                finish(*_combine(*m))
        return [(cost, functools.partial(step, j)) for j in range(7)]

    def c_operand(j, u0, u1):
        return _cat([_cat([_slab(c_ops[u], j, t) for t in range(kt)], 1) for u in range(u0, u1)], 0)

    def project_k(u0, u1):
        def finish(ka0, ka1, kb0, kb1):
            for j, op in enumerate(_lhs_operands(kb0, kb1, ka0, ka1) + (kb1, ka0)):
                for u in range(u0, u1):
                    k_ops[u][j] = op[tile(u - u0)].astype(_BF16)
        product = lambda j: _dot(c_operand(j, u0, u1), _slab(wk_ops, j))
        return seven_products(kt * (u1 - u0) * _T, product, finish)

    def project_q(u0, u1):
        def product(j):
            w = _cat([_slab(wq_ops, j, t) for t in range(wq_ops.shape[1])], 1)[:, :mh]
            return _dot(w, _cat([_slab(x_ops, j, u) for u in range(u0, u1)], 1))

        def finish(*q):
            qa0, qa1, qb0, qb1 = (part * (D ** -0.5 * _LOG2E) for part in q)
            for j, op in enumerate(_rhs_operands(qa0, qb0, qa1, qb1) + (qb0, qa1)):
                for u in range(u0, u1):
                    q_ops[u][j] = op[:, tile(u - u0)].astype(_BF16)
        return seven_products(2 * (u1 - u0) * _T, product, finish)

    def project_v(u0, u1):
        def product(j):
            return _dot(_cat([_slab(wv_ops, j, t) for t in range(kt)], 1), c_operand(j, u0, u1), _NT)

        def finish(va0, va1, vb0, vb1):
            for j, op in enumerate(_lhs_operands(vb0, va0, vb1, va1) + (va0, vb1)):
                for u in range(u0, u1):
                    v_ops[u][j] = op[:, tile(u - u0)].astype(_BF16)
        return seven_products(kt * (u1 - u0) * _T, product, finish)

    out_product = lambda u, j: _dot(_slab(wo_ops, j), _slab(ctx_ops[u], j))

    def project_out(u, _):
        def step(j):
            acc[u][j] += out_product(u, j)
        return [(mh, functools.partial(step, j)) for j in range(7)]

    def run(program, actions):
        ranged = {"K": project_k, "Q": project_q, "V": project_v, "O": project_out, "R": score_tokens}

        def steps(word):
            if word in actions:
                return [(1e-3, actions[word])]
            lo, _, hi = word[1:].partition("-")
            return ranged[word[0]](int(lo), int(hi) if hi else int(lo) + 1)
        for phase in program.split(";"):
            for step in _interleave([[s for word in part.split() for s in steps(word)]
                                     for part in phase.split("|")]):
                step()

    def causal(s):
        key = lax.broadcasted_iota(jnp.int32, (_T, _T), 0)
        query = lax.broadcasted_iota(jnp.int32, (_T, _T), 1)
        return jnp.where(key <= query, s, -1e9 * _LOG2E)

    def weighted_values(u, scores):
        p, total, m, balance = {}, {}, {}, []

        def softmax():
            s = scores()
            exponent = {}
            for half in "ab":
                names = [name for name in s if name[1] == half]
                peaks = [peak for name in (names[::-1] if half in _REVERSED_MAX[u] else names)
                         for peak in _fold(jnp.maximum, s[name], _T)]
                top = jnp.max(functools.reduce(jnp.maximum, peaks), axis=0, keepdims=True)
                p.update({name: jnp.exp2(s[name] - top) for name in names})
                sums = [x for name in names for x in _fold(jnp.add, p[name], _SUM_ROWS[u])]
                total[half] = jnp.sum(functools.reduce(jnp.add, sums), axis=0, keepdims=True)
                estimate = functools.reduce(jnp.add, [jnp.exp2(peak - top) for peak in peaks])
                estimate = jnp.sum(estimate, axis=0, keepdims=True)
                exponent[half] = pltpu.bitcast(estimate, jnp.int32) >> 23
            balance.append(pltpu.bitcast((exponent["a"] - exponent["b"] + 127) << 23, _F32))

        def step(into, v, t, probs):
            if not p:
                softmax()
            product = _dot(_slab(v_ops[t], v), probs(lambda name: p[name][tile(t)]).astype(_BF16))
            m[into] = m[into] + product if into in m else product

        def finish():
            c0a, c0b, c1a, c1b = m["0a"], m["0b"], m["1a"], m["1b"]
            fa, fb = (gate[2 * u + i:2 * u + i + 1] / total[half] for i, half in enumerate("ab"))
            f1b = fb
            if u:
                w = balance[0]
                c0a, c0b = c0a + (m[3] - w * m[4]) + m[0], c0b + m[2] + m[4]
                c1a, c1b = c1a + m[1] + m[3], w * (c1b + m[2]) + (m[5] - m[1]) + m[0]
                f1b = fb / w
            for j, op in enumerate(_rhs_operands(c0a * fa, c0b * fb, c1a * fa, c1b * f1b)):
                ctx_ops[u][j] = op.astype(_BF16)

        def rhs(j):
            def operand(get):
                w = (lambda x: balance[0] * x) if j in (0, 5, 6) else (lambda x: x)
                return _rhs_operands(get("ba"), w(get("bb")), get("aa"), w(get("ab")))[j]
            return operand

        diagonal = [("0a", 7, "aa"), ("0b", 7, "ab"), ("0b", 2, "bb"),
                    ("1a", 3, "aa"), ("1b", 3, "ab"), ("1b", 8, "bb")]
        steps = []
        for j in map(int, _PV_ORDER[u]):
            if j == 7:
                steps += [functools.partial(step, into, v, u, lambda get, name=name: get(name))
                          for into, v, name in (diagonal[int(i)] for i in _DIAGONAL_ORDER[u])]
            else:
                into = "0a" if j == 6 else j
                steps += [functools.partial(step, into, j, t, rhs(j)) for t in range(u)]
        last = steps.pop()
        return steps + [lambda: (last(), finish())]

    def attention():
        load, pending = [0] * 4, []

        def issue(tiles, step):
            load[load.index(min(load))] += tiles
            return step()

        def level():
            while pending and min(load) < max(load):
                issue(1, pending.pop(0))

        below, diagonal = {}, {}

        def diagonal_scores(u):
            def product(name, k, q):
                m = _dot(_slab(k_ops[u], k), _slab(q_ops[u], q))
                diagonal[u, name] = diagonal[u, name] + m if (u, name) in diagonal else m
            return [functools.partial(product, *spec) for spec in (
                ("aa", 8, 1), ("aa", 3, 8), ("ab", 8, 7), ("ab", 3, 4), ("bb", 2, 7), ("bb", 7, 4))]

        def scores(u):
            def product(j):
                keys = lambda: _cat([_slab(k_ops[t], j) for t in range(u)], 0)
                return issue(u, lambda: _dot(keys(), _slab(q_ops[u], j)))
            m = {}
            for group in _SCORE_GROUPS[u].split():
                m.update({j: product(j) for j in map(int, group)})
                level()
            m1, m2, m3, m4, m5, m6, m7 = (m[j] for j in range(7))
            if "024" in _SCORE_GROUPS[u]:
                below[u] = dict(aa=m2 + m4, ba=(m4 + m7) + (m1 - m5), bb=m3 + m5, ab=(m6 - m2) + (m1 + m3))
            else:
                below[u] = dict(aa=m2 + m4, ba=(m7 - m5) + (m1 + m4), bb=m3 + m5, ab=(m6 + m3) + (m1 - m2))

        def all_scores(u):
            s = dict(aa=causal(diagonal[u, "aa"]), bb=causal(diagonal[u, "bb"]), ab=diagonal[u, "ab"])
            if u:
                s = {name: _cat([part] + ([s[name]] if name in s else []), 0)
                     for name, part in below[u].items()}
            return s

        for word in _ATTENTION.split():
            if word[0] == "S":
                scores(int(word[1:]))
            elif word[0] == "-":
                while len(pending) >= 4 + int(word[1:]):
                    for _ in range(4):
                        issue(1, pending.pop(0))
            else:
                u, _, n = word[1:].partition("@")
                steps = (diagonal_scores(int(u)) if word[0] == "D"
                         else weighted_values(int(u), functools.partial(all_scores, int(u))))
                n = min(int(n or 0), len(pending), len(steps))
                tail = [pending.pop() for _ in range(n)][::-1]
                pending.extend([step for pair in zip(tail, steps) for step in pair] + steps[n:])
        for step in pending:
            step()

    for name in _FIRST_COPIES.split():
        for copy in io[name]:
            copy.start()
    for ref in (*acc, y_sel):
        ref[...] = jnp.zeros_like(ref)
    actions = {"!" + name: functools.partial(wait, name) for name in io}
    actions.update({name: functools.partial(prepare_weight, name, 0, True) for name in weights})
    actions.update({f"c{u}": functools.partial(prepare_c, u) for u in range(U)})
    actions.update(x=prepare_x, route=route)
    run(_FIRST_PROJECTIONS, actions)
    for copy in head_copies(0):
        copy.start()

    def head(h, carry):
        attention()
        for copy in head_copies(h):
            copy.wait()

        @pl.when(h + 1 < H)
        def _():
            actions = {name: functools.partial(prepare_weight, name, h + 1, False) for name in weights}
            run(_PROJECTIONS, dict(actions, wo=prepare_wo, **ffn_steps(h)))
            for copy in head_copies(h + 1):
                copy.start()
        return carry

    lax.fori_loop(0, H, head, None)

    prepare_wo()
    add_routed_update()
    for u in range(U):
        attended = _combine(*(acc[u][j] + out_product(u, j) for j in range(7)))
        keep = 1.0 - jnp.concatenate([gate[2 * u:2 * u + 1], gate[2 * u + 1:2 * u + 2]], axis=1)
        for f in range(2):
            rows = slice(f * mh, (f + 1) * mh)
            mixed = (keep * xT[rows, block(u)].astype(_F32)
                     + jnp.concatenate(attended[2 * f:2 * f + 2], axis=1))
            outT[rows, block(u)] = mixed.astype(outT.dtype)
        io[f"out{u}"][0].start()
    for u in range(U):
        wait(f"out{u}")


@jax.jit
def pallas_gated_mix__compressed_kv_cla__moe_arch_mod__prompt_kernel(
    A_x: jax.Array,
    A_c_kv: jax.Array,
    A_w_q: jax.Array,
    A_w_uk: jax.Array,
    A_w_uv: jax.Array,
    A_w_o: jax.Array,
    B_x: jax.Array,
    B_w_r: jax.Array,
    B_w_gate: jax.Array,
    B_w_up: jax.Array,
    B_w_down: jax.Array,
    gate_w: jax.Array,
):
    del B_x
    _, S, M = A_x.shape
    Dc, H, D = A_w_uk.shape
    U = S // (2 * _T)
    assert D == 2 * _T and U == 8 and A_c_kv.shape[1] == S and B_w_gate.shape[1] // _T < H
    vmem = pltpu.VMEM
    tiles = lambda n: [vmem((n, _T, _T), _BF16)] * U
    hbm = pl.BlockSpec(memory_space=pl.ANY)
    outT = pl.pallas_call(
        _kernel,
        in_specs=[hbm] * 11,
        out_specs=hbm,
        out_shape=jax.ShapeDtypeStruct((M, S), A_x.dtype),
        scratch_shapes=[
            vmem((M, S), _BF16), vmem((S, Dc), _BF16), vmem((M,), _BF16), vmem((M,), _BF16),
            [vmem((n, D), _U32) for n in (M, Dc, Dc)],
            [vmem((2, n, _T), _U32) for n in (M, Dc, Dc)],
            vmem((M, D), _BF16), [vmem((M, _T), _BF16)] * 3, vmem((M, S), _BF16),
            pltpu.SemaphoreType.DMA((6 + 2 * U,)), pltpu.SemaphoreType.DMA((10,)),
            vmem((7, U, M // 2, _T), _BF16), [vmem((7, Dc // 2 // _T, _T, _T), _BF16)] * U,
            vmem((7, pl.cdiv(M // 2, _T), _T, _T), _BF16), vmem((7, Dc // 2, _T), _BF16),
            vmem((7, Dc // 2 // _T, _T, _T), _BF16), vmem((7, M // 2, _T), _BF16),
            tiles(9), tiles(9), tiles(9), tiles(7), [vmem((7, M // 2, _T), _F32)] * U,
            vmem((2 * U, _T), _F32), vmem((2 * U, _T), _F32),
            vmem((_ROWS, M), _BF16), vmem((_ROWS, M), _F32), vmem((_CAPACITY, _T), _F32),
            pltpu.SMEM((_CAPACITY,), jnp.int32),
        ],
        compiler_params=pltpu.CompilerParams(
            vmem_limit_bytes=100 * 2**20, disable_bounds_checks=True),
        name="gm_kernel",
    )(A_x.reshape(S, M).T, A_c_kv.reshape(S, Dc), A_w_q, A_w_uk, A_w_uv, A_w_o.transpose(0, 2, 1),
      B_w_r, B_w_gate, B_w_up, B_w_down.T, gate_w)
    return outT.T.reshape(A_x.shape)
```

```python
import functools
import math

import jax
import jax.numpy as jnp
from jax import lax
import jax.experimental.pallas as pl
import jax.experimental.pallas.tpu as pltpu

_NN = (((1,), (0,)), ((), ()))
_NT = (((1,), (1,)), ((), ()))
_F32 = jnp.float32
_BF16 = jnp.bfloat16
_U32 = jnp.uint32
_LOG2E = math.log2(math.e)
_T = 128
_ROWS = 16
_CAPACITY = 2

_FIRST_COPIES = "wv c0 wk c1 c2 c3 c4 c5 c6 c7 vec wq x"
_FIRST_PROJECTIONS = (
    "!wv wv !c0 c0 V0 !wk wk K0 !c1 c1 K1 V1 !c2 !c3 c2 c3 K2-4 V2-4"
    " !c4 !c5 !c6 c4 c5 c6 V4-6 V6 K4-6 !c7 !vec !wq !x c7 wq x;"
    " K6 | R0-8; K7 | Q0 Q1 Q2 Q3; route; V7 | Q4 Q5 Q6 Q7")
_PROJECTIONS = (
    "wo wk wq wv O0 O1 O2;"
    " K0-2 K2-8 V0-2 V2-4 V4-6 V6-8 | up O3 Q0 Q1 down Q2 Q3 Q4 O4 Q5 Q6 Q7; O5 O6 O7")
_ATTENTION = (
    "S1 D0@4 D3@0 D1@6 S2 D2@2 -0 C1@2 D4@8 S3 -1 C2@2 S4 C0@0 D5@0"
    " -3 S5 C3@6 D6@0 -5 C4@2 D7@2 S6 -3 S7 -3 C5@8 C7@2 C6@0")
_SCORE_GROUPS = ("1356 024", "024 1356", "024 1356", "1356 024",
                 "1356 024", "1356 024", "2456 013", "1356 024")
_REVERSED_MAX = ("", "b", "a", "ab", "a", "", "", "")
_SUM_ROWS = (64, 16, 16, 1024, 256, 32, 256, 16)
_PV_ORDER = ("41063527", "41520367", "14325760", "14036752",
             "41073265", "41076523", "41023576", "14275063")
_DIAGONAL_ORDER = ("302145", "253401", "314502", "432150", "035421", "435120", "102354", "130245")


def _dot(a, b, dims=_NN):
    return lax.dot_general(a, b, dims, preferred_element_type=_F32)


def _lhs_operands(a11, a12, a21, a22):
    return (a11 + a22, a21 + a22, a11, a22, a11 + a12, a21 - a11, a12 - a22)


def _rhs_operands(b11, b12, b21, b22):
    return (b11 + b22, b11, b12 - b22, b21 - b11, b22, b11 + b12, b21 + b22)


def _combine(m1, m2, m3, m4, m5, m6, m7):
    return m1 + m4 - m5 + m7, m3 + m5, m2 + m4, m1 - m2 + m3 + m6


def _slab(ref, *lead):
    return pltpu.bitcast(ref.bitcast(_U32)[(*lead, slice(None), slice(None))], _BF16)


def _cat(xs, axis):
    return xs[0] if len(xs) == 1 else jnp.concatenate(xs, axis=axis)


def _fold(op, x, rows):
    return [functools.reduce(op, [x[r:r + 8] for r in range(lo, min(lo + rows, x.shape[0]), 8)])
            for lo in range(0, x.shape[0], rows)]


def _interleave(streams):
    keyed = []
    for steps in streams:
        total, done = sum(cost for cost, _ in steps), 0
        for cost, step in steps:
            keyed.append(((done + cost / 2) / total, len(keyed), step))
            done += cost
    return [step for _, _, step in sorted(keyed, key=lambda item: item[:2])]


def _kernel(
    xT_hbm, c_hbm, wq_hbm, wuk_hbm, wuv_hbm, woT_hbm, wr_hbm, wg_hbm, wu_hbm, wdT_hbm, gw_hbm,
    outT_hbm,
    xT, c, wr, gw, first_words, next_words, woT, ffn_w, outT, io_sems, head_sems,
    x_ops, c_ops, wq_ops, wk_ops, wv_ops, wo_ops, q_ops, k_ops, v_ops, ctx_ops, acc,
    gate, score, x_sel, y_sel, y_scale, routed,
):
    M, S = xT.shape
    Dc, H, D = wuk_hbm.shape
    U = S // (2 * _T)
    n_chunks = wg_hbm.shape[1] // _T
    mh, kt = M // 2, Dc // 2 // _T
    block = lambda u: slice(2 * u * _T, 2 * (u + 1) * _T)
    tile = lambda t: slice(t * _T, (t + 1) * _T)
    weights = {"wq": (0, wq_hbm, wq_ops), "wk": (1, wuk_hbm, wk_ops), "wv": (2, wuv_hbm, wv_ops)}

    io = {name: [(src.bitcast(_U32).at[:, 0, :], first_words[i])]
          for name, (i, src, _) in weights.items()}
    io["x"] = [(xT_hbm, xT)]
    io["vec"] = [(wr_hbm, wr), (gw_hbm, gw)]
    for u in range(U):
        io[f"c{u}"] = [(c_hbm.at[block(u)], c.at[block(u)])]
        io[f"out{u}"] = [(outT.at[:, block(u)], outT_hbm.at[:, block(u)])]
    slots = iter(range(io_sems.shape[0]))
    io = {name: [pltpu.make_async_copy(src, dst, io_sems.at[next(slots)]) for src, dst in pairs]
          for name, pairs in io.items()}

    def wait(name):
        for copy in io[name]:
            copy.wait()

    def head_copies(h):
        pair = jnp.minimum(h + 1, H - 1) // 2
        chunk = pl.ds(pl.multiple_of(jnp.minimum(h, n_chunks - 1) * _T, _T), _T)
        pairs = [(woT_hbm.at[h], woT)]
        pairs += [(src.bitcast(_U32).at[:, pair, tile(n)], next_words[i].at[n])
                  for i, src, _ in weights.values() for n in range(2)]
        pairs += [(src.at[:, chunk], dst) for src, dst in zip((wg_hbm, wu_hbm, wdT_hbm), ffn_w)]
        return [pltpu.make_async_copy(src, dst, head_sems.at[i]) for i, (src, dst) in enumerate(pairs)]

    def prepare_weight(name, head, first):
        i, src, dst = weights[name]
        transposed = name != "wk"
        shift = jnp.asarray(16 * (1 - head % 2)).astype(_U32)

        def load(lo, n_rows, n, transposed):
            rows = slice(lo, lo + n_rows)
            words = first_words[i][rows, tile(n)] if first else next_words[i][n, rows]
            words = words.T if transposed else words
            return pltpu.bitcast((words << shift) & _U32(0xFFFF0000), _F32)

        half = _T if name == "wq" else src.shape[0] // 2
        step = _T if transposed else _ROWS
        for r in range(0, half, step):
            quads = [load(f * half + r, step, n, transposed) for f in range(2) for n in range(2)]
            for j, op in enumerate(_rhs_operands(*quads)):
                dst[j, r:r + step] = op.astype(_BF16)
        if name == "wq":
            (w10, w11), (w20, w21), (w30, w31) = (
                [load(2 * _T + g * _T // 2, _T // 2, n, False) for n in range(2)] for g in range(3))
            for j, parts in enumerate(((w10, w20 - w21), (w11, w31 - w30), (w21, w30))):
                dst[7 + j] = jnp.concatenate(parts, axis=0).T.astype(_BF16)

    def prepare_wo():
        for r in range(0, mh, _ROWS):
            top, bottom = (woT[f * mh + r:f * mh + r + _ROWS].astype(_F32) for f in range(2))
            for j, op in enumerate(_lhs_operands(top[:, :_T], top[:, _T:], bottom[:, :_T], bottom[:, _T:])):
                wo_ops[j, r:r + _ROWS] = op.astype(_BF16)

    def prepare_c(u):
        for r in range(0, _T, _ROWS):
            ca, cb = (c[(2 * u + f) * _T + r:(2 * u + f) * _T + r + _ROWS].astype(_F32) for f in range(2))
            ops = _lhs_operands(ca[:, :Dc // 2], ca[:, Dc // 2:], cb[:, :Dc // 2], cb[:, Dc // 2:])
            for j, op in enumerate(ops):
                for t in range(kt):
                    c_ops[u][j, t, r:r + _ROWS] = op[:, tile(t)].astype(_BF16)

    def prepare_x():
        for u in range(U):
            for r in range(0, _T, _ROWS):
                x0, x1 = (xT[f * _T + r:f * _T + r + _ROWS, block(u)].astype(_F32) for f in range(2))
                for j, op in enumerate(_lhs_operands(x0[:, :_T], x1[:, :_T], x0[:, _T:], x1[:, _T:])):
                    x_ops[u][j, r:r + _ROWS] = op.astype(_BF16)

    lane = lax.broadcasted_iota(jnp.int32, (1, _T), 1)
    tile_of = lambda token: pl.ds(pl.multiple_of(token // _T * _T, _T), _T)

    def score_tokens(u0, u1):
        def step(t):
            row = lax.broadcasted_iota(jnp.int32, (_ROWS, M), 0)
            vectors = jnp.where(row == 0, *(v[...].astype(_F32).reshape(1, M) for v in (wr, gw)))
            dots = _dot(vectors.astype(_BF16), xT[:, tile(t)])
            score[t:t + 1] = dots[0:1].astype(xT.dtype).astype(_F32)
            gate[t:t + 1] = jax.nn.sigmoid(dots[1:2])
        return [(1, functools.partial(step, t)) for t in range(2 * u0, 2 * u1)]

    def route():
        r = score[...]
        r = jnp.where(r == r, r, -jnp.inf)
        token = (lax.broadcasted_iota(jnp.int32, r.shape, 0) * _T
                 + lax.broadcasted_iota(jnp.int32, r.shape, 1)).astype(_F32)
        free = token >= 0
        slot = lax.broadcasted_iota(jnp.int32, (_ROWS, _T), 0)
        picked = []
        for n in range(_CAPACITY):
            best = jnp.max(jnp.where(free, r, -jnp.inf), keepdims=True)
            choice = jnp.min(jnp.where(free & (r == best), token, S - 1.0))
            free = free & (token != choice)
            index = choice.astype(jnp.int32)
            routed[n] = index
            y_scale[n:n + 1] = jnp.broadcast_to(jax.nn.sigmoid(best), (1, _T))
            onehot = jnp.where((slot == n) & (lane == index % _T), 1.0, 0.0)
            picked.append(_dot(onehot.astype(_BF16), xT[:, tile_of(index)], _NT))
        x_sel[...] = functools.reduce(jnp.add, picked).astype(_BF16)

    def ffn_steps(chunk):
        hidden = []

        def up():
            g, u = (_dot(x_sel[...], _slab(w)) for w in ffn_w[:2])
            hidden.append(jnp.where(chunk < n_chunks, g * jax.nn.sigmoid(g) * u, 0.0))

        def down():
            y_sel[...] += _dot(hidden.pop().astype(_BF16), _slab(ffn_w[2]), _NT)
        return {"up": up, "down": down}

    def add_routed_update():
        yT = jnp.concatenate([y_sel[...], jnp.zeros((_T - _ROWS, M), _F32)], axis=0).T
        for n in range(_CAPACITY):
            index = routed[n]
            x = xT[:, tile_of(index)].astype(_F32)
            y = yT[:, n:n + 1] * y_scale[n:n + 1]
            xT[:, tile_of(index)] = jnp.where(lane == index % _T, x + y, x).astype(xT.dtype)

    def seven_products(cost, product, finish):
        m = []

        def step(j):
            m.append(product(j))
            if j == 6:
                finish(*_combine(*m))
        return [(cost, functools.partial(step, j)) for j in range(7)]

    def c_operand(j, u0, u1):
        return _cat([_cat([_slab(c_ops[u], j, t) for t in range(kt)], 1) for u in range(u0, u1)], 0)

    def project_k(u0, u1):
        def finish(ka0, ka1, kb0, kb1):
            for j, op in enumerate(_lhs_operands(kb0, kb1, ka0, ka1) + (kb1, ka0)):
                for u in range(u0, u1):
                    k_ops[u][j] = op[tile(u - u0)].astype(_BF16)
        product = lambda j: _dot(c_operand(j, u0, u1), _slab(wk_ops, j))
        return seven_products(kt * (u1 - u0) * _T, product, finish)

    def project_q(u0, u1):
        m = []

        def step(j):
            if j < 7:
                x = _cat([_slab(x_ops[u], j) for u in range(u0, u1)], 1)
            else:
                groups = ((0, 1), (0, 2), (1, 2))[j - 7]
                x = _cat([xT[2 * _T + g * _T // 2:2 * _T + (g + 1) * _T // 2, 2 * u0 * _T:2 * u1 * _T]
                          for g in groups], 0)
            m.append(_dot(_slab(wq_ops, j), x))
            if j == 9:
                finish()

        def finish():
            main = _combine(*m[:7])
            rest = (m[7] + m[9], m[8] + m[9])
            for u in range(u0, u1):
                qa0, qa1, qb0, qb1 = (
                    (part[:, tile(u - u0)] + rest[i % 2][:, tile(2 * (u - u0) + i // 2)]) * (D ** -0.5 * _LOG2E)
                    for i, part in enumerate(main))
                for j, op in enumerate(_rhs_operands(qa0, qb0, qa1, qb1) + (qb0, qa1)):
                    q_ops[u][j] = op.astype(_BF16)
        return [((1 + (j > 6)) * (u1 - u0) * _T, functools.partial(step, j)) for j in range(10)]

    def project_v(u0, u1):
        def product(j):
            return _dot(_cat([_slab(wv_ops, j)[tile(t)] for t in range(kt)], 1), c_operand(j, u0, u1), _NT)

        def finish(va0, va1, vb0, vb1):
            for j, op in enumerate(_lhs_operands(vb0, va0, vb1, va1) + (va0, vb1)):
                for u in range(u0, u1):
                    v_ops[u][j] = op[:, tile(u - u0)].astype(_BF16)
        return seven_products(kt * (u1 - u0) * _T, product, finish)

    out_product = lambda u, j: _dot(_slab(wo_ops, j), _slab(ctx_ops[u], j))

    def project_out(u, _):
        def step(j):
            acc[u][j] += out_product(u, j)
        return [(mh, functools.partial(step, j)) for j in range(7)]

    def run(program, actions):
        ranged = {"K": project_k, "Q": project_q, "V": project_v, "O": project_out, "R": score_tokens}

        def steps(word):
            if word in actions:
                return [(1e-3, actions[word])]
            lo, _, hi = word[1:].partition("-")
            return ranged[word[0]](int(lo), int(hi) if hi else int(lo) + 1)
        for phase in program.split(";"):
            for step in _interleave([[s for word in part.split() for s in steps(word)]
                                     for part in phase.split("|")]):
                step()

    def causal(s):
        key = lax.broadcasted_iota(jnp.int32, (_T, _T), 0)
        query = lax.broadcasted_iota(jnp.int32, (_T, _T), 1)
        return jnp.where(key <= query, s, -1e9 * _LOG2E)

    def weighted_values(u, scores):
        p, total, m, balance = {}, {}, {}, []

        def softmax():
            s = scores()
            exponent = {}
            for half in "ab":
                names = [name for name in s if name[1] == half]
                peaks = [peak for name in (names[::-1] if half in _REVERSED_MAX[u] else names)
                         for peak in _fold(jnp.maximum, s[name], _T)]
                top = jnp.max(functools.reduce(jnp.maximum, peaks), axis=0, keepdims=True)
                p.update({name: jnp.exp2(s[name] - top) for name in names})
                sums = [x for name in names for x in _fold(jnp.add, p[name], _SUM_ROWS[u])]
                total[half] = jnp.sum(functools.reduce(jnp.add, sums), axis=0, keepdims=True)
                estimate = functools.reduce(jnp.add, [jnp.exp2(peak - top) for peak in peaks])
                estimate = jnp.sum(estimate, axis=0, keepdims=True)
                exponent[half] = pltpu.bitcast(estimate, jnp.int32) >> 23
            balance.append(pltpu.bitcast((exponent["a"] - exponent["b"] + 127) << 23, _F32))

        def step(into, v, t, probs):
            if not p:
                softmax()
            product = _dot(_slab(v_ops[t], v), probs(lambda name: p[name][tile(t)]).astype(_BF16))
            m[into] = m[into] + product if into in m else product

        def finish():
            c0a, c0b, c1a, c1b = m["0a"], m["0b"], m["1a"], m["1b"]
            fa, fb = (gate[2 * u + i:2 * u + i + 1] / total[half] for i, half in enumerate("ab"))
            f1b = fb
            if u:
                w = balance[0]
                c0a, c0b = c0a + (m[3] - w * m[4]) + m[0], c0b + m[2] + m[4]
                c1a, c1b = c1a + m[1] + m[3], w * (c1b + m[2]) + (m[5] - m[1]) + m[0]
                f1b = fb / w
            for j, op in enumerate(_rhs_operands(c0a * fa, c0b * fb, c1a * fa, c1b * f1b)):
                ctx_ops[u][j] = op.astype(_BF16)

        def rhs(j):
            def operand(get):
                w = (lambda x: balance[0] * x) if j in (0, 5, 6) else (lambda x: x)
                return _rhs_operands(get("ba"), w(get("bb")), get("aa"), w(get("ab")))[j]
            return operand

        diagonal = [("0a", 7, "aa"), ("0b", 7, "ab"), ("0b", 2, "bb"),
                    ("1a", 3, "aa"), ("1b", 3, "ab"), ("1b", 8, "bb")]
        steps = []
        for j in map(int, _PV_ORDER[u]):
            if j == 7:
                steps += [functools.partial(step, into, v, u, lambda get, name=name: get(name))
                          for into, v, name in (diagonal[int(i)] for i in _DIAGONAL_ORDER[u])]
            else:
                into = "0a" if j == 6 else j
                steps += [functools.partial(step, into, j, t, rhs(j)) for t in range(u)]
        last = steps.pop()
        return steps + [lambda: (last(), finish())]

    def attention():
        load, pending = [0] * 4, []

        def issue(tiles, step):
            load[load.index(min(load))] += tiles
            return step()

        def level():
            while pending and min(load) < max(load):
                issue(1, pending.pop(0))

        below, diagonal = {}, {}

        def diagonal_scores(u):
            def product(name, k, q):
                m = _dot(_slab(k_ops[u], k), _slab(q_ops[u], q))
                diagonal[u, name] = diagonal[u, name] + m if (u, name) in diagonal else m
            return [functools.partial(product, *spec) for spec in (
                ("aa", 8, 1), ("aa", 3, 8), ("ab", 8, 7), ("ab", 3, 4), ("bb", 2, 7), ("bb", 7, 4))]

        def scores(u):
            def product(j):
                keys = lambda: _cat([_slab(k_ops[t], j) for t in range(u)], 0)
                return issue(u, lambda: _dot(keys(), _slab(q_ops[u], j)))
            m = {}
            for group in _SCORE_GROUPS[u].split():
                m.update({j: product(j) for j in map(int, group)})
                level()
            m1, m2, m3, m4, m5, m6, m7 = (m[j] for j in range(7))
            if "024" in _SCORE_GROUPS[u]:
                below[u] = dict(aa=m2 + m4, ba=(m4 + m7) + (m1 - m5), bb=m3 + m5, ab=(m6 - m2) + (m1 + m3))
            else:
                below[u] = dict(aa=m2 + m4, ba=(m7 - m5) + (m1 + m4), bb=m3 + m5, ab=(m6 + m3) + (m1 - m2))

        def all_scores(u):
            s = dict(aa=causal(diagonal[u, "aa"]), bb=causal(diagonal[u, "bb"]), ab=diagonal[u, "ab"])
            if u:
                s = {name: _cat([part] + ([s[name]] if name in s else []), 0)
                     for name, part in below[u].items()}
            return s

        for word in _ATTENTION.split():
            if word[0] == "S":
                scores(int(word[1:]))
            elif word[0] == "-":
                while len(pending) >= 4 + int(word[1:]):
                    for _ in range(4):
                        issue(1, pending.pop(0))
            else:
                u, _, n = word[1:].partition("@")
                steps = (diagonal_scores(int(u)) if word[0] == "D"
                         else weighted_values(int(u), functools.partial(all_scores, int(u))))
                n = min(int(n or 0), len(pending), len(steps))
                tail = [pending.pop() for _ in range(n)][::-1]
                pending.extend([step for pair in zip(tail, steps) for step in pair] + steps[n:])
        for step in pending:
            step()

    for name in _FIRST_COPIES.split():
        for copy in io[name]:
            copy.start()
    for ref in (*acc, y_sel):
        ref[...] = jnp.zeros_like(ref)
    actions = {"!" + name: functools.partial(wait, name) for name in io}
    actions.update({name: functools.partial(prepare_weight, name, 0, True) for name in weights})
    actions.update({f"c{u}": functools.partial(prepare_c, u) for u in range(U)})
    actions.update(x=prepare_x, route=route)
    run(_FIRST_PROJECTIONS, actions)
    for copy in head_copies(0):
        copy.start()

    def head(h, carry):
        attention()
        for copy in head_copies(h):
            copy.wait()

        @pl.when(h + 1 < H)
        def _():
            actions = {name: functools.partial(prepare_weight, name, h + 1, False) for name in weights}
            run(_PROJECTIONS, dict(actions, wo=prepare_wo, **ffn_steps(h)))
            for copy in head_copies(h + 1):
                copy.start()
        return carry

    lax.fori_loop(0, H, head, None)

    prepare_wo()
    add_routed_update()
    for u in range(U):
        attended = _combine(*(acc[u][j] + out_product(u, j) for j in range(7)))
        keep = 1.0 - jnp.concatenate([gate[2 * u:2 * u + 1], gate[2 * u + 1:2 * u + 2]], axis=1)
        for f in range(2):
            rows = slice(f * mh, (f + 1) * mh)
            mixed = (keep * xT[rows, block(u)].astype(_F32)
                     + jnp.concatenate(attended[2 * f:2 * f + 2], axis=1))
            outT[rows, block(u)] = mixed.astype(outT.dtype)
        io[f"out{u}"][0].start()
    for u in range(U):
        wait(f"out{u}")


@jax.jit
def pallas_gated_mix__compressed_kv_cla__moe_arch_mod__prompt_kernel(
    A_x: jax.Array,
    A_c_kv: jax.Array,
    A_w_q: jax.Array,
    A_w_uk: jax.Array,
    A_w_uv: jax.Array,
    A_w_o: jax.Array,
    B_x: jax.Array,
    B_w_r: jax.Array,
    B_w_gate: jax.Array,
    B_w_up: jax.Array,
    B_w_down: jax.Array,
    gate_w: jax.Array,
):
    del B_x
    _, S, M = A_x.shape
    Dc, H, D = A_w_uk.shape
    U = S // (2 * _T)
    assert (D, U, M) == (2 * _T, 8, 7 * _T // 2) and B_w_gate.shape[1] // _T < H
    vmem = pltpu.VMEM
    tiles = lambda n: [vmem((n, _T, _T), _BF16)] * U
    hbm = pl.BlockSpec(memory_space=pl.ANY)
    outT = pl.pallas_call(
        _kernel,
        in_specs=[hbm] * 11,
        out_specs=hbm,
        out_shape=jax.ShapeDtypeStruct((M, S), A_x.dtype),
        scratch_shapes=[
            vmem((M, S), _BF16), vmem((S, Dc), _BF16), vmem((M,), _BF16), vmem((M,), _BF16),
            [vmem((n, D), _U32) for n in (M, Dc, Dc)],
            [vmem((2, n, _T), _U32) for n in (M, Dc, Dc)],
            vmem((M, D), _BF16), [vmem((M, _T), _BF16)] * 3, vmem((M, S), _BF16),
            pltpu.SemaphoreType.DMA((6 + 2 * U,)), pltpu.SemaphoreType.DMA((10,)),
            tiles(7), [vmem((7, Dc // 2 // _T, _T, _T), _BF16)] * U,
            vmem((10, _T, _T), _BF16), vmem((7, Dc // 2, _T), _BF16),
            vmem((7, Dc // 2, _T), _BF16), vmem((7, M // 2, _T), _BF16),
            tiles(9), tiles(9), tiles(9), tiles(7), [vmem((7, M // 2, _T), _F32)] * U,
            vmem((2 * U, _T), _F32), vmem((2 * U, _T), _F32),
            vmem((_ROWS, M), _BF16), vmem((_ROWS, M), _F32), vmem((_CAPACITY, _T), _F32),
            pltpu.SMEM((_CAPACITY,), jnp.int32),
        ],
        compiler_params=pltpu.CompilerParams(
            vmem_limit_bytes=100 * 2**20, disable_bounds_checks=True),
        name="gm_kernel",
    )(A_x.reshape(S, M).T, A_c_kv.reshape(S, Dc), A_w_q, A_w_uk, A_w_uv, A_w_o.transpose(0, 2, 1),
      B_w_r, B_w_gate, B_w_up, B_w_down.T, gate_w)
    return outT.T.reshape(A_x.shape)
```

```python
import functools
import math

import jax
import jax.numpy as jnp
import numpy as np
from jax import lax
import jax.experimental.pallas as pl
import jax.experimental.pallas.tpu as pltpu

_NN = (((1,), (0,)), ((), ()))
_NT = (((1,), (1,)), ((), ()))
_F32 = jnp.float32
_BF16 = jnp.bfloat16
_U32 = jnp.uint32
_LOG2E = math.log2(math.e)
_T = 128
_ROWS = 16
_CAPACITY = 2

_FIRST_COPIES = "wv c0 wk c1 c2 c3 c4 c5 c6 c7 vec wq x"
_FIRST_PROJECTIONS = (
    "!wv wv !c0 c0 V0 !wk wk K0 !c1 c1 K1 V1 !c2 !c3 c2 c3 K2-4 V2-4"
    " !c4 !c5 !c6 c4 c5 c6 V4-6 V6 K4-6 !c7 !vec !wq !x c7 wq x;"
    " K6 | R0-8; K7 | Q0 Q1 Q2 Q3; route; V7 | Q4 Q5 Q6 Q7")
_PROJECTIONS = (
    "wo wk wq wv O0 O1 O2;"
    " K0-2 K2-8 V0-2 V2-4 V4-6 V6-8 | up O3 Q0 Q1 down Q2 Q3 Q4 O4 Q5 Q6 Q7; O5 O6 O7")
_ATTENTION = (
    "S1 D0@4 D3@0 D1@6 S2 D2@2 -0 C1@2 D4@8 S3 -1 C2@2 S4 C0@0 D5@0"
    " -3 S5 C3@6 D6@0 -5 C4@2 D7@2 S6 -3 S7 -3 C5@8 C7@2 C6@0")
_SCORE_GROUPS = ("1356 024", "024 1356", "024 1356", "1356 024",
                 "1356 024", "1356 024", "2456 013", "1356 024")
_REVERSED_MAX = ("", "b", "a", "ab", "a", "", "", "")
_SUM_ROWS = (64, 16, 16, 1024, 256, 32, 256, 16)
_PV_ORDER = ("41063527", "41520367", "14325760", "14036752",
             "41073265", "41076523", "41023576", "14275063")
_DIAGONAL_ORDER = ("302145", "253401", "314502", "432150", "035421", "435120", "102354", "130245")


def _dot(a, b, dims=_NN):
    return lax.dot_general(a, b, dims, preferred_element_type=_F32)


def _lhs_operands(a11, a12, a21, a22):
    return (a11 + a22, a21 + a22, a11, a22, a11 + a12, a21 - a11, a12 - a22)


def _rhs_operands(b11, b12, b21, b22):
    return (b11 + b22, b11, b12 - b22, b21 - b11, b22, b11 + b12, b21 + b22)


def _combine(m1, m2, m3, m4, m5, m6, m7):
    return m1 + m4 - m5 + m7, m3 + m5, m2 + m4, m1 - m2 + m3 + m6


def _slab(ref, *lead):
    return pltpu.bitcast(ref.bitcast(_U32)[(*lead, slice(None), slice(None))], _BF16)


def _cat(xs, axis):
    return xs[0] if len(xs) == 1 else jnp.concatenate(xs, axis=axis)


def _fold(op, x, rows):
    return [functools.reduce(op, [x[r:r + 8] for r in range(lo, min(lo + rows, x.shape[0]), 8)])
            for lo in range(0, x.shape[0], rows)]


def _interleave(streams):
    keyed = []
    for steps in streams:
        total, done = sum(cost for cost, _ in steps), 0
        for cost, step in steps:
            keyed.append(((done + cost / 2) / total, len(keyed), step))
            done += cost
    return [step for _, _, step in sorted(keyed, key=lambda item: item[:2])]


def _kernel(
    xT_hbm, c_hbm, wq_hbm, wuk_hbm, wuv_hbm, woT_hbm, wr_hbm, wg_hbm, wu_hbm, wdT_hbm, gw_hbm,
    outT_hbm,
    xT, c, wr, gw, first_words, next_words, woT, ffn_w, outT, io_sems, head_sems,
    x_ops, c_ops, wq_ops, wk_ops, wv_ops, wo_ops, q_ops, k_ops, v_ops, ctx_ops, acc,
    gate, score, x_sel, y_sel, y_scale, routed,
):
    M, S = xT.shape
    Dc, H, D = wuk_hbm.shape
    U = S // (2 * _T)
    n_chunks = wg_hbm.shape[1] // _T
    mh, kt = M // 2, Dc // 2 // _T
    block = lambda u: slice(2 * u * _T, 2 * (u + 1) * _T)
    tile = lambda t: slice(t * _T, (t + 1) * _T)
    weights = {"wq": (0, wq_hbm, wq_ops), "wk": (1, wuk_hbm, wk_ops), "wv": (2, wuv_hbm, wv_ops)}

    io = {name: [(src.bitcast(_U32).at[:, 0, :], first_words[i])]
          for name, (i, src, _) in weights.items()}
    io["x"] = [(xT_hbm, xT)]
    io["vec"] = [(wr_hbm, wr), (gw_hbm, gw)]
    for u in range(U):
        io[f"c{u}"] = [(c_hbm.at[block(u)], c.at[block(u)])]
        io[f"out{u}"] = [(outT.at[:, block(u)], outT_hbm.at[:, block(u)])]
    slots = iter(range(io_sems.shape[0]))
    io = {name: [pltpu.make_async_copy(src, dst, io_sems.at[next(slots)]) for src, dst in pairs]
          for name, pairs in io.items()}

    def wait(name):
        for copy in io[name]:
            copy.wait()

    def head_copies(h):
        if isinstance(h, int):
            pair, chunk = (h + 1) // 2, tile(h)
        else:
            pair = jnp.minimum(h + 1, H - 1) // 2
            chunk = pl.ds(pl.multiple_of(jnp.minimum(h, n_chunks - 1) * _T, _T), _T)
        pairs = [(woT_hbm.at[h], woT)]
        pairs += [(src.bitcast(_U32).at[:, pair, tile(n)], next_words[i].at[n])
                  for i, src, _ in weights.values() for n in range(2)]
        pairs += [(src.at[:, chunk], dst) for src, dst in zip((wg_hbm, wu_hbm, wdT_hbm), ffn_w)]
        return [pltpu.make_async_copy(src, dst, head_sems.at[i]) for i, (src, dst) in enumerate(pairs)]

    def prepare_weight(name, head, first):
        i, src, dst = weights[name]
        transposed = name != "wk"
        shift = np.uint32(16) if first else (16 * (1 - head % 2)).astype(_U32)

        def load(lo, n_rows, n, transposed):
            rows = slice(lo, lo + n_rows)
            words = first_words[i][rows, tile(n)] if first else next_words[i][n, rows]
            words = words.T if transposed else words
            return pltpu.bitcast((words << shift) & np.uint32(0xFFFF0000), _F32)

        half = _T if name == "wq" else src.shape[0] // 2
        step = _T if transposed else _ROWS
        for r in range(0, half, step):
            quads = [load(f * half + r, step, n, transposed) for f in range(2) for n in range(2)]
            for j, op in enumerate(_rhs_operands(*quads)):
                dst[j, r:r + step] = op.astype(_BF16)
        if name == "wq":
            (w10, w11), (w20, w21), (w30, w31) = (
                [load(2 * _T + g * _T // 2, _T // 2, n, False) for n in range(2)] for g in range(3))
            for j, parts in enumerate(((w10, w20 - w21), (w11, w31 - w30), (w21, w30))):
                dst[7 + j] = jnp.concatenate(parts, axis=0).T.astype(_BF16)

    def prepare_wo():
        for r in range(0, mh, _ROWS):
            top, bottom = (woT[f * mh + r:f * mh + r + _ROWS].astype(_F32) for f in range(2))
            for j, op in enumerate(_lhs_operands(top[:, :_T], top[:, _T:], bottom[:, :_T], bottom[:, _T:])):
                wo_ops[j, r:r + _ROWS] = op.astype(_BF16)

    def prepare_c(u):
        for r in range(0, _T, _ROWS):
            ca, cb = (c[(2 * u + f) * _T + r:(2 * u + f) * _T + r + _ROWS].astype(_F32) for f in range(2))
            ops = _lhs_operands(ca[:, :Dc // 2], ca[:, Dc // 2:], cb[:, :Dc // 2], cb[:, Dc // 2:])
            for j, op in enumerate(ops):
                for t in range(kt):
                    c_ops[u][j, t, r:r + _ROWS] = op[:, tile(t)].astype(_BF16)

    def prepare_x():
        for u in range(U):
            for r in range(0, _T, _ROWS):
                x0, x1 = (xT[f * _T + r:f * _T + r + _ROWS, block(u)].astype(_F32) for f in range(2))
                for j, op in enumerate(_lhs_operands(x0[:, :_T], x1[:, :_T], x0[:, _T:], x1[:, _T:])):
                    x_ops[u][j, r:r + _ROWS] = op.astype(_BF16)

    lane = lax.broadcasted_iota(jnp.int32, (1, _T), 1)
    tile_of = lambda token: pl.ds(pl.multiple_of(token // _T * _T, _T), _T)

    def score_tokens(u0, u1):
        def step(t):
            row = lax.broadcasted_iota(jnp.int32, (_ROWS, M), 0)
            vectors = jnp.where(row == 0, *(v[...].astype(_F32).reshape(1, M) for v in (wr, gw)))
            dots = _dot(vectors.astype(_BF16), xT[:, tile(t)])
            score[t:t + 1] = dots[0:1].astype(xT.dtype).astype(_F32)
            gate[t:t + 1] = jax.nn.sigmoid(dots[1:2])
        return [(1, functools.partial(step, t)) for t in range(2 * u0, 2 * u1)]

    def route():
        r = score[...]
        r = jnp.where(r == r, r, -jnp.inf)
        token = (lax.broadcasted_iota(jnp.int32, r.shape, 0) * _T
                 + lax.broadcasted_iota(jnp.int32, r.shape, 1)).astype(_F32)
        free = token >= 0
        slot = lax.broadcasted_iota(jnp.int32, (_ROWS, _T), 0)
        picked = []
        for n in range(_CAPACITY):
            best = jnp.max(jnp.where(free, r, -jnp.inf), keepdims=True)
            choice = jnp.min(jnp.where(free & (r == best), token, S - 1.0))
            free = free & (token != choice)
            index = choice.astype(jnp.int32)
            routed[n] = index
            y_scale[n:n + 1] = jnp.broadcast_to(jax.nn.sigmoid(best), (1, _T))
            onehot = jnp.where((slot == n) & (lane == index % _T), 1.0, 0.0)
            picked.append(_dot(onehot.astype(_BF16), xT[:, tile_of(index)], _NT))
        x_sel[...] = functools.reduce(jnp.add, picked).astype(_BF16)

    def ffn_steps(chunk):
        hidden = []

        def up():
            g, u = (_dot(x_sel[...], _slab(w)) for w in ffn_w[:2])
            hidden.append(jnp.where(chunk < n_chunks, g * jax.nn.sigmoid(g) * u, 0.0))

        def down():
            y_sel[...] += _dot(hidden.pop().astype(_BF16), _slab(ffn_w[2]), _NT)
        return {"up": up, "down": down}

    def add_routed_update():
        yT = jnp.concatenate([y_sel[...], jnp.zeros((_T - _ROWS, M), _F32)], axis=0).T
        for n in range(_CAPACITY):
            index = routed[n]
            x = xT[:, tile_of(index)].astype(_F32)
            y = yT[:, n:n + 1] * y_scale[n:n + 1]
            xT[:, tile_of(index)] = jnp.where(lane == index % _T, x + y, x).astype(xT.dtype)

    def seven_products(cost, product, finish):
        m = []

        def step(j):
            m.append(product(j))
            if j == 6:
                finish(*_combine(*m))
        return [(cost, functools.partial(step, j)) for j in range(7)]

    def c_operand(j, u0, u1):
        return _cat([_cat([_slab(c_ops[u], j, t) for t in range(kt)], 1) for u in range(u0, u1)], 0)

    def project_k(u0, u1):
        def finish(ka0, ka1, kb0, kb1):
            for j, op in enumerate(_lhs_operands(kb0, kb1, ka0, ka1) + (kb1, ka0)):
                for u in range(u0, u1):
                    k_ops[u][j] = op[tile(u - u0)].astype(_BF16)
        product = lambda j: _dot(c_operand(j, u0, u1), _slab(wk_ops, j))
        return seven_products(kt * (u1 - u0) * _T, product, finish)

    def project_q(u0, u1):
        m = []

        def step(j):
            if j < 7:
                x = _cat([_slab(x_ops[u], j) for u in range(u0, u1)], 1)
            else:
                groups = ((0, 1), (0, 2), (1, 2))[j - 7]
                x = _cat([xT[2 * _T + g * _T // 2:2 * _T + (g + 1) * _T // 2, 2 * u0 * _T:2 * u1 * _T]
                          for g in groups], 0)
            m.append(_dot(_slab(wq_ops, j), x))
            if j == 9:
                finish()

        def finish():
            main = _combine(*m[:7])
            rest = (m[7] + m[9], m[8] + m[9])
            for u in range(u0, u1):
                qa0, qa1, qb0, qb1 = (
                    (part[:, tile(u - u0)] + rest[i % 2][:, tile(2 * (u - u0) + i // 2)]) * (D ** -0.5 * _LOG2E)
                    for i, part in enumerate(main))
                for j, op in enumerate(_rhs_operands(qa0, qb0, qa1, qb1) + (qb0, qa1)):
                    q_ops[u][j] = op.astype(_BF16)
        return [((1 + (j > 6)) * (u1 - u0) * _T, functools.partial(step, j)) for j in range(10)]

    def project_v(u0, u1):
        def product(j):
            return _dot(_cat([_slab(wv_ops, j)[tile(t)] for t in range(kt)], 1), c_operand(j, u0, u1), _NT)

        def finish(va0, va1, vb0, vb1):
            for j, op in enumerate(_lhs_operands(vb0, va0, vb1, va1) + (va0, vb1)):
                for u in range(u0, u1):
                    v_ops[u][j] = op[:, tile(u - u0)].astype(_BF16)
        return seven_products(kt * (u1 - u0) * _T, product, finish)

    out_product = lambda u, j: _dot(_slab(wo_ops, j), _slab(ctx_ops[u], j))

    def project_out(u, _):
        def step(j):
            acc[u][j] += out_product(u, j)
        return [(mh, functools.partial(step, j)) for j in range(7)]

    def run(program, actions):
        ranged = {"K": project_k, "Q": project_q, "V": project_v, "O": project_out, "R": score_tokens}

        def steps(word):
            if word in actions:
                return [(1e-3, actions[word])]
            lo, _, hi = word[1:].partition("-")
            return ranged[word[0]](int(lo), int(hi) if hi else int(lo) + 1)
        for phase in program.split(";"):
            for step in _interleave([[s for word in part.split() for s in steps(word)]
                                     for part in phase.split("|")]):
                step()

    def causal(s):
        key = lax.broadcasted_iota(jnp.int32, (_T, _T), 0)
        query = lax.broadcasted_iota(jnp.int32, (_T, _T), 1)
        return jnp.where(key <= query, s, -1e9 * _LOG2E)

    def weighted_values(u, scores):
        p, total, m, balance = {}, {}, {}, []

        def softmax():
            s = scores()
            exponent = {}
            for half in "ab":
                names = [name for name in s if name[1] == half]
                peaks = [peak for name in (names[::-1] if half in _REVERSED_MAX[u] else names)
                         for peak in _fold(jnp.maximum, s[name], _T)]
                top = jnp.max(functools.reduce(jnp.maximum, peaks), axis=0, keepdims=True)
                p.update({name: jnp.exp2(s[name] - top) for name in names})
                sums = [x for name in names for x in _fold(jnp.add, p[name], _SUM_ROWS[u])]
                total[half] = jnp.sum(functools.reduce(jnp.add, sums), axis=0, keepdims=True)
                estimate = functools.reduce(jnp.add, [jnp.exp2(peak - top) for peak in peaks])
                estimate = jnp.sum(estimate, axis=0, keepdims=True)
                exponent[half] = pltpu.bitcast(estimate, jnp.int32) >> 23
            balance.append(pltpu.bitcast((exponent["a"] - exponent["b"] + 127) << 23, _F32))

        def step(into, v, t, probs):
            if not p:
                softmax()
            product = _dot(_slab(v_ops[t], v), probs(lambda name: p[name][tile(t)]).astype(_BF16))
            m[into] = m[into] + product if into in m else product

        def finish():
            c0a, c0b, c1a, c1b = m["0a"], m["0b"], m["1a"], m["1b"]
            fa, fb = (gate[2 * u + i:2 * u + i + 1] / total[half] for i, half in enumerate("ab"))
            f1b = fb
            if u:
                w = balance[0]
                c0a, c0b = c0a + (m[3] - w * m[4]) + m[0], c0b + m[2] + m[4]
                c1a, c1b = c1a + m[1] + m[3], w * (c1b + m[2]) + (m[5] - m[1]) + m[0]
                f1b = fb / w
            for j, op in enumerate(_rhs_operands(c0a * fa, c0b * fb, c1a * fa, c1b * f1b)):
                ctx_ops[u][j] = op.astype(_BF16)

        def rhs(j):
            def operand(get):
                w = (lambda x: balance[0] * x) if j in (0, 5, 6) else (lambda x: x)
                return _rhs_operands(get("ba"), w(get("bb")), get("aa"), w(get("ab")))[j]
            return operand

        diagonal = [("0a", 7, "aa"), ("0b", 7, "ab"), ("0b", 2, "bb"),
                    ("1a", 3, "aa"), ("1b", 3, "ab"), ("1b", 8, "bb")]
        steps = []
        for j in map(int, _PV_ORDER[u]):
            if j == 7:
                steps += [functools.partial(step, into, v, u, lambda get, name=name: get(name))
                          for into, v, name in (diagonal[int(i)] for i in _DIAGONAL_ORDER[u])]
            else:
                into = "0a" if j == 6 else j
                steps += [functools.partial(step, into, j, t, rhs(j)) for t in range(u)]
        last = steps.pop()
        return steps + [lambda: (last(), finish())]

    def attention():
        load, pending = [0] * 4, []

        def issue(tiles, step):
            load[load.index(min(load))] += tiles
            return step()

        def level():
            while pending and min(load) < max(load):
                issue(1, pending.pop(0))

        below, diagonal = {}, {}

        def diagonal_scores(u):
            def product(name, k, q):
                m = _dot(_slab(k_ops[u], k), _slab(q_ops[u], q))
                diagonal[u, name] = diagonal[u, name] + m if (u, name) in diagonal else m
            return [functools.partial(product, *spec) for spec in (
                ("aa", 8, 1), ("aa", 3, 8), ("ab", 8, 7), ("ab", 3, 4), ("bb", 2, 7), ("bb", 7, 4))]

        def scores(u):
            def product(j):
                keys = lambda: _cat([_slab(k_ops[t], j) for t in range(u)], 0)
                return issue(u, lambda: _dot(keys(), _slab(q_ops[u], j)))
            m = {}
            for group in _SCORE_GROUPS[u].split():
                m.update({j: product(j) for j in map(int, group)})
                level()
            m1, m2, m3, m4, m5, m6, m7 = (m[j] for j in range(7))
            if "024" in _SCORE_GROUPS[u]:
                below[u] = dict(aa=m2 + m4, ba=(m4 + m7) + (m1 - m5), bb=m3 + m5, ab=(m6 - m2) + (m1 + m3))
            else:
                below[u] = dict(aa=m2 + m4, ba=(m7 - m5) + (m1 + m4), bb=m3 + m5, ab=(m6 + m3) + (m1 - m2))

        def all_scores(u):
            s = dict(aa=causal(diagonal[u, "aa"]), bb=causal(diagonal[u, "bb"]), ab=diagonal[u, "ab"])
            if u:
                s = {name: _cat([part] + ([s[name]] if name in s else []), 0)
                     for name, part in below[u].items()}
            return s

        for word in _ATTENTION.split():
            if word[0] == "S":
                scores(int(word[1:]))
            elif word[0] == "-":
                while len(pending) >= 4 + int(word[1:]):
                    for _ in range(4):
                        issue(1, pending.pop(0))
            else:
                u, _, n = word[1:].partition("@")
                steps = (diagonal_scores(int(u)) if word[0] == "D"
                         else weighted_values(int(u), functools.partial(all_scores, int(u))))
                n = min(int(n or 0), len(pending), len(steps))
                tail = [pending.pop() for _ in range(n)][::-1]
                pending.extend([step for pair in zip(tail, steps) for step in pair] + steps[n:])
        for step in pending:
            step()

    for name in _FIRST_COPIES.split():
        for copy in io[name]:
            copy.start()
    for ref in (*acc, y_sel):
        ref[...] = jnp.zeros_like(ref)
    actions = {"!" + name: functools.partial(wait, name) for name in io}
    actions.update({name: functools.partial(prepare_weight, name, 0, True) for name in weights})
    actions.update({f"c{u}": functools.partial(prepare_c, u) for u in range(U)})
    actions.update(x=prepare_x, route=route)
    run(_FIRST_PROJECTIONS, actions)
    for copy in head_copies(0):
        copy.start()

    def head(h, carry):
        attention()
        for copy in head_copies(h):
            copy.wait()

        @pl.when(h + 1 < H)
        def _():
            actions = {name: functools.partial(prepare_weight, name, h + 1, False) for name in weights}
            run(_PROJECTIONS, dict(actions, wo=prepare_wo, **ffn_steps(h)))
            for copy in head_copies(h + 1):
                copy.start()
        return carry

    lax.fori_loop(0, H, head, None)

    prepare_wo()
    add_routed_update()
    for u in range(U):
        attended = _combine(*(acc[u][j] + out_product(u, j) for j in range(7)))
        keep = 1.0 - jnp.concatenate([gate[2 * u:2 * u + 1], gate[2 * u + 1:2 * u + 2]], axis=1)
        for f in range(2):
            rows = slice(f * mh, (f + 1) * mh)
            mixed = (keep * xT[rows, block(u)].astype(_F32)
                     + jnp.concatenate(attended[2 * f:2 * f + 2], axis=1))
            outT[rows, block(u)] = mixed.astype(outT.dtype)
        io[f"out{u}"][0].start()
    for u in range(U):
        wait(f"out{u}")


@jax.jit
def pallas_gated_mix__compressed_kv_cla__moe_arch_mod__prompt_kernel(
    A_x: jax.Array,
    A_c_kv: jax.Array,
    A_w_q: jax.Array,
    A_w_uk: jax.Array,
    A_w_uv: jax.Array,
    A_w_o: jax.Array,
    B_x: jax.Array,
    B_w_r: jax.Array,
    B_w_gate: jax.Array,
    B_w_up: jax.Array,
    B_w_down: jax.Array,
    gate_w: jax.Array,
):
    del B_x
    _, S, M = A_x.shape
    Dc, H, D = A_w_uk.shape
    U = S // (2 * _T)
    assert (D, U, M) == (2 * _T, 8, 7 * _T // 2) and B_w_gate.shape[1] // _T < H
    vmem = pltpu.VMEM
    tiles = lambda n: [vmem((n, _T, _T), _BF16)] * U
    hbm = pl.BlockSpec(memory_space=pl.ANY)
    outT = pl.pallas_call(
        _kernel,
        in_specs=[hbm] * 11,
        out_specs=hbm,
        out_shape=jax.ShapeDtypeStruct((M, S), A_x.dtype),
        scratch_shapes=[
            vmem((M, S), _BF16), vmem((S, Dc), _BF16), vmem((M,), _BF16), vmem((M,), _BF16),
            [vmem((n, D), _U32) for n in (M, Dc, Dc)],
            [vmem((2, n, _T), _U32) for n in (M, Dc, Dc)],
            vmem((M, D), _BF16), [vmem((M, _T), _BF16)] * 3, vmem((M, S), _BF16),
            pltpu.SemaphoreType.DMA((6 + 2 * U,)), pltpu.SemaphoreType.DMA((10,)),
            tiles(7), [vmem((7, Dc // 2 // _T, _T, _T), _BF16)] * U,
            vmem((10, _T, _T), _BF16), vmem((7, Dc // 2, _T), _BF16),
            vmem((7, Dc // 2, _T), _BF16), vmem((7, M // 2, _T), _BF16),
            tiles(9), tiles(9), tiles(9), tiles(7), [vmem((7, M // 2, _T), _F32)] * U,
            vmem((2 * U, _T), _F32), vmem((2 * U, _T), _F32),
            vmem((_ROWS, M), _BF16), vmem((_ROWS, M), _F32), vmem((_CAPACITY, _T), _F32),
            pltpu.SMEM((_CAPACITY,), jnp.int32),
        ],
        compiler_params=pltpu.CompilerParams(
            vmem_limit_bytes=100 * 2**20, disable_bounds_checks=True),
        name="gm_kernel",
    )(A_x.reshape(S, M).T, A_c_kv.reshape(S, Dc), A_w_q, A_w_uk, A_w_uv, A_w_o.transpose(0, 2, 1),
      B_w_r, B_w_gate, B_w_up, B_w_down.T, gate_w)
    return outT.T.reshape(A_x.shape)
```
